```python
import jax
import jax.numpy as jnp

def _softmax(x, axis=-1):
    return jax.nn.softmax(x, axis=axis)
def _gelu(x):
    return jax.nn.gelu(x, approximate=True)
def _silu(x):
    return jax.nn.silu(x)
def _sigmoid(x):
    return jax.nn.sigmoid(x)
def _layernorm(x, axis=-1, eps=1e-5):
    m = jnp.mean(x, axis=axis, keepdims=True)
    v = jnp.var(x, axis=axis, keepdims=True)
    return (x - m) / jnp.sqrt(v + eps)
def _scatter_add(tgt, idx, src, axis=0):
    return tgt.at[idx].add(src)
def _segment_sum(src, seg, n):
    return jax.ops.segment_sum(src, seg, n)
class _Rng:
    def __init__(self, key):
        self._k = key
    def _next(self):
        self._k, sub = jax.random.split(self._k)
        return sub
    def normal(self, shape):
        return jax.random.normal(self._next(), shape, dtype=jnp.bfloat16)
    def randint(self, lo, hi, shape):
        return jax.random.randint(self._next(), shape, lo, hi, dtype=jnp.int32)
    def uniform(self, shape, lo=0.0, hi=1.0):
        return jax.random.uniform(self._next(), shape, jnp.bfloat16, lo, hi)
    def permutation(self, n):
        return jax.random.permutation(self._next(), n)


kernel_name = 'recurrent_scan__ssm_conv_s4__moe_arch_mod__prompt'

def setup_inputs():
    _rng = _Rng(jax.random.key(int.from_bytes(__import__("os").urandom(4), "little")))
    _w = (lambda a: (lambda t: t.astype(jnp.bfloat16) if jnp.issubdtype(t.dtype, jnp.floating) else t)(jnp.asarray(a)))
    def _A_setup():
        B, L, D, N = 1, 2048, 576, 128
        A_re = -jnp.exp((lambda *s: _rng.normal(s) * 0.05)(D, N))
        A_im = jnp.pi * (lambda *s: _rng.normal(s) * 0.05)(D, N)
        B_re = (lambda *s: _rng.normal(s) * 0.05)(D, N)
        B_im = (lambda *s: _rng.normal(s) * 0.05)(D, N)
        C_re = (lambda *s: _rng.normal(s) * 0.05)(D, N)
        C_im = (lambda *s: _rng.normal(s) * 0.05)(D, N)
        log_dt = (lambda *s: _rng.normal(s) * 0.05)(D) * 0.5 - 4.0
        Dskip = (lambda *s: _rng.normal(s) * 0.05)(D)
        return {
            "u": _w((lambda *s: _rng.normal(s) * 0.05)(B, L, D)),
            "A_re": _w(A_re),
            "A_im": _w(A_im),
            "B_re": _w(B_re),
            "B_im": _w(B_im),
            "C_re": _w(C_re),
            "C_im": _w(C_im),
            "log_dt": _w(log_dt),
            "Dskip": _w(Dskip),
        }
    _A_in = _A_setup()

    def _B_setup():
        B, S, D, F, C = 1, 2048, 576, 4608, 8
        return {
            "x": _w((lambda *s: _rng.normal(s) * 0.05)(B, S, D)),
            "w_r": _w((lambda *s: _rng.normal(s) * 0.05)(D)),
            "w_gate": _w((lambda *s: _rng.normal(s) * 0.05)(D, F)),
            "w_up": _w((lambda *s: _rng.normal(s) * 0.05)(D, F)),
            "w_down": _w((lambda *s: _rng.normal(s) * 0.05)(F, D)),
        }
    _B_in = _B_setup()

    return {
        "A_u": _A_in["u"],
        "A_A_re": _A_in["A_re"],
        "A_A_im": _A_in["A_im"],
        "A_B_re": _A_in["B_re"],
        "A_B_im": _A_in["B_im"],
        "A_C_re": _A_in["C_re"],
        "A_C_im": _A_in["C_im"],
        "A_log_dt": _A_in["log_dt"],
        "A_Dskip": _A_in["Dskip"],
        "B_x": _B_in["x"],
        "B_w_r": _B_in["w_r"],
        "B_w_gate": _B_in["w_gate"],
        "B_w_up": _B_in["w_up"],
        "B_w_down": _B_in["w_down"],
    }

def reference(A_u, A_A_re, A_A_im, A_B_re, A_B_im, A_C_re, A_C_im, A_log_dt, A_Dskip, B_x, B_w_r, B_w_gate, B_w_up, B_w_down):
    def _A_ref(u, A_re, A_im, B_re, B_im, C_re, C_im, log_dt, Dskip):
        Bsz, L, D = u.shape
        dt = jnp.exp(log_dt)[:, None]
        A = A_re + 1j * A_im
        Bc = B_re + 1j * B_im
        Cc = C_re + 1j * C_im
        logdA = dt * A
        dB = dt * Bc
        l = (lambda x, dt: x.astype(dt))(jnp.arange(L), A_re.dtype)
        P = jnp.exp(logdA[:, :, None] * l[None, None, :])
        K = jnp.einsum("dn,dnl,dn->dl", Cc, P, dB).real
        L2 = 2 * L
        Kp = jnp.pad(K, ((0, 0), (0, L)))
        up = (lambda x, *d: x.transpose(*d))(u, 0, 2, 1)
        up = jnp.pad(up, ((0, 0), (0, 0), (0, L)))
        Kf = (lambda x, axes=(-2,-1): jnp.fft.rfft2(x.astype(jnp.float32), axes=axes))(Kp[:, None, :], axes=(-2, -1))
        Uf = (lambda x, axes=(-2,-1): jnp.fft.rfft2(x.astype(jnp.float32), axes=axes))(up[:, :, None, :], axes=(-2, -1))
        Yf = Uf * Kf[None, :, :, :]
        y = (lambda x, s, axes=(-2,-1): jnp.fft.irfft2(x, s=s, axes=axes).astype(jnp.bfloat16))(Yf, (1, L2), axes=(-2, -1))[:, :, 0, :L]
        y = (lambda x, *d: x.transpose(*d))(y, 0, 2, 1) + u * Dskip[None, None, :]
        return y

    def _B_ref(x, w_r, w_gate, w_up, w_down):
        B, S, D = x.shape
        C = 8
        r = x @ w_r
        idx = jnp.argsort(-r, axis=-1)[:, :C]
        idx_e = jnp.repeat(idx.reshape(B, C, 1), D, axis=2)
        x_sel = jnp.take_along_axis(x, idx_e, axis=1)
        g = _silu(x_sel @ w_gate)
        u = x_sel @ w_up
        y = (g * u) @ w_down
        r_sel = _sigmoid(jnp.take_along_axis(r, idx, axis=1))
        y = y * r_sel.reshape(B, C, 1)
        b_off = (jnp.arange(B) * S).reshape(B, 1)
        flat_idx = (idx + b_off).reshape(B * C)
        zero = (x * 0.0).reshape(B * S, D)
        upd = _scatter_add(zero, flat_idx, y.reshape(B * C, D), axis=0)
        return x + upd.reshape(B, S, D)

    x = A_u
    xn = _layernorm(x, axis=-1)
    s = _A_ref(xn, A_A_re, A_A_im, A_B_re, A_B_im, A_C_re, A_C_im, A_log_dt, A_Dskip)
    g = _silu(_B_ref(xn, B_w_r, B_w_gate, B_w_up, B_w_down))
    return x + s * g
```

```python
import math

import jax
import jax.numpy as jnp
from jax import lax
import jax.experimental.pallas as pl
import jax.experimental.pallas.tpu as pltpu

F32, BF16, I32 = jnp.float32, jnp.bfloat16, jnp.int32
L, D, N, F, TOPK = 2048, 576, 128, 4608, 8
G = 16
NG = D // G
EPS = 1e-5
NT = (((1,), (1,)), ((), ()))
DOWN_CHUNKS = ((0, 128), (128, 128), (256, 128), (384, 128), (512, 64))
UP_CHUNKS = 4


def _iota(shape, dim):
    return lax.broadcasted_iota(I32, shape, dim)


def _cmul(a, b):
    return a[0] * b[0] - a[1] * b[1], a[0] * b[1] + a[1] * b[0]


def _csq(a):
    return a[0] * a[0] - a[1] * a[1], (a[0] + a[0]) * a[1]


def _cadd(a, b):
    return a[0] + b[0], a[1] + b[1]


def _csub(a, b):
    return a[0] - b[0], a[1] - b[1]


def _cadd_i(a, b):
    return a[0] - b[1], a[1] + b[0]


def _csub_i(a, b):
    return a[0] + b[1], a[1] - b[0]


def _dft4(v, sign):
    s02, d02 = _cadd(v[0], v[2]), _csub(v[0], v[2])
    s13, d13 = _cadd(v[1], v[3]), _csub(v[1], v[3])
    a, b = _cadd_i(d02, d13), _csub_i(d02, d13)
    if sign < 0:
        a, b = b, a
    return [_cadd(s02, s13), a, _csub(s02, s13), b]


def _root(n):
    ang = (((n + 1024) & 2047) - 1024).astype(F32) * (2.0 * math.pi / 2048)
    return jnp.cos(ang), jnp.sin(ang)


def _pack(x):
    return pltpu.bitcast(x.astype(BF16), I32)


def _bf(x):
    return pltpu.bitcast(x, BF16)


def _round_bf16(x):
    return x.astype(BF16).astype(F32)


def _silu(x):
    h = 0.5 * x
    return h + h * jnp.tanh(h)


def _skew(r):
    lane = _iota(r[0].shape, 1)
    b0, b1 = (lane & 1) != 0, (lane & 2) != 0
    t = [jnp.where(b0, r[(k + 1) % 4], r[k]) for k in range(4)]
    u = [jnp.where(b1, t[(k + 2) % 4], t[k]) for k in range(4)]
    return [u[(-j) % 4] for j in range(4)]


def _x_time(j, m):
    q = (m - j) & 3
    return 128 * q + ((m - q) & 127)


def _column(v_ref, out_ref, fn):
    v = fn(v_ref[...].astype(F32).reshape(1, D))
    for lo in range(0, D, 128):
        n = min(128, D - lo)
        out_ref[pl.ds(lo, n), :] = jnp.broadcast_to(v[:, lo:lo + n], (128, n)).T


def _make_transforms(fx_ref, fxt_ref, fk_ref, fd_ref):
    freq = 4 * _iota((8, 128), 1) + 1
    row = _iota((8, 128), 0)

    def store(ref, idx, cols, vals):
        for c, part in zip(cols, (0, 1)):
            m = jnp.concatenate([v[part] for v in vals], axis=0)
            ref[idx + (slice(None), pl.ds(c, 128))] = _pack(m)

    step8, step32, step1 = _root(8 * freq), _root(32 * freq), _root(freq)
    kbase = _root(4 * row * freq)
    for j in range(4):
        vals = [_root(_x_time(j, row) * freq), _root(_x_time(j, row + 8) * freq)]
        for _ in range(14):
            vals.append(_cmul(vals[-1], step8))
        store(fx_ref, (j,), (0, 128), vals)
        for part in range(2):
            m = jnp.concatenate([v[part] for v in vals], axis=0)
            fxt_ref[j, pl.ds(64 * part, 64), :] = _pack(m.T)
        vals = [kbase]
        for _ in range(15):
            vals.append(_cmul(vals[-1], step32))
        store(fk_ref, (j,), (0, 128), vals)
        kbase = _cmul(kbase, step1)

    rows = [_root((256 * (row & 1) + 8 * (row >> 1)) * freq)]
    for _ in range(7):
        rows.append(_cmul(rows[-1], step32))
    zero = jnp.zeros((8, 128), F32)
    rho = step1
    for k2 in range(4):
        p2 = _csq(rho)
        p3, p4 = _cmul(p2, rho), _csq(p2)
        s3 = _cadd(_cadd(rho, p2), p3)
        s4 = _cadd(s3, p4)
        box = 1.0 + 2.0 * jnp.where((row & 2) == 0, s4[0], s3[0])
        vals = [(r[0] * box, r[1] * box) for r in rows]
        first = row == 0
        vals[0] = (jnp.where(first, 1.0 + s4[0], vals[0][0]),
                   jnp.where(first, s4[1], vals[0][1]))
        vals.append((jnp.where(first, s4[1], 0.0), jnp.where(first, s4[0], 0.0)))
        vals += [(zero, zero)] * 7
        store(fd_ref, (), (256 * k2, 256 * k2 + 128), vals)
        rho = (-rho[1], rho[0])


def _ssm_bases(g, par_ref, dt_ref, base_ref):
    rows = pl.ds(pl.multiple_of(g * G, G), G)
    a_re, a_im, b_re, b_im, c_re, c_im = (
        par_ref[i, rows, :].astype(F32) for i in range(6))
    dt = dt_ref[rows, :]
    decay, phase = dt * a_re, dt * a_im
    dts = dt * (1.0 / 512)
    w = _cmul((c_re, c_im), (dts * b_re, dts * b_im))
    z, unit = {}, (jnp.cos(phase), jnp.sin(phase))
    for e in (1, 2, 4, 8, 16, 32, 64, 128, 256, 512, 1024):
        if e in (1, 4, 8, 16, 256, 1024):
            mag = jnp.exp(decay * float(e))
            z[e] = (mag * unit[0], mag * unit[1])
        if e < 1024:
            unit = _csq(unit)
    w1024 = _cmul(w, z[1024])
    seq = [(jnp.ones_like(dt), jnp.zeros_like(dt)), z[8], z[16], z[16], z[1], z[1],
           z[256], z[256], w, _cmul(w, z[4]), _cmul(w, z[8]), w1024,
           _cmul(w1024, z[1024])]
    for h in range(2):
        for part in range(2):
            for i, v in enumerate(seq):
                base_ref[2 * g + h, part, pl.ds(8 * i, 8), :] = v[part][8 * h:8 * h + 8]


_OFFSETS = ((0, 4), (1, 5), (2, 6), (3, 7), (256, 260), (512, 516), (768, 772),
            (258, 262), (264, 1280), (520, 1536), (776, 1792), (1024, 2048))


def _ssm_values(g, base_ref, kv_ref):
    for h in range(2):
        for quad in range(2):
            def pair(i):
                return tuple(base_ref[2 * g + h, part, pl.ds(8 * i + quad, 8, stride=2), :]
                             for part in range(2))
            v, z16 = [pair(0)], pair(2)
            for _ in range(15):
                v.append(_cmul(v[-1], z16))
            z1, z256 = pair(4), pair(6)
            w = [pair(8)]
            for _ in range(3):
                w.append(_cmul(w[-1], z1))
            w.append(_cmul(w[0], z256))
            for _ in range(2):
                w.append(_cmul(w[-1], z256))
            w.append(_cmul(w[2], z256))
            w.append(_cmul(pair(10), z256))
            for _ in range(2):
                w.append(_cmul(w[-1], z256))
            w.append(pair(11))
            re, im = (lax.dot_general(
                jnp.concatenate([t[part] for t in w], axis=0).astype(BF16),
                jnp.concatenate([t[part] for t in v], axis=0).astype(BF16),
                NT, preferred_element_type=F32) for part in range(2))
            out = re - im
            for u in range(12):
                kv_ref[2 * g + h, pl.ds(16 * u + quad, 8, stride=2), :] = out[8 * u:8 * u + 8]


def _ssm_spectrum(g, kv_ref, fk_ref, fd_ref, kf_ref):
    lane = _iota((8, 128), 1)
    src = 4 * ((lane >> 1) & 31) + (_iota((8, 128), 0) & 3)
    val = {}
    for u, pair in enumerate(_OFFSETS):
        for s, e in enumerate(pair):
            x = jnp.concatenate(
                [kv_ref[2 * g + h, pl.ds(16 * u + 8 * s, 8), :] for h in range(2)], axis=0)
            val[e] = jnp.take_along_axis(_pack(x), src, axis=1, mode="promise_in_bounds")

    def even(a, b):
        return jnp.where((lane & 1) == 0, a, b)

    def low(a, b):
        return jnp.where(lane < 64, a, b)

    mid = even(val[256], val[260])
    blk0 = [low(even(val[0], val[4]), mid), low(even(val[1], val[5]), mid),
            low(even(val[2], val[6]), even(val[258], val[262])),
            low(even(val[3], val[7]), even(val[260], val[264]))]
    q0, q4, q8 = low(val[512], val[768]), low(val[516], val[772]), low(val[520], val[776])
    blk1 = [even(q0, q4), even(q0, q4), even(q0, q8), even(q4, q8)]
    blk2 = low(even(val[1024], val[1280]), val[1536])
    blk3 = low(even(val[1536], val[1792]), jnp.where(lane == 64, val[2048], 0))

    comp = [jnp.dot(_bf(jnp.concatenate([blk0[j], blk1[j]], axis=0)), _bf(fk_ref[j]),
                    preferred_element_type=F32) for j in range(4)]
    spec = [_dft4([(c[G * p:G * p + G, :128], c[G * p:G * p + G, 128:]) for c in comp], 1)
            for p in range(2)]
    far = jnp.dot(_bf(jnp.concatenate([blk2, blk3], axis=0)), _bf(fd_ref[...]),
                  preferred_element_type=F32)
    for p in range(2):
        spec.append([(far[G * p:G * p + G, 256 * k:256 * k + 128],
                      far[G * p:G * p + G, 256 * k + 128:256 * k + 256]) for k in range(4)])
    for k in range(4):
        for p in range(4):
            v = spec[p][k] if p == 0 else _csub_i(spec[p][k], spec[p - 1][k])
            for part in range(2):
                kf_ref[g, k, 2 * p + part] = v[part]


def _layernorm(x_ref, xp_ref, xn_ref):
    def permute(g, _):
        for p in range(4):
            r = [pltpu.bitcast(x_ref[pl.ds(pl.multiple_of(g * G, G), G),
                                     pl.ds(512 * p + 128 * q, 128)], I32) for q in range(4)]
            r = _skew([r[0]] + [pltpu.roll(r[q], q, 1) for q in range(1, 4)])
            for j in range(4):
                xp_ref[pl.ds(pl.multiple_of(g * 8, 8), 8), pl.ds(512 * p + 128 * j, 128)] = r[j]
        return _

    lax.fori_loop(0, NG, permute, 0, unroll=4)
    mean = jnp.dot(jnp.ones((16, D), BF16), _bf(xp_ref[...]),
                   preferred_element_type=F32) / D
    mean_bf = _round_bf16(mean)
    for p in range(4):
        cols = pl.ds(512 * p, 512)
        m = mean_bf[:, 512 * p:512 * p + 512]

        def centre(g, acc):
            rows = pl.ds(pl.multiple_of(g * 8, 8), 8)
            c = _bf(xp_ref[rows, cols]).astype(F32) - m
            xn_ref[rows, cols] = _pack(c)
            return acc + c * c

        acc = lax.fori_loop(0, NG, centre, jnp.zeros((G, 512), F32), unroll=6)
        shift = mean[:, 512 * p:512 * p + 512] - m
        var = jnp.sum(acc, axis=0, keepdims=True) / D - shift * shift
        var = _round_bf16(jnp.maximum(var, 0.0))
        eps = _round_bf16(jnp.full_like(var, EPS))
        inv = 1.0 / _round_bf16(jnp.sqrt(_round_bf16(var + eps)))

        def scale(g, _):
            rows = pl.ds(pl.multiple_of(g * 8, 8), 8)
            xn_ref[rows, cols] = _pack(_bf(xn_ref[rows, cols]).astype(F32) * inv)
            return _

        lax.fori_loop(0, NG, scale, 0, unroll=6)


def _route(wr_ref, xn_ref, hot_ref, xs_ref, gate_ref):
    w = jnp.broadcast_to(wr_ref[...].astype(F32).reshape(1, D), (16, D)).astype(BF16)
    xn = _bf(xn_ref[...])
    score = _round_bf16(jnp.dot(w, xn, preferred_element_type=F32))
    blk = _iota((16, 128), 0)
    dense = score[:, :128]
    for c in range(1, 16):
        dense = jnp.where(blk == c, score[:, 128 * c:128 * c + 128], dense)
    bits = pltpu.bitcast(jnp.where(dense == 0.0, 0.0, dense), I32) >> 16
    order = jnp.where(bits < 0, bits ^ 0x7FFF, bits) + 0x8000
    time = 512 * (blk >> 2) + _x_time(blk & 3, _iota((16, 128), 1))
    key = pltpu.bitcast((1 << 29) + (order << 11) + (L - 1 - time), F32)
    rank = jnp.full((16, 128), 16, I32)
    best_score = jnp.zeros((16, 128), F32)
    for i in range(TOPK):
        top = jnp.max(jnp.max(key, axis=0, keepdims=True), axis=1, keepdims=True)
        top = jnp.broadcast_to(top, (16, 128))
        hit = key == top
        rank = jnp.where(hit, i, rank)
        key = jnp.where(hit, 0.0, key)
        best_score = jnp.where(blk == i, top, best_score)
    order = ((pltpu.bitcast(best_score, I32) >> 11) & 0xFFFF) - 0x8000
    best_score = pltpu.bitcast(jnp.where(order < 0, order ^ 0x7FFF, order) << 16, F32)
    gate_ref[...] = _round_bf16(jax.nn.sigmoid(jnp.where(blk < TOPK, best_score, 0.0)))
    hot = jnp.concatenate(
        [jnp.where(jnp.broadcast_to(rank[c:c + 1], (16, 128)) == blk, 1.0, 0.0)
         for c in range(16)], axis=1).astype(BF16)
    hot_ref[...] = pltpu.bitcast(hot, I32)
    xs_ref[...] = lax.dot_general(hot, xn, NT, preferred_element_type=F32)


def _convolve(g, xn_ref, kf_ref, fx_ref, fxt_ref, y_ref):
    rows = pl.ds(pl.multiple_of(g * 8, 8), 8)
    comp = [jnp.dot(
        _bf(jnp.concatenate([xn_ref[rows, pl.ds(512 * p + 128 * j, 128)]
                             for p in range(4)], axis=0)),
        _bf(fx_ref[j]), preferred_element_type=F32) for j in range(4)]
    spec = [_dft4([(c[G * p:G * p + G, :128], c[G * p:G * p + G, 128:]) for c in comp], 1)
            for p in range(4)]
    prod = [[None] * 4 for _ in range(4)]
    for k in range(4):
        kf = [(kf_ref[g, k, 2 * p], kf_ref[g, k, 2 * p + 1]) for p in range(4)]
        for c in range(4):
            acc = _cmul(kf[0], spec[c][k])
            for p in range(1, c + 1):
                acc = _cadd(acc, _cmul(kf[p], spec[c - p][k]))
            prod[c][k] = acc
    back = [_dft4(prod[c], -1) for c in range(4)]
    for j in range(4):
        lhs = jnp.concatenate([jnp.concatenate(back[c][j], axis=1) for c in range(4)], axis=0)
        y = jnp.dot(lhs.astype(BF16), _bf(fxt_ref[j]), preferred_element_type=F32)
        for c in range(4):
            y_ref[pl.ds(pl.multiple_of(g * G, G), G), pl.ds(512 * c + 128 * j, 128)] = (
                y[G * c:G * c + G])


def _finish(lo, n, h, wd_ref, gate_ref, hot_ref, xp_ref, xn_ref, y_ref, ds_ref, o_ref):
    ffn = lax.dot_general(h, wd_ref[pl.ds(lo, n), :], NT, preferred_element_type=F32)
    ffn = _round_bf16(ffn) * gate_ref[:, :n]
    ffn_t = ffn.T.astype(BF16)
    for g0 in range(0, n, G):
        g = (lo + g0) // G
        upd = jnp.dot(ffn_t[g0:g0 + G], _bf(hot_ref[...]), preferred_element_type=F32)
        ds = ds_ref[pl.ds(g * G, G), :]
        for p in range(4):
            r = []
            for j in range(4):
                c0 = 512 * p + 128 * j
                xn = _bf(xn_ref[pl.ds(g * 8, 8), pl.ds(c0, 128)]).astype(F32)
                x = _bf(xp_ref[pl.ds(g * 8, 8), pl.ds(c0, 128)]).astype(F32)
                s = y_ref[pl.ds(g * G, G), pl.ds(c0, 128)] + xn * ds
                r.append(_pack(x + s * _silu(xn + upd[:, c0:c0 + 128])))
            r = _skew(r)
            for q in range(4):
                v = r[q] if q == 0 else pltpu.roll(r[q], 128 - q, 1)
                o_ref[pl.ds(g * G, G), pl.ds(512 * p + 128 * q, 128)] = _bf(v)


def _kernel(x_hbm, are_hbm, aim_hbm, bre_hbm, bim_hbm, cre_hbm, cim_hbm, ldt_hbm, dsk_hbm,
            wr_hbm, wg_hbm, wu_hbm, wd_hbm, o_hbm,
            x_ref, par_ref, ldt_ref, dsk_ref, wr_ref, wg_ref, wu_ref, wd_ref, o_ref,
            fx_ref, fxt_ref, fk_ref, fd_ref, dt_ref, ds_ref, base_ref, kv_ref, kf_ref,
            xp_ref, xn_ref, y_ref, hot_ref, xs_ref, gate_ref, h_ref, sems):
    copies = []

    def fetch(src, dst):
        cp = pltpu.make_async_copy(src, dst, sems.at[len(copies)])
        copies.append(cp)
        cp.start()
        return cp

    small = [fetch(s, d) for s, d in
             ((ldt_hbm, ldt_ref), (dsk_hbm, dsk_ref), (wr_hbm, wr_ref))]
    params = [fetch(s, par_ref.at[i]) for i, s in
              enumerate((are_hbm, aim_hbm, bre_hbm, bim_hbm, cre_hbm, cim_hbm))]
    x_copy = fetch(x_hbm, x_ref)
    fc = F // UP_CHUNKS
    ups = [[fetch(s.at[:, pl.ds(i * fc, fc)], d.at[:, pl.ds(i * fc, fc)])
            for s, d in ((wg_hbm, wg_ref), (wu_hbm, wu_ref))] for i in range(UP_CHUNKS)]
    downs = [fetch(wd_hbm.at[pl.ds(lo, n), :], wd_ref.at[pl.ds(lo, n), :])
             for lo, n in DOWN_CHUNKS]

    with jax.named_scope("setup"):
        _make_transforms(fx_ref, fxt_ref, fk_ref, fd_ref)
        for cp in small:
            cp.wait()
        _column(ldt_ref, dt_ref, lambda v: _round_bf16(jnp.exp(v)))
        _column(dsk_ref, ds_ref, lambda v: v)
        for cp in params:
            cp.wait()

    with jax.named_scope("ssm_kernel"):
        def ssm(g, _):
            _ssm_bases(g, par_ref, dt_ref, base_ref)
            _ssm_values(g, base_ref, kv_ref)
            _ssm_spectrum(g, kv_ref, fk_ref, fd_ref, kf_ref)
            return _

        lax.fori_loop(0, NG, ssm, 0)

    with jax.named_scope("layernorm"):
        x_copy.wait()
        _layernorm(x_ref, xp_ref, xn_ref)
    with jax.named_scope("route"):
        _route(wr_ref, xn_ref, hot_ref, xs_ref, gate_ref)

    with jax.named_scope("convolve"):
        def conv(g, _):
            _convolve(g, xn_ref, kf_ref, fx_ref, fxt_ref, y_ref)
            return _

        lax.fori_loop(0, NG, conv, 0)

    with jax.named_scope("ffn_up"):
        xs = xs_ref[...].astype(BF16)
        for i in range(UP_CHUNKS):
            for cp in ups[i]:
                cp.wait()
            cols = pl.ds(i * fc, fc)
            a = _round_bf16(jnp.dot(xs, wg_ref[:, cols], preferred_element_type=F32))
            b = _round_bf16(jnp.dot(xs, wu_ref[:, cols], preferred_element_type=F32))
            h_ref[:, cols] = _pack(_round_bf16(_silu(a)) * b)

    with jax.named_scope("finish"):
        outs = []
        for (lo, n), cp in zip(DOWN_CHUNKS, downs):
            cp.wait()
            _finish(lo, n, _bf(h_ref[...]), wd_ref, gate_ref, hot_ref, xp_ref, xn_ref,
                    y_ref, ds_ref, o_ref)
            outs.append(fetch(o_ref.at[pl.ds(lo, n), :], o_hbm.at[pl.ds(lo, n), :]))
        for cp in outs:
            cp.wait()


@jax.jit
def pallas_recurrent_scan__ssm_conv_s4__moe_arch_mod__prompt_kernel(
    A_u: jax.Array,
    A_A_re: jax.Array,
    A_A_im: jax.Array,
    A_B_re: jax.Array,
    A_B_im: jax.Array,
    A_C_re: jax.Array,
    A_C_im: jax.Array,
    A_log_dt: jax.Array,
    A_Dskip: jax.Array,
    B_x: jax.Array,
    B_w_r: jax.Array,
    B_w_gate: jax.Array,
    B_w_up: jax.Array,
    B_w_down: jax.Array,
):
    del B_x
    assert A_u.shape == (1, L, D) and A_A_re.shape == (D, N) and B_w_gate.shape == (D, F)
    assert A_A_re.dtype == BF16
    n_copies = 10 + 2 * UP_CHUNKS + 2 * len(DOWN_CHUNKS)
    vmem = pltpu.VMEM
    scratch = [
        vmem((D, L), BF16), vmem((6, D, N), BF16),
        vmem((D,), BF16), vmem((D,), BF16), vmem((D,), BF16),
        vmem((D, F), BF16), vmem((D, F), BF16), vmem((D, F), BF16), vmem((D, L), BF16),
        vmem((4, 64, 256), I32), vmem((4, 128, 128), I32), vmem((4, 64, 256), I32),
        vmem((64, 1024), I32), vmem((D, 128), F32), vmem((D, 128), F32),
        vmem((2 * NG, 2, 104, 128), F32), vmem((2 * NG, 192, 128), F32),
        vmem((NG, 4, 8, G, 128), F32),
        vmem((D // 2, L), I32), vmem((D // 2, L), I32), vmem((D, L), F32),
        vmem((8, L), I32), vmem((16, D), F32), vmem((16, 128), F32), vmem((8, F), I32),
        pltpu.SemaphoreType.DMA((n_copies,)),
    ]
    out = pl.pallas_call(
        _kernel,
        out_shape=jax.ShapeDtypeStruct((D, L), BF16),
        in_specs=[pl.BlockSpec(memory_space=pl.ANY)] * 13,
        out_specs=pl.BlockSpec(memory_space=pl.ANY),
        scratch_shapes=scratch,
        compiler_params=pltpu.CompilerParams(vmem_limit_bytes=100 * 1024 * 1024),
    )(A_u[0].T, A_A_re, A_A_im, A_B_re, A_B_im, A_C_re, A_C_im, A_log_dt, A_Dskip,
      B_w_r, B_w_gate, B_w_up, B_w_down.T)
    return out.T[None]
```

```python
import itertools
import math

import jax
import jax.numpy as jnp
from jax import lax
import jax.experimental.pallas as pl
import jax.experimental.pallas.tpu as pltpu

F32, BF16, I32 = jnp.float32, jnp.bfloat16, jnp.int32
L, D, N, F, TOPK = 2048, 576, 128, 4608, 8
G = 16
NG = D // G
EPS = 1e-5
NN = (((1,), (0,)), ((), ()))
NT = (((1,), (1,)), ((), ()))
CHUNKS = ((0, 128), (128, 128), (256, 128), (384, 128), (512, 64))
FLAGS = None
RA = 17
HB = 3
RB = 2
SPLIT = (6, 6, 6)
CUTS = (13, 26, 39)
ORDER_C = "eob01"


def _iota(shape, dim):
    return lax.broadcasted_iota(I32, shape, dim)


def _cmul(a, b):
    return a[0] * b[0] - a[1] * b[1], a[0] * b[1] + a[1] * b[0]


def _csq(a):
    return a[0] * a[0] - a[1] * a[1], (a[0] + a[0]) * a[1]


def _cadd(a, b):
    return a[0] + b[0], a[1] + b[1]


def _csub(a, b):
    return a[0] - b[0], a[1] - b[1]


def _cadd_i(a, b):
    return a[0] - b[1], a[1] + b[0]


def _csub_i(a, b):
    return a[0] + b[1], a[1] - b[0]


def _dft4(v, sign):
    s02, d02 = _cadd(v[0], v[2]), _csub(v[0], v[2])
    s13, d13 = _cadd(v[1], v[3]), _csub(v[1], v[3])
    a, b = _cadd_i(d02, d13), _csub_i(d02, d13)
    if sign < 0:
        a, b = b, a
    return [_cadd(s02, s13), a, _csub(s02, s13), b]


def _root(n):
    ang = (((n + 1024) & 2047) - 1024).astype(F32) * (2.0 * math.pi / 2048)
    return jnp.cos(ang), jnp.sin(ang)


def _pack(x):
    return pltpu.bitcast(x.astype(BF16), I32)


def _bf(x):
    return pltpu.bitcast(x, BF16)


def _round_bf16(x):
    return x.astype(BF16).astype(F32)


def _silu(x):
    h = 0.5 * x
    return h + h * jnp.tanh(h)


def _skew(r):
    lane = _iota(r[0].shape, 1)
    b0, b1 = (lane & 1) != 0, (lane & 2) != 0
    t = [jnp.where(b0, r[(k + 1) % 4], r[k]) for k in range(4)]
    u = [jnp.where(b1, t[(k + 2) % 4], t[k]) for k in range(4)]
    return [u[(-j) % 4] for j in range(4)]


def _x_time(j, m):
    q = (m - j) & 3
    return 128 * q + ((m - q) & 127)


def _mm(a, b, dims=NN):
    return lax.dot_general(a, b, dims, precision=lax.Precision.DEFAULT,
                           preferred_element_type=F32)


def _rows(i, n):
    return pl.ds(i * n if isinstance(i, int) else pl.multiple_of(i * n, n), n)


def _weave(main, side, rate=1.0):
    credit = 0.0
    for _ in main:
        credit += rate
        while credit >= 1.0:
            credit -= 1.0
            next(side, None)
    for _ in side:
        pass


def _column(v_ref, out_ref, fn):
    v = fn(v_ref[...].astype(F32).reshape(1, D))
    for lo in range(0, D, 128):
        n = min(128, D - lo)
        out_ref[pl.ds(lo, n), :] = jnp.broadcast_to(v[:, lo:lo + n], (128, n)).T


def _make_transforms(fx_ref, fxt_ref, fk_ref, fd_ref):
    freq = 4 * _iota((8, 128), 1) + 1
    row = _iota((8, 128), 0)
    step1 = _root(freq)
    step8 = _csq(_csq(_csq(step1)))
    step32 = _csq(_csq(step8))
    step128 = _csq(_csq(step32))

    def stack(vals, part):
        return jnp.concatenate([v[part] for v in vals], axis=0)

    def component(j, kbase):
        start = _root((_x_time(j, row + 8) - 8) * freq)
        wrapped = _cmul(start, step128)
        wraps = row < ((row - j) & 3)
        vals = [start]
        for _ in range(15):
            vals.append(_cmul(vals[-1], step8))
        vals[0] = tuple(jnp.where(wraps, a, b) for a, b in zip(wrapped, start))
        for part in range(2):
            fx_ref[j, part] = _pack(stack(vals, part))
            fxt_ref[j, pl.ds(64 * part, 64), :] = _pack(stack(vals, part).T)
        vals = [kbase]
        for _ in range(15):
            vals.append(_cmul(vals[-1], step32))
        for part in range(2):
            fk_ref[j, part] = _pack(stack(vals, part))
        return _cmul(kbase, step1)

    lax.fori_loop(0, 4, component, _root(4 * row * freq))

    rows = [_root((256 * (row & 1) + 8 * (row >> 1)) * freq)]
    for _ in range(7):
        rows.append(_cmul(rows[-1], step32))
    zero = jnp.zeros((8, 128), F32)
    rho = step1
    for k in range(4):
        p2 = _csq(rho)
        s3 = _cadd(_cadd(rho, p2), _cmul(p2, rho))
        s4 = _cadd(s3, _csq(p2))
        box = 1.0 + 2.0 * jnp.where((row & 2) == 0, s4[0], s3[0])
        vals = [(r[0] * box, r[1] * box) for r in rows]
        first = row == 0
        vals[0] = (jnp.where(first, 1.0 + s4[0], vals[0][0]),
                   jnp.where(first, s4[1], vals[0][1]))
        vals.append((jnp.where(first, s4[1], 0.0), jnp.where(first, s4[0], 0.0)))
        vals += [(zero, zero)] * 7
        for part in range(2):
            fd_ref[k, part] = _pack(stack(vals, part))
        rho = (-rho[1], rho[0])


def _ssm_bases(g, par_ref, dt_ref, base_ref):
    rows = _rows(g, G)
    a_re, a_im, b_re, b_im, c_re, c_im = (
        par_ref[k, rows, :].astype(F32) for k in range(6))
    dt = dt_ref[rows, :]
    decay, phase = dt * a_re, dt * a_im
    dts = dt * (2.0 / 512)
    w = _cmul((c_re, c_im), (dts * b_re, dts * b_im))
    z, unit = {}, (jnp.cos(phase), jnp.sin(phase))
    for e in (1, 2, 4, 8, 16, 32, 64, 128, 256, 512, 1024):
        if e in (1, 4, 8, 16, 256, 1024):
            mag = jnp.exp(decay * float(e))
            z[e] = (mag * unit[0], mag * unit[1])
        if e < 1024:
            unit = _csq(unit)
    w1024 = _cmul(w, z[1024])
    seq = [(jnp.ones_like(dt), jnp.zeros_like(dt)), z[8], z[16], z[16], z[1], z[1],
           z[256], z[256], w, _cmul(w, z[4]), _cmul(w, z[8]), w1024,
           _cmul(w1024, z[1024])]
    for k, v in enumerate(seq):
        for t in range(2):
            for part in range(2):
                base_ref[t, part, pl.ds(8 * k, 8), :] = v[part][8 * t:8 * t + 8]


_OFFSETS = ((0, 4), (1, 5), (2, 6), (3, 7), (256, 260), (512, 516), (768, 772),
            (258, 262), (264, 1280), (520, 1536), (776, 1792), (1024, 2048))


def _ssm_values(h, base_ref, kv_ref):
    for quad in range(2):
        def pair(k):
            return tuple(base_ref[h, part, pl.ds(8 * k + quad, 8, stride=2), :]
                         for part in range(2))
        v, z16 = [pair(0)], pair(2)
        for _ in range(15):
            v.append(_cmul(v[-1], z16))
        z1, z256 = pair(4), pair(6)
        w = [pair(8)]
        for _ in range(3):
            w.append(_cmul(w[-1], z1))
        w.append(_cmul(w[0], z256))
        for _ in range(2):
            w.append(_cmul(w[-1], z256))
        w.append(_cmul(w[2], z256))
        w.append(_cmul(pair(10), z256))
        for _ in range(2):
            w.append(_cmul(w[-1], z256))
        w.append(pair(11))
        re, im = (_mm(jnp.concatenate([t[part] for t in w], axis=0),
                      jnp.concatenate([t[part] for t in v[::-1]], axis=0), NT)
                  for part in range(2))
        out = re - im
        for u in range(12):
            kv_ref[h, pl.ds(16 * u + quad, 8, stride=2), :] = out[8 * u:8 * u + 8]


def _ssm_arrange(h, slot, kv_ref, kr_ref):
    lane = _iota((8, 128), 1)
    src = 4 * (((lane >> 1) & 31) ^ 30) + (_iota((8, 128), 0) >> 1)

    def even(a, b):
        return jnp.where((lane & 1) == 0, a, b)

    def low(a, b):
        return jnp.where(lane < 64, a, b)

    val = {}
    for u, pair in enumerate(_OFFSETS):
        for s, e in enumerate(pair):
            val[e] = jnp.take_along_axis(kv_ref[h, pl.ds(16 * u + 8 * s, 8), :], src,
                                         axis=1, mode="promise_in_bounds")
    mid = even(val[256], val[260])
    blk0 = [low(even(val[0], val[4]), mid), low(even(val[1], val[5]), mid),
            low(even(val[2], val[6]), even(val[258], val[262])),
            low(even(val[3], val[7]), even(val[260], val[264])),
            low(even(val[1024], val[1280]), val[1536])]
    q0, q4, q8 = low(val[512], val[768]), low(val[516], val[772]), low(val[520], val[776])
    blk1 = [even(q0, q4), even(q0, q4), even(q0, q8), even(q4, q8),
            low(even(val[1536], val[1792]), jnp.where(lane == 64, val[2048], 0.0))]
    for j in range(5):
        kr_ref[slot, j, 0] = blk0[j]
        kr_ref[slot, j, 1] = blk1[j]


def _ssm_kernel(par_ref, dt_ref, base_ref, kv_ref, kr_ref):
    def step(g, bases=True, values=True, arrange=True):
        for h in range(2):
            if arrange:
                _ssm_arrange(h, 2 * (g - 2) + h, kv_ref, kr_ref)
            if values:
                _ssm_values(h, base_ref, kv_ref)
        if bases:
            _ssm_bases(g, par_ref, dt_ref, base_ref)

    def body(n, zero):
        for r in range(RA):
            step(2 + n * RA + r)
        return jnp.minimum(zero, n)

    step(0, values=False, arrange=False)
    step(1, arrange=False)
    zero = lax.fori_loop(0, (NG - 2) // RA, body, NG)
    step(NG, bases=False)
    step(NG + 1, bases=False, values=False)
    return zero


def _ssm_spectrum(first, count, kr_ref, fk_ref, fd_ref, kf_ref):
    for h0 in range(0, count, HB):
        def lhs(j):
            return jnp.concatenate([kr_ref[first + h0 + h, j, p]
                                    for h in range(HB) for p in range(2)], axis=0)

        near, far = [], []
        for part in range(2):
            near.append([_mm(lhs(j), _bf(fk_ref[j, part])) for j in range(4)])
            yield
        for k in range(4):
            far.append([_mm(lhs(4), _bf(fd_ref[k, part])) for part in range(2)])
            if k % 2:
                yield
        for h in range(HB):
            r = [slice(8 * (2 * h + p), 8 * (2 * h + p + 1)) for p in range(2)]
            spec = [_dft4([(near[0][j][r[p]], near[1][j][r[p]]) for j in range(4)], 1)
                    for p in range(2)]
            spec += [[(far[k][0][r[p]], far[k][1][r[p]]) for k in range(4)]
                     for p in range(2)]
            for p in range(4):
                for k in range(4):
                    v = spec[p][k] if p == 0 else _csub_i(spec[p][k], spec[p - 1][k])
                    for part in range(2):
                        kf_ref[first + h0 + h, k, 2 * p + part] = v[part]


XN = 32


def _norm_mean(p, x_ref, xp_ref, stat_ref):
    acc = [None] * 4
    for g in range(NG):
        r = [pltpu.bitcast(x_ref[_rows(g, G), _rows(4 * p + q, 128)], I32) for q in range(4)]
        r = _skew([r[0]] + [pltpu.roll(r[q], q, 1) for q in range(1, 4)])
        for j in range(4):
            xp_ref[4 * p + j, _rows(g, 8), :] = r[j]
            x = _bf(r[j]).astype(F32)
            acc[j] = x[:8] + x[8:] if g == 0 else acc[j] + (x[:8] + x[8:])
        yield
    for j in range(4):
        stat_ref[0, 4 * p + j] = jnp.broadcast_to(
            jnp.sum(acc[j], axis=0, keepdims=True), (8, 128))


def _norm_centre(p, xp_ref, cen_ref, stat_ref):
    m = [_round_bf16(stat_ref[1, 4 * p + j]) for j in range(4)]
    acc = [None] * 4
    for g in range(NG):
        for j in range(4):
            x = _bf(xp_ref[4 * p + j, _rows(g, 8), :]).astype(F32)
            d = [x[:8] - m[j], x[8:] - m[j]]
            sq = d[0] * d[0] + d[1] * d[1]
            acc[j] = sq if g == 0 else acc[j] + sq
            cen_ref[4 * p + j, _rows(g, 8), :] = jnp.concatenate(d, axis=1).astype(BF16)
        yield
    for j in range(4):
        stat_ref[0, 4 * p + j] = jnp.broadcast_to(
            jnp.sum(acc[j], axis=0, keepdims=True), (8, 128))


def _norm_stats(stat_ref):
    shift = stat_ref[1] - _round_bf16(stat_ref[1])
    var = _round_bf16(jnp.maximum(stat_ref[0] / D - shift * shift, 0.0))
    eps = _round_bf16(jnp.full_like(var, EPS))
    stat_ref[1] = 0.5 / _round_bf16(jnp.sqrt(_round_bf16(var + eps)))


def _norm_scale(p, wr, cen_ref, stat_ref, work_ref):
    for c in (4 * p + j for j in range(4)):
        score = None
        for lo in range(0, NG, 8):
            vals = []
            for g in range(lo, min(lo + 8, NG)):
                d = cen_ref[c, _rows(g, 8), :].astype(F32)
                for t in range(2):
                    vals.append(d[:, 128 * t:128 * t + 128] * stat_ref[1, c])
                    work_ref[2 * g + t, XN + c] = vals[-1]
            part = _mm(wr[:, G * lo:G * lo + 8 * len(vals)], jnp.concatenate(vals, axis=0))
            score = part if lo == 0 else score + part
        stat_ref[0, c] = score
        yield


def _route(stat_ref, work_ref, hot_ref, xs_ref, gate_ref):
    row = _iota((8, 128), 0)
    halves = []
    for lo in (0, 8):
        dense = stat_ref[0, lo]
        for c in range(1, 8):
            dense = jnp.where(row == c, stat_ref[0, lo + c], dense)
        halves.append(dense)
    score = _round_bf16(jnp.concatenate(halves, axis=0))
    blk = _iota((16, 128), 0)
    bits = pltpu.bitcast(jnp.where(score == 0.0, 0.0, score), I32) >> 16
    order = jnp.where(bits < 0, bits ^ 0x7FFF, bits) + 0x8000
    time = 512 * (blk >> 2) + _x_time(blk & 3, _iota((16, 128), 1))
    key = pltpu.bitcast((1 << 29) + (order << 11) + (L - 1 - time), F32)
    rank = jnp.full((16, 128), TOPK, I32)
    best = jnp.zeros((8, 128), F32)
    for i in range(TOPK):
        top = jnp.max(jnp.max(key, axis=0, keepdims=True), axis=1, keepdims=True)
        hit = key == top
        rank = jnp.where(hit, i, rank)
        key = jnp.where(hit, 0.0, key)
        best = jnp.where(row == i, top, best)
        yield
        yield
    order = ((pltpu.bitcast(best, I32) >> 11) & 0xFFFF) - 0x8000
    best = pltpu.bitcast(jnp.where(order < 0, order ^ 0x7FFF, order) << 16, F32)
    gate_ref[...] = 0.5 * _round_bf16(jax.nn.sigmoid(best))
    for c in range(16):
        hot_ref[c] = jnp.where(jnp.broadcast_to(rank[c:c + 1], (8, 128)) == row, 1.0, 0.0)
    for lo in range(0, D, 128):
        n, picked = min(128, D - lo), None
        for c in range(16):
            tokens = work_ref[pl.ds(lo // 8, n // 8), XN + c].reshape(n, 128)
            part = _mm(hot_ref[c], tokens, NT)
            picked = part if c == 0 else picked + part
            if c % 4 == 3:
                yield
        xs_ref[:, pl.ds(lo, n)] = 2.0 * picked


def _ffn_up(first, count, xs_ref, wg_ref, wu_ref, h_ref):
    for col in range(first, first + count, 256):
        acc = [None, None]
        for lo in range(0, D, 128):
            rows = pl.ds(lo, min(128, D - lo))
            for n, w_ref in enumerate((wg_ref, wu_ref)):
                part = _mm(xs_ref[:, rows], w_ref[rows, pl.ds(col, 256)])
                acc[n] = part if lo == 0 else acc[n] + part
            yield
        h_ref[:, pl.ds(col, 256)] = (
            _round_bf16(_silu(_round_bf16(acc[0]))) * _round_bf16(acc[1]))


def _conv_step(i, same, live, later, kf_ref, fx_ref, fxt_ref, xf_ref, work_ref, s_ref):
    def products():
        for t in range(2):
            h = 2 * (i - 2) + t
            for k in range(4):
                kf = [(kf_ref[h, k, 2 * p], kf_ref[h, k, 2 * p + 1]) for p in range(4)]
                x = [(xf_ref[h, k, 2 * p], xf_ref[h, k, 2 * p + 1]) for p in range(4)]
                for c in (3, 0, 2, 1):
                    acc = _cmul(kf[0], x[c])
                    for p in range(1, c + 1):
                        acc = _cadd(acc, _cmul(kf[p], x[c - p]))
                    for part in range(2):
                        work_ref[2 * (same - 2) + t, 8 * c + 2 * k + part] = acc[part]
                    if c < 2:
                        yield

    fill = products() if live[2] else iter(())
    comp = [None] * 2

    def forward(part):
        lhs = [[] for _ in range(4)]
        for t in range(2):
            for p in range(4):
                for j in range(4):
                    lhs[j].append(work_ref[2 * i + t, XN + 4 * p + j])
                if p % 2:
                    next(fill, None)
        comp[part] = [_mm(jnp.concatenate(lhs[j], axis=0), _bf(fx_ref[j, part]))
                      for j in range(4)]

    def butterflies():
        for t in range(2):
            for p in range(4):
                r = slice(8 * (4 * t + p), 8 * (4 * t + p + 1))
                spec = _dft4([(comp[0][j][r], comp[1][j][r]) for j in range(4)], 1)
                for k in range(4):
                    for part in range(2):
                        xf_ref[2 * same + t, k, 2 * p + part] = spec[k][part]

    def inverse(odd):
        lhs = [[], []]
        for t in range(2):
            h = 2 * (i - 3) + t
            for c in range(4):
                v = [(work_ref[h, 8 * c + 2 * k], work_ref[h, 8 * c + 2 * k + 1])
                     for k in range(4)]
                if odd:
                    a, b = _csub(v[0], v[2]), _csub(v[1], v[3])
                    back = _csub_i(a, b), _cadd_i(a, b)
                else:
                    a, b = _cadd(v[0], v[2]), _cadd(v[1], v[3])
                    back = _cadd(a, b), _csub(a, b)
                for n in range(2):
                    lhs[n].append(jnp.concatenate(back[n], axis=1))
                if c % 2:
                    next(fill, None)
        y = [_mm(jnp.concatenate(lhs[n], axis=0), _bf(fxt_ref[odd + 2 * n]))
             for n in range(2)]
        for t in range(2):
            for c in range(4):
                for n in range(2):
                    s_ref[2 * (i - 3) + t, 4 * c + odd + 2 * n] = (
                        y[n][32 * t + 8 * c:32 * t + 8 * c + 8])

    for op in ORDER_C:
        if op in "01" and live[0]:
            forward(int(op))
        if op in "eo" and live[3]:
            inverse(int(op == "o"))
        while op == "b" and later:
            later.pop()()
        if op != "b":
            yield
    for _ in fill:
        pass
    if live[0]:
        later.append(butterflies)


def _ffn_down(lo, n, h_ref, wd_ref, gate_ref, upd_ref):
    ffn = None
    for k in range(0, F, 512):
        part = _mm(h_ref[:, pl.ds(k, 512)], wd_ref[pl.ds(lo, n), pl.ds(k, 512)], NT)
        ffn = part if ffn is None else ffn + part
        if k + 512 < F:
            yield
    upd_ref[pl.ds(lo, n), :] = (_round_bf16(ffn) * gate_ref[:, :n]).T


def _gate(lo, n, upd_ref, hot_ref, xp_ref, work_ref, s_ref, ds_ref, o_ref):
    for h0 in range(lo // 8, (lo + n) // 8, 8):
        nh = min(8, (lo + n) // 8 - h0)
        for p in range(4):
            scattered = [_mm(upd_ref[pl.ds(8 * h0, 8 * nh), :], hot_ref[4 * p + j])
                         for j in range(4)]
            for h in range(h0, h0 + nh):
                r = []
                for j in range(4):
                    x = _bf(xp_ref[4 * p + j, _rows(h // 2, 8), :]).astype(F32)
                    half = work_ref[h, XN + 4 * p + j]
                    s = s_ref[h, 4 * p + j] + half * ds_ref[_rows(h, 8), :]
                    half = half + scattered[j][8 * (h - h0):8 * (h - h0) + 8]
                    r.append(x[8 * (h % 2):8 * (h % 2) + 8]
                             + s * (half + half * jnp.tanh(half)))
                r = _skew(r)
                r = [r[0]] + [pltpu.roll(r[q], 128 - q, 1) for q in range(1, 4)]
                o_ref[_rows(h, 8), pl.ds(512 * p, 512)] = (
                    jnp.concatenate(r, axis=1).astype(BF16))
            yield


def _kernel(x_hbm, are_hbm, aim_hbm, bre_hbm, bim_hbm, cre_hbm, cim_hbm, ldt_hbm, dsk_hbm,
            wr_hbm, wg_hbm, wu_hbm, wd_hbm, o_hbm,
            x_ref, par_ref, ldt_ref, dsk_ref, wr_ref, wg_ref, wu_ref, wd_ref, o_ref,
            fx_ref, fxt_ref, fk_ref, fd_ref, dt_ref, ds_ref, base_ref, kv_ref, kr_ref, kf_ref,
            xp_ref, stat_ref, cen_ref, work_ref, xf_ref, s_ref,
            hot_ref, xs_ref, gate_ref, h_ref, upd_ref, sems):
    copies = []

    def fetch(src, dst):
        cp = pltpu.make_async_copy(src, dst, sems.at[len(copies)])
        copies.append(cp)
        cp.start()
        return cp

    small = [fetch(s, d) for s, d in
             ((ldt_hbm, ldt_ref), (dsk_hbm, dsk_ref), (wr_hbm, wr_ref))]
    params = [fetch(s, par_ref.at[i]) for i, s in
              enumerate((are_hbm, aim_hbm, bre_hbm, bim_hbm, cre_hbm, cim_hbm))]
    x_copy = fetch(x_hbm, x_ref)
    ups = [[fetch(src.at[:, _rows(i, F // 2)], dst.at[:, _rows(i, F // 2)])
            for src, dst in ((wg_hbm, wg_ref), (wu_hbm, wu_ref))] for i in range(2)]

    with jax.named_scope("setup"):
        _make_transforms(fx_ref, fxt_ref, fk_ref, fd_ref)
        for cp in small:
            cp.wait()
        _column(ldt_ref, dt_ref, lambda v: _round_bf16(jnp.exp(v)))
        _column(dsk_ref, ds_ref, lambda v: 2.0 * v)
        for cp in params:
            cp.wait()

    with jax.named_scope("ssm_kernel"):
        zero = _ssm_kernel(par_ref, dt_ref, base_ref, kv_ref, kr_ref)

    with jax.named_scope("layernorm"):
        x_copy.wait()
        downs = [fetch(wd_hbm.at[pl.ds(*c)], wd_ref.at[pl.ds(*c)]) for c in CHUNKS]

        def norm_pass(n, job, pieces):
            first, count = sum(SPLIT[:n]) * 4, SPLIT[n] * RB

            def body(i, carry):
                jobs = itertools.chain(*[job(i * RB + r) for r in range(RB)])
                _weave(_ssm_spectrum(first + i * count, count, kr_ref, fk_ref, fd_ref, kf_ref),
                       jobs, pieces * RB * HB / (4 * count - HB))
                return carry

            lax.fori_loop(0, 4 // RB, body, 0)

        norm_pass(0, lambda p: _norm_mean(p, x_ref, xp_ref, stat_ref), NG)
        stat_ref[1] = stat_ref[0] / D
        norm_pass(1, lambda p: _norm_centre(p, xp_ref, cen_ref, stat_ref), NG)
        _norm_stats(stat_ref)
        wr = jnp.broadcast_to(2.0 * wr_ref[...].astype(F32).reshape(1, D), (8, D))
        norm_pass(2, lambda p: _norm_scale(p, wr, cen_ref, stat_ref, work_ref), 4)

    with jax.named_scope("convolve"):
        def convolve(lo, hi):
            later = []
            for i in range(lo, hi):
                yield from _conv_step(i, i + zero, [0 <= i - k < NG for k in range(4)], later,
                                      kf_ref, fx_ref, fxt_ref, xf_ref, work_ref, s_ref)
            while later:
                later.pop()()

        _weave(convolve(0, CUTS[0]), _route(stat_ref, work_ref, hot_ref, xs_ref, gate_ref))
        for i in range(2):
            for cp in ups[i]:
                cp.wait()
            _weave(convolve(CUTS[i], CUTS[i + 1]),
                   _ffn_up(i * F // 2, F // 2, xs_ref, wg_ref, wu_ref, h_ref))

    with jax.named_scope("finish"):
        outs = []
        for i in range(len(CHUNKS) + 1):
            jobs = []
            if i < len(CHUNKS):
                downs[i].wait()
                jobs.append(_ffn_down(*CHUNKS[i], h_ref, wd_ref, gate_ref, upd_ref))
            if i > 0:
                jobs.append(_gate(*CHUNKS[i - 1], upd_ref, hot_ref, xp_ref, work_ref, s_ref,
                                  ds_ref, o_ref))
            for _ in itertools.zip_longest(*jobs):
                pass
            if i > 0:
                rows = pl.ds(*CHUNKS[i - 1])
                outs.append(fetch(o_ref.at[rows], o_hbm.at[rows]))
        for cp in outs:
            cp.wait()


@jax.jit
def pallas_recurrent_scan__ssm_conv_s4__moe_arch_mod__prompt_kernel(
    A_u: jax.Array,
    A_A_re: jax.Array,
    A_A_im: jax.Array,
    A_B_re: jax.Array,
    A_B_im: jax.Array,
    A_C_re: jax.Array,
    A_C_im: jax.Array,
    A_log_dt: jax.Array,
    A_Dskip: jax.Array,
    B_x: jax.Array,
    B_w_r: jax.Array,
    B_w_gate: jax.Array,
    B_w_up: jax.Array,
    B_w_down: jax.Array,
):
    del B_x
    assert A_u.shape == (1, L, D) and A_A_re.shape == (D, N) and B_w_gate.shape == (D, F)
    assert A_A_re.dtype == BF16
    vmem = pltpu.VMEM
    nh = 2 * NG
    scratch = [
        vmem((D, L), BF16), vmem((6, D, N), BF16),
        vmem((D,), BF16), vmem((D,), BF16), vmem((D,), BF16),
        vmem((D, F), BF16), vmem((D, F), BF16), vmem((D, F), BF16), vmem((D, L), BF16),
        vmem((4, 2, 64, 128), I32), vmem((4, 128, 128), I32),
        vmem((4, 2, 64, 128), I32), vmem((4, 2, 64, 128), I32),
        vmem((D, 128), F32), vmem((D, 128), F32),
        vmem((2, 2, 104, 128), F32), vmem((2, 192, 128), F32),
        vmem((nh, 5, 2, 8, 128), F32), vmem((nh, 4, 8, 8, 128), F32),
        vmem((16, D // 2, 128), I32), vmem((2, 16, 8, 128), F32),
        vmem((16, D // 2, 256), BF16),
        vmem((nh, XN + 16, 8, 128), F32), vmem((nh, 4, 8, 8, 128), F32),
        vmem((nh, 16, 8, 128), F32),
        vmem((16, 8, 128), F32), vmem((8, D), F32), vmem((8, 128), F32), vmem((8, F), F32),
        vmem((D, TOPK), F32),
        pltpu.SemaphoreType.DMA((14 + 2 * len(CHUNKS),)),
    ]
    out = pl.pallas_call(
        _kernel,
        out_shape=jax.ShapeDtypeStruct((D, L), BF16),
        in_specs=[pl.BlockSpec(memory_space=pl.ANY)] * 13,
        out_specs=pl.BlockSpec(memory_space=pl.ANY),
        scratch_shapes=scratch,
        compiler_params=pltpu.CompilerParams(vmem_limit_bytes=100 * 1024 * 1024, flags=FLAGS),
    )(A_u[0].T, A_A_re, A_A_im, A_B_re, A_B_im, A_C_re, A_C_im, A_log_dt, A_Dskip,
      B_w_r, B_w_gate, B_w_up, B_w_down.T)
    return out.T[None]
```

```python
import itertools
import math

import jax
import jax.numpy as jnp
from jax import lax
import jax.experimental.pallas as pl
import jax.experimental.pallas.tpu as pltpu

F32, BF16, I32 = jnp.float32, jnp.bfloat16, jnp.int32
L, D, N, F, TOPK = 2048, 576, 128, 4608, 8
G = 16
NG = D // G
EPS = 1e-5
NN = (((1,), (0,)), ((), ()))
NT = (((1,), (1,)), ((), ()))
CHUNKS = ((0, 128), (128, 128), (256, 128), (384, 128), (512, 64))
FLAGS = None
STOP = 0
RA = 4
PIECE = 3
PIECE2 = 6
BATCH = (2, 3, 3)
SPLIT = (24, 30, 18)
CUTS = (10, 22, 34)
SEND = ((), (), (0, 1), (2,), (3,))
DOWN_RATE = 1.8
ORDER_C = "eob01"


def _iota(shape, dim):
    return lax.broadcasted_iota(I32, shape, dim)


def _cmul(a, b):
    return a[0] * b[0] - a[1] * b[1], a[0] * b[1] + a[1] * b[0]


def _csq(a):
    return a[0] * a[0] - a[1] * a[1], (a[0] + a[0]) * a[1]


def _cadd(a, b):
    return a[0] + b[0], a[1] + b[1]


def _csub(a, b):
    return a[0] - b[0], a[1] - b[1]


def _cadd_i(a, b):
    return a[0] - b[1], a[1] + b[0]


def _csub_i(a, b):
    return a[0] + b[1], a[1] - b[0]


def _dft4(v, sign):
    s02, d02 = _cadd(v[0], v[2]), _csub(v[0], v[2])
    s13, d13 = _cadd(v[1], v[3]), _csub(v[1], v[3])
    a, b = _cadd_i(d02, d13), _csub_i(d02, d13)
    if sign < 0:
        a, b = b, a
    return [_cadd(s02, s13), a, _csub(s02, s13), b]


def _root(n):
    ang = (((n + 1024) & 2047) - 1024).astype(F32) * (2.0 * math.pi / 2048)
    return jnp.cos(ang), jnp.sin(ang)


def _pack(x):
    return pltpu.bitcast(x.astype(BF16), I32)


def _bf(x):
    return pltpu.bitcast(x, BF16)


def _round_bf16(x):
    return x.astype(BF16).astype(F32)


def _silu(x):
    h = 0.5 * x
    return h + h * jnp.tanh(h)


def _skew(r):
    lane = _iota(r[0].shape, 1)
    b0, b1 = (lane & 1) != 0, (lane & 2) != 0
    t = [jnp.where(b0, r[(k + 1) % 4], r[k]) for k in range(4)]
    u = [jnp.where(b1, t[(k + 2) % 4], t[k]) for k in range(4)]
    return [u[(-j) % 4] for j in range(4)]


def _x_time(j, m):
    q = (m - j) & 3
    return 128 * q + ((m - q) & 127)


def _mm(a, b, dims=NN):
    return lax.dot_general(a, b, dims, precision=lax.Precision.DEFAULT,
                           preferred_element_type=F32)


def _rows(i, n):
    return pl.ds(i * n if isinstance(i, int) else pl.multiple_of(i * n, n), n)


def _weave(main, side, rate=1.0):
    credit = 0.0
    for _ in main:
        credit += rate
        while credit >= 1.0:
            credit -= 1.0
            next(side, None)
    for _ in side:
        pass


def _column(v_ref, out_ref, fn):
    v = fn(v_ref[...].astype(F32).reshape(1, D))
    for lo in range(0, D, 128):
        n = min(128, D - lo)
        out_ref[pl.ds(lo, n), :] = jnp.broadcast_to(v[:, lo:lo + n], (128, n)).T


def _make_transforms(fx_ref, fxt_ref, fk_ref, fd_ref):
    freq = 4 * _iota((8, 128), 1) + 1
    row = _iota((8, 128), 0)
    step1 = _root(freq)
    step8 = _csq(_csq(_csq(step1)))
    step32 = _csq(_csq(step8))
    step128 = _csq(_csq(step32))

    def stack(vals, part):
        return jnp.concatenate([v[part] for v in vals], axis=0)

    def component(j, kbase):
        start = _root((_x_time(j, row + 8) - 8) * freq)
        wrapped = _cmul(start, step128)
        wraps = row < ((row - j) & 3)
        vals = [start]
        for _ in range(15):
            vals.append(_cmul(vals[-1], step8))
        vals[0] = tuple(jnp.where(wraps, a, b) for a, b in zip(wrapped, start))
        for part in range(2):
            fx_ref[j, part] = _pack(stack(vals, part))
            fxt_ref[j, pl.ds(64 * part, 64), :] = _pack(stack(vals, part).T)
        vals = [kbase]
        for _ in range(15):
            vals.append(_cmul(vals[-1], step32))
        for part in range(2):
            fk_ref[j, part] = _pack(stack(vals, part))
        return _cmul(kbase, step1)

    lax.fori_loop(0, 4, component, _root(4 * row * freq), unroll=True)

    rows = [_root((256 * (row & 1) + 8 * (row >> 1)) * freq)]
    for _ in range(7):
        rows.append(_cmul(rows[-1], step32))
    zero = jnp.zeros((8, 128), F32)
    rho = step1
    for k in range(4):
        p2 = _csq(rho)
        s3 = _cadd(_cadd(rho, p2), _cmul(p2, rho))
        s4 = _cadd(s3, _csq(p2))
        box = 1.0 + 2.0 * jnp.where((row & 2) == 0, s4[0], s3[0])
        vals = [(r[0] * box, r[1] * box) for r in rows]
        first = row == 0
        vals[0] = (jnp.where(first, 1.0 + s4[0], vals[0][0]),
                   jnp.where(first, s4[1], vals[0][1]))
        vals.append((jnp.where(first, s4[1], 0.0), jnp.where(first, s4[0], 0.0)))
        vals += [(zero, zero)] * 7
        for part in range(2):
            fd_ref[k, part] = _pack(stack(vals, part))
        rho = (-rho[1], rho[0])


def _ssm_bases(g, h, par_ref, dt_ref, base_ref):
    rows = _rows(g, G)
    a_re, a_im, b_re, b_im, c_re, c_im = (
        par_ref[k, rows, :].astype(F32) for k in range(6))
    dt = dt_ref[rows, :]
    decay, phase = dt * a_re, dt * a_im
    dts = dt * (2.0 / 512)
    w = _cmul((c_re, c_im), (dts * b_re, dts * b_im))
    z, unit = {}, (jnp.cos(phase), jnp.sin(phase))
    for e in (1, 2, 4, 8, 16, 32, 64, 128, 256, 512, 1024):
        if e in (1, 4, 8, 16, 256, 1024):
            mag = jnp.exp(decay * float(e))
            z[e] = (mag * unit[0], mag * unit[1])
        if e < 1024:
            unit = _csq(unit)
    w1024 = _cmul(w, z[1024])
    seq = [(jnp.ones_like(dt), jnp.zeros_like(dt)), z[8], z[16], z[16], z[1], z[1],
           z[256], z[256], w, _cmul(w, z[4]), _cmul(w, z[8]), w1024,
           _cmul(w1024, z[1024])]
    for k, v in enumerate(seq):
        for t in range(2):
            for part in range(2):
                base_ref[h + t, part, pl.ds(8 * k, 8), :] = v[part][8 * t:8 * t + 8]


_OFFSETS = ((0, 4), (1, 5), (2, 6), (3, 7), (256, 260), (512, 516), (768, 772),
            (258, 262), (264, 1280), (520, 1536), (776, 1792), (1024, 2048))


def _ssm_values(h, base_ref, kv_ref):
    for quad in range(2):
        def pair(k):
            return tuple(base_ref[h, part, pl.ds(8 * k + quad, 8, stride=2), :]
                         for part in range(2))
        v, z16 = [pair(0)], pair(2)
        for _ in range(15):
            v.append(_cmul(v[-1], z16))
        z1, z256 = pair(4), pair(6)
        w = [pair(8)]
        for _ in range(3):
            w.append(_cmul(w[-1], z1))
        w.append(_cmul(w[0], z256))
        for _ in range(2):
            w.append(_cmul(w[-1], z256))
        w.append(_cmul(w[2], z256))
        w.append(_cmul(pair(10), z256))
        for _ in range(2):
            w.append(_cmul(w[-1], z256))
        w.append(pair(11))
        re, im = (_mm(jnp.concatenate([t[part] for t in w], axis=0),
                      jnp.concatenate([t[part] for t in v[::-1]], axis=0), NT)
                  for part in range(2))
        out = re - im
        for u in range(12):
            kv_ref[h, pl.ds(16 * u + quad, 8, stride=2), :] = out[8 * u:8 * u + 8]


def _ssm_arrange(h, slot, kv_ref, kr_ref):
    lane = _iota((8, 128), 1)
    src = 4 * (((lane >> 1) & 31) ^ 30) + (_iota((8, 128), 0) >> 1)

    def even(a, b):
        return jnp.where((lane & 1) == 0, a, b)

    def low(a, b):
        return jnp.where(lane < 64, a, b)

    val = {}
    for u, pair in enumerate(_OFFSETS):
        for s, e in enumerate(pair):
            val[e] = jnp.take_along_axis(kv_ref[h, pl.ds(16 * u + 8 * s, 8), :], src,
                                         axis=1, mode="promise_in_bounds")
    mid = even(val[256], val[260])
    blk0 = [low(even(val[0], val[4]), mid), low(even(val[1], val[5]), mid),
            low(even(val[2], val[6]), even(val[258], val[262])),
            low(even(val[3], val[7]), even(val[260], val[264])),
            low(even(val[1024], val[1280]), val[1536])]
    q0, q4, q8 = low(val[512], val[768]), low(val[516], val[772]), low(val[520], val[776])
    blk1 = [even(q0, q4), even(q0, q4), even(q0, q8), even(q4, q8),
            low(even(val[1536], val[1792]), jnp.where(lane == 64, val[2048], 0.0))]
    for j in range(5):
        kr_ref[slot, j, 0] = blk0[j]
        kr_ref[slot, j, 1] = blk1[j]


def _ssm_kernel(par_ref, dt_ref, base_ref, kv_ref, kr_ref):
    def step(g, slot, bases=True, values=True, arrange=True):
        for t in range(2):
            if arrange:
                _ssm_arrange(2 * slot + t, 4 + 2 * (g - 4) + t, kv_ref, kr_ref)
            if values:
                _ssm_values(2 * slot + t, base_ref, kv_ref)
        if bases:
            _ssm_bases(g, 2 * slot, par_ref, dt_ref, base_ref)

    def body(n, zero):
        for r in range(RA):
            step(4 + n * RA + r, r % 2)
        return jnp.minimum(zero, n * L)

    for g in range(4):
        step(g, g % 2, values=g >= 2, arrange=False)
    zero = lax.fori_loop(0, (NG - 4) // RA, body, L)
    for g in range(NG, NG + 4):
        step(g, g % 2, bases=False, values=g < NG + 2)
    return zero


def _ssm_spectrum(first, count, HB, fine, kr_ref, fk_ref, fd_ref, kf_ref):
    for h0 in range(0, count, HB):
        near, far = [], []
        for n in range(4):
            lhs = {j: [] for j in ((0, 1, 2, 3) if n < 2 else (4,))}
            for h in range(HB):
                for p in range(2):
                    for j, rows in lhs.items():
                        rows.append(kr_ref[4 + first + h0 + h, j, p])
                if fine:
                    yield
            lhs = {j: jnp.concatenate(rows, axis=0) for j, rows in lhs.items()}
            if n < 2:
                near.append([_mm(lhs[j], _bf(fk_ref[j, n])) for j in range(4)])
            else:
                far += [[_mm(lhs[4], _bf(fd_ref[k, part])) for part in range(2)]
                        for k in (2 * n - 4, 2 * n - 3)]
            if not fine:
                yield
        for h in range(HB):
            r = [slice(8 * (2 * h + p), 8 * (2 * h + p + 1)) for p in range(2)]
            spec = [_dft4([(near[0][j][r[p]], near[1][j][r[p]]) for j in range(4)], 1)
                    for p in range(2)]
            spec += [[(far[k][0][r[p]], far[k][1][r[p]]) for k in range(4)]
                     for p in range(2)]
            for p in range(4):
                for k in range(4):
                    v = spec[p][k] if p == 0 else _csub_i(spec[p][k], spec[p - 1][k])
                    for part in range(2):
                        kf_ref[first + h0 + h, k, 2 * p + part] = v[part]


XN = 32


def _norm_mean(x_ref, xp_ref, tally):
    for p in range(4):
        acc = [None] * 4
        for g in range(NG):
            r = [pltpu.bitcast(x_ref[_rows(g, G), _rows(4 * p + q, 128)], I32)
                 for q in range(4)]
            r = _skew([r[0]] + [pltpu.roll(r[q], q, 1) for q in range(1, 4)])
            for j in range(4):
                xp_ref[4 * p + j, _rows(g, 8), :] = r[j]
                x = _bf(r[j]).astype(F32)
                acc[j] = x[:8] + x[8:] if g % PIECE == 0 else acc[j] + (x[:8] + x[8:])
                if g % PIECE == PIECE - 1:
                    tally(p, j, 0, acc[j], g < PIECE)
            yield


def _norm_centre(xp_ref, cen_ref, stat_ref, tally):
    for lo in range(0, NG, PIECE2):
        for c in range(16):
            m, acc = stat_ref[16 + c], None
            for g in range(lo, lo + PIECE2):
                x = _bf(xp_ref[c, _rows(g, 8), :]).astype(F32)
                d = [x[:8] - m, x[8:] - m]
                sq = d[0] * d[0] + d[1] * d[1]
                acc = sq if g == lo else acc + sq
                cen_ref[c, _rows(g, 8), :] = jnp.concatenate(d, axis=1).astype(BF16)
            tally(c // 4, c % 4, 1, acc, lo == 0)
            yield


def _average(v):
    return jnp.broadcast_to(jnp.sum(v, axis=0, keepdims=True), v.shape) / D


def _norm_factor(squares, mean):
    shift = mean - _round_bf16(mean)
    var = _round_bf16(jnp.maximum(_average(squares) - shift * shift, 0.0))
    eps = _round_bf16(jnp.full_like(var, EPS))
    return 0.5 / _round_bf16(jnp.sqrt(_round_bf16(var + eps)))


def _norm_scale(wr_ref, cen_ref, stat_ref, work_ref):
    wr = jnp.broadcast_to(2.0 * wr_ref[...].astype(F32).reshape(1, D), (8, D))
    for p in range(4):
        cols = range(4 * p, 4 * p + 4)
        inv, score = {c: stat_ref[c] for c in cols}, {}
        for lo in range(0, NG, 8):
            for c in cols:
                vals = []
                for g in reversed(range(lo, min(lo + 8, NG))):
                    d = cen_ref[c, _rows(g, 8), :].astype(F32)
                    for t in (1, 0):
                        vals.insert(0, d[:, 128 * t:128 * t + 128] * inv[c])
                        work_ref[2 * g + t, XN + c] = vals[0]
                part = _mm(wr[:, G * lo:G * lo + 8 * len(vals)],
                           jnp.concatenate(vals, axis=0))
                score[c] = part if lo == 0 else score[c] + part
            yield
        for c in cols:
            stat_ref[c] = score[c]


def _route(stat_ref, work_ref, hot_ref, xs_ref, gate_ref):
    row = _iota((8, 128), 0)
    halves = []
    for lo in (0, 8):
        dense = stat_ref[lo]
        for c in range(1, 8):
            dense = jnp.where(row == c, stat_ref[lo + c], dense)
        halves.append(dense)
    score = _round_bf16(jnp.concatenate(halves, axis=0))
    blk = _iota((16, 128), 0)
    bits = pltpu.bitcast(jnp.where(score == 0.0, 0.0, score), I32) >> 16
    order = jnp.where(bits < 0, bits ^ 0x7FFF, bits) + 0x8000
    time = 512 * (blk >> 2) + _x_time(blk & 3, _iota((16, 128), 1))
    key = pltpu.bitcast((1 << 29) + (order << 11) + (L - 1 - time), F32)
    rank = jnp.full((16, 128), TOPK, I32)
    best = jnp.zeros((8, 128), F32)
    for i in range(TOPK):
        top = jnp.max(jnp.max(key, axis=0, keepdims=True), axis=1, keepdims=True)
        hit = key == top
        rank = jnp.where(hit, i, rank)
        key = jnp.where(hit, 0.0, key)
        best = jnp.where(row == i, top, best)
        yield
        yield
    order = ((pltpu.bitcast(best, I32) >> 11) & 0xFFFF) - 0x8000
    best = pltpu.bitcast(jnp.where(order < 0, order ^ 0x7FFF, order) << 16, F32)
    gate_ref[...] = 0.5 * _round_bf16(jax.nn.sigmoid(best))
    for c in range(16):
        hot_ref[c] = jnp.where(jnp.broadcast_to(rank[c:c + 1], (8, 128)) == row, 1.0, 0.0)
    for lo in range(0, D, 128):
        n, picked = min(128, D - lo), None
        for c in range(16):
            tokens = work_ref[pl.ds(lo // 8, n // 8), XN + c].reshape(n, 128)
            part = _mm(hot_ref[c], tokens, NT)
            picked = part if c == 0 else picked + part
            if c % 4 == 3:
                yield
        xs_ref[:, pl.ds(lo, n)] = 2.0 * picked


def _ffn_up(first, count, xs_ref, wg_ref, wu_ref, h_ref):
    for col in range(first, first + count, 256):
        acc = [None, None]
        for lo in range(0, D, 128):
            rows = pl.ds(lo, min(128, D - lo))
            for n, w_ref in enumerate((wg_ref, wu_ref)):
                part = _mm(xs_ref[:, rows], w_ref[rows, pl.ds(col, 256)])
                acc[n] = part if lo == 0 else acc[n] + part
            yield
        h_ref[:, pl.ds(col, 256)] = (
            _round_bf16(_silu(_round_bf16(acc[0]))) * _round_bf16(acc[1]))


def _conv_step(i, same, live, later, kf_ref, fx_ref, fxt_ref, xf_ref, work_ref, s_ref):
    def products():
        for t in range(2):
            h = 2 * (i - 2) + t
            for k in range(4):
                kf = [(kf_ref[h, k, 2 * p], kf_ref[h, k, 2 * p + 1]) for p in range(4)]
                x = [(xf_ref[h, k, 2 * p], xf_ref[h, k, 2 * p + 1]) for p in range(4)]
                for c in (3, 0, 2, 1):
                    acc = _cmul(kf[0], x[c])
                    for p in range(1, c + 1):
                        acc = _cadd(acc, _cmul(kf[p], x[c - p]))
                    for part in range(2):
                        work_ref[2 * (same - 2) + t, 8 * c + 2 * k + part] = acc[part]
                    if c < 2:
                        yield

    fill = products() if live[2] else iter(())
    comp = [None] * 2

    def forward(part):
        lhs = [[] for _ in range(4)]
        for t in range(2):
            for p in range(4):
                for j in range(4):
                    lhs[j].append(work_ref[2 * i + t, XN + 4 * p + j])
                if p % 2:
                    next(fill, None)
        comp[part] = [_mm(jnp.concatenate(lhs[j], axis=0), _bf(fx_ref[j, part]))
                      for j in range(4)]

    def butterflies():
        for t in range(2):
            for p in range(4):
                r = slice(8 * (4 * t + p), 8 * (4 * t + p + 1))
                spec = _dft4([(comp[0][j][r], comp[1][j][r]) for j in range(4)], 1)
                for k in range(4):
                    for part in range(2):
                        xf_ref[2 * same + t, k, 2 * p + part] = spec[k][part]

    def inverse(odd):
        lhs = [[], []]
        for t in range(2):
            h = 2 * (i - 3) + t
            for c in range(4):
                v = [(work_ref[h, 8 * c + 2 * k], work_ref[h, 8 * c + 2 * k + 1])
                     for k in range(4)]
                if odd:
                    a, b = _csub(v[0], v[2]), _csub(v[1], v[3])
                    back = _csub_i(a, b), _cadd_i(a, b)
                else:
                    a, b = _cadd(v[0], v[2]), _cadd(v[1], v[3])
                    back = _cadd(a, b), _csub(a, b)
                for n in range(2):
                    lhs[n].append(jnp.concatenate(back[n], axis=1))
                if c % 2:
                    next(fill, None)
        y = [_mm(jnp.concatenate(lhs[n], axis=0), _bf(fxt_ref[odd + 2 * n]))
             for n in range(2)]
        for t in range(2):
            for c in range(4):
                for n in range(2):
                    s_ref[2 * (i - 3) + t, 4 * c + odd + 2 * n] = (
                        y[n][32 * t + 8 * c:32 * t + 8 * c + 8])

    for op in ORDER_C:
        if op in "01" and live[0]:
            forward(int(op))
        if op in "eo" and live[3]:
            inverse(int(op == "o"))
        while op == "b" and later:
            later.pop()()
        if op != "b":
            yield
    for _ in fill:
        pass
    if live[0]:
        later.append(butterflies)


def _ffn_down(lo, n, h_ref, wd_ref, gate_ref, upd_ref):
    ffn = None
    for k in range(0, F, 512):
        part = _mm(h_ref[:, pl.ds(k, 512)], wd_ref[pl.ds(lo, n), pl.ds(k, 512)], NT)
        ffn = part if ffn is None else ffn + part
        if k + 512 < F:
            yield
    upd_ref[pl.ds(lo, n), :] = (_round_bf16(ffn) * gate_ref[:, :n]).T


def _gate(lo, n, upd_ref, hot_ref, xp_ref, work_ref, s_ref, ds_ref, o_ref):
    for h0 in range(lo // 8, (lo + n) // 8, 8):
        nh = min(8, (lo + n) // 8 - h0)
        for p in range(4):
            scattered = [_mm(upd_ref[pl.ds(8 * h0, 8 * nh), :], hot_ref[4 * p + j])
                         for j in range(4)]
            for h in range(h0, h0 + nh):
                r = []
                for j in range(4):
                    x = _bf(xp_ref[4 * p + j, _rows(h // 2, 8), :]).astype(F32)
                    half = work_ref[h, XN + 4 * p + j]
                    s = s_ref[h, 4 * p + j] + half * ds_ref[_rows(h, 8), :]
                    half = half + scattered[j][8 * (h - h0):8 * (h - h0) + 8]
                    r.append(x[8 * (h % 2):8 * (h % 2) + 8]
                             + s * (half + half * jnp.tanh(half)))
                r = _skew(r)
                r = [r[0]] + [pltpu.roll(r[q], 128 - q, 1) for q in range(1, 4)]
                o_ref[_rows(h, 8), pl.ds(512 * p, 512)] = (
                    jnp.concatenate(r, axis=1).astype(BF16))
            yield


def _kernel(x_hbm, are_hbm, aim_hbm, bre_hbm, bim_hbm, cre_hbm, cim_hbm, ldt_hbm, dsk_hbm,
            wr_hbm, wg_hbm, wu_hbm, wd_hbm, o_hbm,
            x_ref, par_ref, ldt_ref, dsk_ref, wr_ref, wg_ref, wu_ref, wd_ref, o_ref,
            fx_ref, fxt_ref, fk_ref, fd_ref, dt_ref, ds_ref, base_ref, kv_ref, kr_ref, kf_ref,
            xp_ref, stat_ref, cen_ref, work_ref, xf_ref, s_ref,
            hot_ref, xs_ref, gate_ref, h_ref, upd_ref, sems):
    copies = []

    def fetch(src, dst):
        cp = pltpu.make_async_copy(src, dst, sems.at[len(copies)])
        copies.append(cp)
        cp.start()
        return cp

    small = [fetch(s, d) for s, d in
             ((ldt_hbm, ldt_ref), (dsk_hbm, dsk_ref), (wr_hbm, wr_ref))]
    params = [fetch(s, par_ref.at[i]) for i, s in
              enumerate((are_hbm, aim_hbm, bre_hbm, bim_hbm, cre_hbm, cim_hbm))]
    x_copy = fetch(x_hbm, x_ref)
    ups = [[fetch(src.at[:, _rows(i, F // 2)], dst.at[:, _rows(i, F // 2)])
            for src, dst in ((wg_hbm, wg_ref), (wu_hbm, wu_ref))] for i in range(2)]

    with jax.named_scope("setup"):
        for cp in small:
            cp.wait()
        _make_transforms(fx_ref, fxt_ref, fk_ref, fd_ref)
        _column(ldt_ref, dt_ref, lambda v: _round_bf16(jnp.exp(v)))
        _column(dsk_ref, ds_ref, lambda v: 2.0 * v)
        for cp in params:
            cp.wait()

    with jax.named_scope("ssm_kernel"):
        zero = _ssm_kernel(par_ref, dt_ref, base_ref, kv_ref, kr_ref)

    with jax.named_scope("layernorm"):
        x_copy.wait()
        downs = [fetch(wd_hbm.at[pl.ds(*c)], wd_ref.at[pl.ds(*c)]) for c in CHUNKS]

        def tally(p, j, n, value, first):
            kr_ref[p + zero, j, n] = value if first else kr_ref[p, j, n] + value

        def norm_pass(n, job, pieces, fine):
            @pl.when(zero < NG)
            def _():
                batches = 4 * SPLIT[n] // (1 if fine else BATCH[n])
                _weave(_ssm_spectrum(sum(SPLIT[:n]), SPLIT[n], BATCH[n], fine, kr_ref,
                                     fk_ref, fd_ref, kf_ref), job, pieces / (batches - 1))

        norm_pass(0, _norm_mean(x_ref, xp_ref, tally), 4 * NG, True)
        for c in range(16):
            stat_ref[c] = _average(kr_ref[c // 4, c % 4, 0])
            stat_ref[16 + c] = _round_bf16(stat_ref[c])
        norm_pass(1, _norm_centre(xp_ref, cen_ref, stat_ref, tally), 16 * NG // PIECE2, True)
        for c in range(16):
            stat_ref[c] = _norm_factor(kr_ref[c // 4, c % 4, 1], stat_ref[c])
        norm_pass(2, _norm_scale(wr_ref, cen_ref, stat_ref, work_ref), 20, False)

    if STOP:
        for cp in downs + ups[0] + ups[1]:
            cp.wait()
        o_ref[0:8, 0:128] = (kf_ref[zero, 0, 0] + work_ref[zero, zero] + stat_ref[zero]).astype(BF16)
        fetch(o_ref, o_hbm).wait()
        return
    with jax.named_scope("convolve"):
        def convolve(lo, hi):
            later = []
            for i in range(lo, hi):
                yield from _conv_step(i, i + zero, [0 <= i - k < NG for k in range(4)], later,
                                      kf_ref, fx_ref, fxt_ref, xf_ref, work_ref, s_ref)
            while later:
                later.pop()()

        _weave(convolve(0, CUTS[0]), _route(stat_ref, work_ref, hot_ref, xs_ref, gate_ref))
        for i in range(2):
            for cp in ups[i]:
                cp.wait()
            _weave(convolve(CUTS[i], CUTS[i + 1]),
                   _ffn_up(i * F // 2, F // 2, xs_ref, wg_ref, wu_ref, h_ref))

        downs[0].wait()
        _weave(convolve(CUTS[2], NG + 3),
               _ffn_down(*CHUNKS[0], h_ref, wd_ref, gate_ref, upd_ref))

    with jax.named_scope("finish"):
        outs = []
        for i, chunk in enumerate(CHUNKS):
            down = iter(())
            if i + 1 < len(CHUNKS):
                downs[i + 1].wait()
                down = _ffn_down(*CHUNKS[i + 1], h_ref, wd_ref, gate_ref, upd_ref)
            for k in SEND[i]:
                outs.append(fetch(o_ref.at[pl.ds(*CHUNKS[k])], o_hbm.at[pl.ds(*CHUNKS[k])]))
            _weave(_gate(*chunk, upd_ref, hot_ref, xp_ref, work_ref, s_ref, ds_ref, o_ref),
                   down, DOWN_RATE)
        outs.append(fetch(o_ref.at[pl.ds(*chunk)], o_hbm.at[pl.ds(*chunk)]))
        for cp in outs:
            cp.wait()


@jax.jit
def pallas_recurrent_scan__ssm_conv_s4__moe_arch_mod__prompt_kernel(
    A_u: jax.Array,
    A_A_re: jax.Array,
    A_A_im: jax.Array,
    A_B_re: jax.Array,
    A_B_im: jax.Array,
    A_C_re: jax.Array,
    A_C_im: jax.Array,
    A_log_dt: jax.Array,
    A_Dskip: jax.Array,
    B_x: jax.Array,
    B_w_r: jax.Array,
    B_w_gate: jax.Array,
    B_w_up: jax.Array,
    B_w_down: jax.Array,
):
    del B_x
    assert A_u.shape == (1, L, D) and A_A_re.shape == (D, N) and B_w_gate.shape == (D, F)
    assert A_A_re.dtype == BF16
    vmem = pltpu.VMEM
    nh = 2 * NG
    scratch = [
        vmem((D, L), BF16), vmem((6, D, N), BF16),
        vmem((D,), BF16), vmem((D,), BF16), vmem((D,), BF16),
        vmem((D, F), BF16), vmem((D, F), BF16), vmem((D, F), BF16), vmem((D, L), BF16),
        vmem((4, 2, 64, 128), I32), vmem((4, 128, 128), I32),
        vmem((4, 2, 64, 128), I32), vmem((4, 2, 64, 128), I32),
        vmem((D, 128), F32), vmem((D, 128), F32),
        vmem((4, 2, 104, 128), F32), vmem((4, 192, 128), F32),
        vmem((nh + 4, 5, 2, 8, 128), F32), vmem((nh, 4, 8, 8, 128), F32),
        vmem((16, D // 2, 128), I32), vmem((32, 8, 128), F32),
        vmem((16, D // 2, 256), BF16),
        vmem((nh, XN + 16, 8, 128), F32), vmem((nh, 4, 8, 8, 128), F32),
        vmem((nh, 16, 8, 128), F32),
        vmem((16, 8, 128), F32), vmem((8, D), F32), vmem((8, 128), F32), vmem((8, F), F32),
        vmem((D, TOPK), F32),
        pltpu.SemaphoreType.DMA((14 + 2 * len(CHUNKS),)),
    ]
    out = pl.pallas_call(
        _kernel,
        out_shape=jax.ShapeDtypeStruct((D, L), BF16),
        in_specs=[pl.BlockSpec(memory_space=pl.ANY)] * 13,
        out_specs=pl.BlockSpec(memory_space=pl.ANY),
        scratch_shapes=scratch,
        compiler_params=pltpu.CompilerParams(vmem_limit_bytes=100 * 1024 * 1024, flags=FLAGS),
    )(A_u[0].T, A_A_re, A_A_im, A_B_re, A_B_im, A_C_re, A_C_im, A_log_dt, A_Dskip,
      B_w_r, B_w_gate, B_w_up, B_w_down.T)
    return out.T[None]
```

```python
import itertools
import math

import jax
import jax.numpy as jnp
from jax import lax
import jax.experimental.pallas as pl
import jax.experimental.pallas.tpu as pltpu

F32, BF16, I32 = jnp.float32, jnp.bfloat16, jnp.int32
L, D, N, F, TOPK = 2048, 576, 128, 4608, 8
G = 16
NG = D // G
EPS = 1e-5
NN = (((1,), (0,)), ((), ()))
NT = (((1,), (1,)), ((), ()))
CHUNKS = ((0, 128), (128, 128), (256, 128), (384, 128), (512, 64))
FLAGS = None
RA = 6
PIECE = 3
PIECE2 = 6
BATCH = (2, 3, 3)
SPLIT = (24, 30, 18)
CUTS = (10, 22, 34)
SEND = ((), (0,), (1,), (2,), (3,))
DOWN_RATE = 1.8
ORDER_C = "eob01"


def _iota(shape, dim):
    return lax.broadcasted_iota(I32, shape, dim)


def _cmul(a, b):
    return a[0] * b[0] - a[1] * b[1], a[0] * b[1] + a[1] * b[0]


def _csq(a):
    return a[0] * a[0] - a[1] * a[1], (a[0] + a[0]) * a[1]


def _cadd(a, b):
    return a[0] + b[0], a[1] + b[1]


def _csub(a, b):
    return a[0] - b[0], a[1] - b[1]


def _cadd_i(a, b):
    return a[0] - b[1], a[1] + b[0]


def _csub_i(a, b):
    return a[0] + b[1], a[1] - b[0]


def _dft4(v, sign):
    s02, d02 = _cadd(v[0], v[2]), _csub(v[0], v[2])
    s13, d13 = _cadd(v[1], v[3]), _csub(v[1], v[3])
    a, b = _cadd_i(d02, d13), _csub_i(d02, d13)
    if sign < 0:
        a, b = b, a
    return [_cadd(s02, s13), a, _csub(s02, s13), b]


def _root(n):
    ang = (((n + 1024) & 2047) - 1024).astype(F32) * (2.0 * math.pi / 2048)
    return jnp.cos(ang), jnp.sin(ang)


def _pack(x):
    return pltpu.bitcast(x.astype(BF16), I32)


def _bf(x):
    return pltpu.bitcast(x, BF16)


def _round_bf16(x):
    return x.astype(BF16).astype(F32)


def _silu(x):
    h = 0.5 * x
    return h + h * jnp.tanh(h)


def _skew(r):
    lane = _iota(r[0].shape, 1)
    b0, b1 = (lane & 1) != 0, (lane & 2) != 0
    t = [jnp.where(b0, r[(k + 1) % 4], r[k]) for k in range(4)]
    u = [jnp.where(b1, t[(k + 2) % 4], t[k]) for k in range(4)]
    return [u[(-j) % 4] for j in range(4)]


def _x_time(j, m):
    q = (m - j) & 3
    return 128 * q + ((m - q) & 127)


def _mm(a, b, dims=NN):
    return lax.dot_general(a, b, dims, precision=lax.Precision.DEFAULT,
                           preferred_element_type=F32)


def _rows(i, n):
    return pl.ds(i * n if isinstance(i, int) else pl.multiple_of(i * n, n), n)


def _weave(main, side, rate=1.0):
    credit = 0.0
    for _ in main:
        credit += rate
        while credit >= 1.0:
            credit -= 1.0
            next(side, None)
    for _ in side:
        pass


def _column(v_ref, out_ref, fn):
    v = fn(v_ref[...].astype(F32).reshape(1, D))
    for lo in range(0, D, 128):
        n = min(128, D - lo)
        out_ref[pl.ds(lo, n), :] = jnp.broadcast_to(v[:, lo:lo + n], (128, n)).T


def _make_transforms(fx_ref, fxt_ref, fk_ref, fd_ref):
    freq = 4 * _iota((8, 128), 1) + 1
    row = _iota((8, 128), 0)
    step1 = _root(freq)
    step8 = _csq(_csq(_csq(step1)))
    step32 = _csq(_csq(step8))
    step128 = _csq(_csq(step32))

    def stack(vals, part):
        return jnp.concatenate([v[part] for v in vals], axis=0)

    def component(j, kbase):
        start = _root((_x_time(j, row + 8) - 8) * freq)
        wrapped = _cmul(start, step128)
        wraps = row < ((row - j) & 3)
        vals = [start]
        for _ in range(15):
            vals.append(_cmul(vals[-1], step8))
        vals[0] = tuple(jnp.where(wraps, a, b) for a, b in zip(wrapped, start))
        for part in range(2):
            fx_ref[j, part] = _pack(stack(vals, part))
            fxt_ref[j, pl.ds(64 * part, 64), :] = _pack(stack(vals, part).T)
        vals = [kbase]
        for _ in range(15):
            vals.append(_cmul(vals[-1], step32))
        for part in range(2):
            fk_ref[j, part] = _pack(stack(vals, part))
        return _cmul(kbase, step1)

    lax.fori_loop(0, 4, component, _root(4 * row * freq), unroll=True)

    rows = [_root((256 * (row & 1) + 8 * (row >> 1)) * freq)]
    for _ in range(7):
        rows.append(_cmul(rows[-1], step32))
    zero = jnp.zeros((8, 128), F32)
    rho = step1
    for k in range(4):
        p2 = _csq(rho)
        s3 = _cadd(_cadd(rho, p2), _cmul(p2, rho))
        s4 = _cadd(s3, _csq(p2))
        box = 1.0 + 2.0 * jnp.where((row & 2) == 0, s4[0], s3[0])
        vals = [(r[0] * box, r[1] * box) for r in rows]
        first = row == 0
        vals[0] = (jnp.where(first, 1.0 + s4[0], vals[0][0]),
                   jnp.where(first, s4[1], vals[0][1]))
        vals.append((jnp.where(first, s4[1], 0.0), jnp.where(first, s4[0], 0.0)))
        vals += [(zero, zero)] * 7
        for part in range(2):
            fd_ref[k, part] = _pack(stack(vals, part))
        rho = (-rho[1], rho[0])


def _ssm_bases(g, h, par_ref, dt_ref, base_ref):
    rows = _rows(g, G)
    a_re, a_im, b_re, b_im, c_re, c_im = (
        par_ref[k, rows, :].astype(F32) for k in range(6))
    dt = dt_ref[rows, :]
    decay, phase = dt * a_re, dt * a_im
    dts = dt * (2.0 / 512)
    w = _cmul((c_re, c_im), (dts * b_re, dts * b_im))
    row = _iota((8, 128), 0)

    def deal(v):
        return jnp.concatenate(
            [jnp.take_along_axis(v[lo:lo + 8], (row >> 1) + 4 * (row & 1), axis=0,
                                 mode="promise_in_bounds") for lo in (0, 8)], axis=0)

    decay, phase, w = deal(decay), deal(phase), (deal(w[0]), deal(w[1]))
    z, unit = {}, (jnp.cos(phase), jnp.sin(phase))
    for e in (1, 2, 4, 8, 16, 32, 64, 128, 256, 512, 1024):
        if e in (1, 4, 8, 16, 256, 1024):
            mag = jnp.exp2(decay * (e * math.log2(math.e)))
            z[e] = (mag * unit[0], mag * unit[1])
        if e < 1024:
            unit = _csq(unit)
    w8, w1024 = _cmul(w, z[8]), _cmul(w, z[1024])
    seq = [(jnp.ones_like(dt), jnp.zeros_like(dt)), z[8], z[16], z[16], _cmul(z[16], z[8]),
           z[1], z[1], z[256], z[256], w, _cmul(w, z[4]), w, w8, w1024, w8,
           w1024, _cmul(w1024, z[1024]), w1024]
    for k, v in enumerate(seq):
        for t in range(2):
            for part in range(2):
                base_ref[h + t, part, pl.ds(8 * k, 8), :] = v[part][8 * t:8 * t + 8]


_OFFSETS = ((0, 4), (1, 5), (2, 6), (3, 7), (256, 260), (512, 516), (768, 772),
            (258, 262), (264, 1280), (520, 1536), (776, 1792), (1024, 2048))


def _ssm_values(h, base_ref, kv_ref):
    for quad in range(2):
        def pair(k):
            return tuple(base_ref[h, part, pl.ds(8 * k + quad, 8, stride=2), :]
                         for part in range(2))
        v, z16 = [pair(0), pair(3)], pair(2)
        for _ in range(14):
            v.append(_cmul(v[-1], z16))
        z1, z256 = pair(5), pair(7)
        w = [pair(9 + quad)]
        for _ in range(3):
            w.append(_cmul(w[-1], z1))
        w.append(_cmul(w[0], z256))
        for _ in range(2):
            w.append(_cmul(w[-1], z256))
        w.append(_cmul(w[2], z256))
        w.append(_cmul(pair(12 + quad), z256))
        for _ in range(2):
            w.append(_cmul(w[-1], z256))
        w.append(pair(15 + quad))
        re, im = (_mm(jnp.concatenate([t[part] for t in w], axis=0),
                      jnp.concatenate([t[part] for t in v[::-1]], axis=0), NT)
                  for part in range(2))
        out = re - im
        for u in range(12):
            kv_ref[h, pl.ds(16 * u + 8 * quad, 8), :] = out[8 * u:8 * u + 8]


def _ssm_arrange(h, slot, kv_ref, kr_ref):
    lane, row = _iota((8, 128), 1), _iota((8, 128), 0)
    src = 4 * (((lane >> 1) & 31) ^ 30) + (row & 3)

    def even(a, b):
        return jnp.where((lane & 1) == 0, a, b)

    def low(a, b):
        return jnp.where(lane < 64, a, b)

    val = {}
    for u, pair in enumerate(_OFFSETS):
        a, b = kv_ref[h, pl.ds(16 * u, 8), :], kv_ref[h, pl.ds(16 * u + 8, 8), :]
        for e, x in zip(pair, (jnp.where(row < 4, a, b),
                               pltpu.roll(jnp.where(row < 4, b, a), 4, 0))):
            val[e] = jnp.take_along_axis(x, src, axis=1, mode="promise_in_bounds")
    mid = even(val[256], val[260])
    blk0 = [low(even(val[0], val[4]), mid), low(even(val[1], val[5]), mid),
            low(even(val[2], val[6]), even(val[258], val[262])),
            low(even(val[3], val[7]), even(val[260], val[264])),
            low(even(val[1024], val[1280]), val[1536])]
    q0, q4, q8 = low(val[512], val[768]), low(val[516], val[772]), low(val[520], val[776])
    blk1 = [even(q0, q4), even(q0, q4), even(q0, q8), even(q4, q8),
            low(even(val[1536], val[1792]), jnp.where(lane == 64, val[2048], 0.0))]
    for j in range(5):
        kr_ref[slot, j, 0] = blk0[j]
        kr_ref[slot, j, 1] = blk1[j]


def _ssm_kernel(wait_rest, par_ref, dt_ref, base_ref, kv_ref, kr_ref):
    def body(n, zero):
        pl.when(n == 1)(wait_rest)
        for r in range(RA):
            g, slot = n * RA + r, 2 * (r % 2)
            for t in range(2):
                _ssm_arrange(slot + t, 2 * g + t, kv_ref, kr_ref)
                _ssm_values(slot + t, base_ref, kv_ref)
            ahead = g + 2 if r + 2 < RA else jnp.minimum(g + 2, NG - 1)
            _ssm_bases(ahead, slot, par_ref, dt_ref, base_ref)
        return jnp.minimum(zero, n * L)

    for g in range(2):
        _ssm_bases(g, 2 * g, par_ref, dt_ref, base_ref)
    kv_ref[...] = jnp.zeros_like(kv_ref)
    zero = lax.fori_loop(0, NG // RA, body, L)
    for h in range(4):
        _ssm_arrange(h, 2 * NG + h, kv_ref, kr_ref)
    return zero


def _ssm_spectrum(first, count, HB, fine, kr_ref, fk_ref, fd_ref, kf_ref):
    for h0 in range(0, count, HB):
        near, far = [], []
        for n in range(4):
            lhs = {j: [] for j in ((0, 1, 2, 3) if n < 2 else (4,))}
            for h in range(HB):
                for p in range(2):
                    for j, rows in lhs.items():
                        rows.append(kr_ref[4 + first + h0 + h, j, p])
                if fine:
                    yield
            lhs = {j: jnp.concatenate(rows, axis=0) for j, rows in lhs.items()}
            if n < 2:
                near.append([_mm(lhs[j], _bf(fk_ref[j, n])) for j in range(4)])
            else:
                far += [[_mm(lhs[4], _bf(fd_ref[k, part])) for part in range(2)]
                        for k in (2 * n - 4, 2 * n - 3)]
            if not fine:
                yield
        for h in range(HB):
            r = [slice(8 * (2 * h + p), 8 * (2 * h + p + 1)) for p in range(2)]
            spec = [_dft4([(near[0][j][r[p]], near[1][j][r[p]]) for j in range(4)], 1)
                    for p in range(2)]
            spec += [[(far[k][0][r[p]], far[k][1][r[p]]) for k in range(4)]
                     for p in range(2)]
            for p in range(4):
                for k in range(4):
                    v = spec[p][k] if p == 0 else _csub_i(spec[p][k], spec[p - 1][k])
                    for part in range(2):
                        kf_ref[first + h0 + h, k, 2 * p + part] = v[part]


XN = 32


def _norm_mean(x_ref, xp_ref, tally):
    for p in range(4):
        acc = [None] * 4
        for g in range(NG):
            r = [pltpu.bitcast(x_ref[_rows(g, G), _rows(4 * p + q, 128)], I32)
                 for q in range(4)]
            r = _skew([r[0]] + [pltpu.roll(r[q], q, 1) for q in range(1, 4)])
            for j in range(4):
                xp_ref[4 * p + j, _rows(g, 8), :] = r[j]
                x = _bf(r[j]).astype(F32)
                acc[j] = x[:8] + x[8:] if g % PIECE == 0 else acc[j] + (x[:8] + x[8:])
                if g % PIECE == PIECE - 1:
                    tally(p, j, 0, acc[j], g < PIECE)
            yield


def _norm_centre(xp_ref, cen_ref, stat_ref, tally):
    for lo in range(0, NG, PIECE2):
        for c in range(16):
            m, acc = stat_ref[16 + c], None
            for g in range(lo, lo + PIECE2):
                x = _bf(xp_ref[c, _rows(g, 8), :]).astype(F32)
                d = [x[:8] - m, x[8:] - m]
                sq = d[0] * d[0] + d[1] * d[1]
                acc = sq if g == lo else acc + sq
                cen_ref[c, _rows(g, 8), :] = jnp.concatenate(d, axis=1).astype(BF16)
            tally(c // 4, c % 4, 1, acc, lo == 0)
            yield


def _average(v):
    return jnp.broadcast_to(jnp.sum(v, axis=0, keepdims=True), v.shape) / D


def _norm_factor(squares, mean):
    shift = mean - _round_bf16(mean)
    var = _round_bf16(jnp.maximum(_average(squares) - shift * shift, 0.0))
    eps = _round_bf16(jnp.full_like(var, EPS))
    return 0.5 / _round_bf16(jnp.sqrt(_round_bf16(var + eps)))


def _norm_scale(wr_ref, cen_ref, stat_ref, work_ref):
    wr = jnp.broadcast_to(2.0 * wr_ref[...].astype(F32).reshape(1, D), (8, D))
    for p in range(4):
        cols = range(4 * p, 4 * p + 4)
        inv, score = {c: stat_ref[c] for c in cols}, {}
        for lo in range(0, NG, 8):
            for c in cols:
                vals = []
                for g in reversed(range(lo, min(lo + 8, NG))):
                    d = cen_ref[c, _rows(g, 8), :].astype(F32)
                    for t in (1, 0):
                        vals.insert(0, d[:, 128 * t:128 * t + 128] * inv[c])
                        work_ref[2 * g + t, XN + c] = vals[0]
                part = _mm(wr[:, G * lo:G * lo + 8 * len(vals)],
                           jnp.concatenate(vals, axis=0))
                score[c] = part if lo == 0 else score[c] + part
            yield
        for c in cols:
            stat_ref[c] = score[c]


def _route(stat_ref, work_ref, hot_ref, xs_ref, gate_ref):
    row = _iota((8, 128), 0)
    halves = []
    for lo in (0, 8):
        dense = stat_ref[lo]
        for c in range(1, 8):
            dense = jnp.where(row == c, stat_ref[lo + c], dense)
        halves.append(dense)
    score = _round_bf16(jnp.concatenate(halves, axis=0))
    blk = _iota((16, 128), 0)
    bits = pltpu.bitcast(jnp.where(score == 0.0, 0.0, score), I32) >> 16
    order = jnp.where(bits < 0, bits ^ 0x7FFF, bits) + 0x8000
    time = 512 * (blk >> 2) + _x_time(blk & 3, _iota((16, 128), 1))
    key = pltpu.bitcast((1 << 29) + (order << 11) + (L - 1 - time), F32)
    rank = jnp.full((16, 128), TOPK, I32)
    best = jnp.zeros((8, 128), F32)
    for i in range(TOPK):
        top = jnp.max(jnp.max(key, axis=0, keepdims=True), axis=1, keepdims=True)
        hit = key == top
        rank = jnp.where(hit, i, rank)
        key = jnp.where(hit, 0.0, key)
        best = jnp.where(row == i, top, best)
        yield
        yield
    order = ((pltpu.bitcast(best, I32) >> 11) & 0xFFFF) - 0x8000
    best = pltpu.bitcast(jnp.where(order < 0, order ^ 0x7FFF, order) << 16, F32)
    gate_ref[...] = 0.5 * _round_bf16(jax.nn.sigmoid(best))
    for c in range(16):
        hot_ref[c] = jnp.where(jnp.broadcast_to(rank[c:c + 1], (8, 128)) == row, 1.0, 0.0)
    for lo in range(0, D, 128):
        n, picked = min(128, D - lo), None
        for c in range(16):
            tokens = work_ref[pl.ds(lo // 8, n // 8), XN + c].reshape(n, 128)
            part = _mm(hot_ref[c], tokens, NT)
            picked = part if c == 0 else picked + part
            if c % 4 == 3:
                yield
        xs_ref[:, pl.ds(lo, n)] = 2.0 * picked


def _ffn_up(first, count, xs_ref, wg_ref, wu_ref, h_ref):
    for col in range(first, first + count, 256):
        acc = [None, None]
        for lo in range(0, D, 128):
            rows = pl.ds(lo, min(128, D - lo))
            for n, w_ref in enumerate((wg_ref, wu_ref)):
                part = _mm(xs_ref[:, rows], w_ref[rows, pl.ds(col, 256)])
                acc[n] = part if lo == 0 else acc[n] + part
            yield
        h_ref[:, pl.ds(col, 256)] = (
            _round_bf16(_silu(_round_bf16(acc[0]))) * _round_bf16(acc[1]))


def _conv_step(i, same, live, later, kf_ref, fx_ref, fxt_ref, xf_ref, work_ref, s_ref):
    def products():
        for t in range(2):
            h = 2 * (i - 2) + t
            for k in range(4):
                kf = [(kf_ref[h, k, 2 * p], kf_ref[h, k, 2 * p + 1]) for p in range(4)]
                x = [(xf_ref[h, k, 2 * p], xf_ref[h, k, 2 * p + 1]) for p in range(4)]
                for c in (3, 0, 2, 1):
                    acc = _cmul(kf[0], x[c])
                    for p in range(1, c + 1):
                        acc = _cadd(acc, _cmul(kf[p], x[c - p]))
                    for part in range(2):
                        work_ref[2 * (same - 2) + t, 8 * c + 2 * k + part] = acc[part]
                    if c < 2:
                        yield

    fill = products() if live[2] else iter(())
    comp = [None] * 2

    def forward(part):
        lhs = [[] for _ in range(4)]
        for t in range(2):
            for p in range(4):
                for j in range(4):
                    lhs[j].append(work_ref[2 * i + t, XN + 4 * p + j])
                if p % 2:
                    next(fill, None)
        comp[part] = [_mm(jnp.concatenate(lhs[j], axis=0), _bf(fx_ref[j, part]))
                      for j in range(4)]

    def butterflies():
        for t in range(2):
            for p in range(4):
                r = slice(8 * (4 * t + p), 8 * (4 * t + p + 1))
                spec = _dft4([(comp[0][j][r], comp[1][j][r]) for j in range(4)], 1)
                for k in range(4):
                    for part in range(2):
                        xf_ref[2 * same + t, k, 2 * p + part] = spec[k][part]

    def inverse(odd):
        lhs = [[], []]
        for t in range(2):
            h = 2 * (i - 3) + t
            for c in range(4):
                v = [(work_ref[h, 8 * c + 2 * k], work_ref[h, 8 * c + 2 * k + 1])
                     for k in range(4)]
                if odd:
                    a, b = _csub(v[0], v[2]), _csub(v[1], v[3])
                    back = _csub_i(a, b), _cadd_i(a, b)
                else:
                    a, b = _cadd(v[0], v[2]), _cadd(v[1], v[3])
                    back = _cadd(a, b), _csub(a, b)
                for n in range(2):
                    lhs[n].append(jnp.concatenate(back[n], axis=1))
                if c % 2:
                    next(fill, None)
        y = [_mm(jnp.concatenate(lhs[n], axis=0), _bf(fxt_ref[odd + 2 * n]))
             for n in range(2)]
        for t in range(2):
            for c in range(4):
                for n in range(2):
                    s_ref[2 * (i - 3) + t, 4 * c + odd + 2 * n] = (
                        y[n][32 * t + 8 * c:32 * t + 8 * c + 8])

    for op in ORDER_C:
        if op in "01" and live[0]:
            forward(int(op))
        if op in "eo" and live[3]:
            inverse(int(op == "o"))
        while op == "b" and later:
            later.pop()()
        if op != "b":
            yield
    for _ in fill:
        pass
    if live[0]:
        later.append(butterflies)


def _ffn_down(lo, n, h_ref, wd_ref, gate_ref, upd_ref):
    ffn = None
    for k in range(0, F, 512):
        part = _mm(h_ref[:, pl.ds(k, 512)], wd_ref[pl.ds(lo, n), pl.ds(k, 512)], NT)
        ffn = part if ffn is None else ffn + part
        if k + 512 < F:
            yield
    upd_ref[pl.ds(lo, n), :] = (_round_bf16(ffn) * gate_ref[:, :n]).T


def _gate(lo, n, upd_ref, hot_ref, xp_ref, work_ref, s_ref, ds_ref, o_ref):
    for h0 in range(lo // 8, (lo + n) // 8, 8):
        nh = min(8, (lo + n) // 8 - h0)
        for p in range(4):
            scattered = [_mm(upd_ref[pl.ds(8 * h0, 8 * nh), :], hot_ref[4 * p + j])
                         for j in range(4)]
            for h in range(h0, h0 + nh):
                r = []
                for j in range(4):
                    x = _bf(xp_ref[4 * p + j, _rows(h // 2, 8), :]).astype(F32)
                    half = work_ref[h, XN + 4 * p + j]
                    s = s_ref[h, 4 * p + j] + half * ds_ref[_rows(h, 8), :]
                    half = half + scattered[j][8 * (h - h0):8 * (h - h0) + 8]
                    r.append(x[8 * (h % 2):8 * (h % 2) + 8]
                             + s * (half + half * jnp.tanh(half)))
                r = _skew(r)
                r = [r[0]] + [pltpu.roll(r[q], 128 - q, 1) for q in range(1, 4)]
                o_ref[_rows(h, 8), pl.ds(512 * p, 512)] = (
                    jnp.concatenate(r, axis=1).astype(BF16))
            yield


def _kernel(x_hbm, are_hbm, aim_hbm, bre_hbm, bim_hbm, cre_hbm, cim_hbm, ldt_hbm, dsk_hbm,
            wr_hbm, wg_hbm, wu_hbm, wd_hbm, o_hbm,
            x_ref, par_ref, ldt_ref, dsk_ref, wr_ref, wg_ref, wu_ref, wd_ref, o_ref,
            fx_ref, fxt_ref, fk_ref, fd_ref, dt_ref, ds_ref, base_ref, kv_ref, kr_ref, kf_ref,
            xp_ref, stat_ref, cen_ref, work_ref, xf_ref, s_ref,
            hot_ref, xs_ref, gate_ref, h_ref, upd_ref, sems):
    copies = []

    def fetch(src, dst):
        cp = pltpu.make_async_copy(src, dst, sems.at[len(copies)])
        copies.append(cp)
        cp.start()
        return cp

    def fetch_params(rows):
        return [fetch(src.at[rows], par_ref.at[i, rows]) for i, src in
                enumerate((are_hbm, aim_hbm, bre_hbm, bim_hbm, cre_hbm, cim_hbm))]

    head = [fetch(ldt_hbm, ldt_ref)] + fetch_params(pl.ds(0, (RA + 2) * G))
    rest = fetch_params(pl.ds((RA + 2) * G, D - (RA + 2) * G)) + [fetch(dsk_hbm, dsk_ref)]
    x_copies = [fetch(x_hbm, x_ref), fetch(wr_hbm, wr_ref)]

    with jax.named_scope("setup"):
        _make_transforms(fx_ref, fxt_ref, fk_ref, fd_ref)
        for cp in head:
            cp.wait()
        ups = [[fetch(src.at[:, _rows(i, F // 2)], dst.at[:, _rows(i, F // 2)])
                for src, dst in ((wg_hbm, wg_ref), (wu_hbm, wu_ref))] for i in range(2)]
        _column(ldt_ref, dt_ref, lambda v: _round_bf16(jnp.exp(v)))

    def wait_rest():
        for cp in rest:
            cp.wait()

    with jax.named_scope("ssm_kernel"):
        zero = _ssm_kernel(wait_rest, par_ref, dt_ref, base_ref, kv_ref, kr_ref)

    with jax.named_scope("layernorm"):
        for cp in x_copies:
            cp.wait()
        downs = [fetch(wd_hbm.at[pl.ds(*c)], wd_ref.at[pl.ds(*c)]) for c in CHUNKS]

        def tally(p, j, n, value, first):
            kr_ref[p + zero, j, n] = value if first else kr_ref[p, j, n] + value

        def norm_pass(n, job, pieces, fine):
            @pl.when(zero < NG)
            def _():
                batches = 4 * SPLIT[n] // (1 if fine else BATCH[n])
                _weave(_ssm_spectrum(sum(SPLIT[:n]), SPLIT[n], BATCH[n], fine, kr_ref,
                                     fk_ref, fd_ref, kf_ref), job, pieces / (batches - 1))

        norm_pass(0, _norm_mean(x_ref, xp_ref, tally), 4 * NG, True)
        for c in range(16):
            stat_ref[c] = _average(kr_ref[c // 4, c % 4, 0])
            stat_ref[16 + c] = _round_bf16(stat_ref[c])
        norm_pass(1, _norm_centre(xp_ref, cen_ref, stat_ref, tally), 16 * NG // PIECE2, True)
        for c in range(16):
            stat_ref[c] = _norm_factor(kr_ref[c // 4, c % 4, 1], stat_ref[c])
        norm_pass(2, _norm_scale(wr_ref, cen_ref, stat_ref, work_ref), 20, False)

    with jax.named_scope("convolve"):
        def convolve(lo, hi):
            later = []
            for i in range(lo, hi):
                yield from _conv_step(i, i + zero, [0 <= i - k < NG for k in range(4)], later,
                                      kf_ref, fx_ref, fxt_ref, xf_ref, work_ref, s_ref)
            while later:
                later.pop()()

        _weave(convolve(0, CUTS[0]), _route(stat_ref, work_ref, hot_ref, xs_ref, gate_ref))
        for i in range(2):
            for cp in ups[i]:
                cp.wait()
            _weave(convolve(CUTS[i], CUTS[i + 1]),
                   _ffn_up(i * F // 2, F // 2, xs_ref, wg_ref, wu_ref, h_ref))

        downs[0].wait()
        _column(dsk_ref, ds_ref, lambda v: 2.0 * v)
        _weave(convolve(CUTS[2], NG + 3),
               _ffn_down(*CHUNKS[0], h_ref, wd_ref, gate_ref, upd_ref))

    with jax.named_scope("finish"):
        outs = []
        for i, chunk in enumerate(CHUNKS):
            down = iter(())
            if i + 1 < len(CHUNKS):
                downs[i + 1].wait()
                down = _ffn_down(*CHUNKS[i + 1], h_ref, wd_ref, gate_ref, upd_ref)
            for k in SEND[i]:
                outs.append(fetch(o_ref.at[pl.ds(*CHUNKS[k])], o_hbm.at[pl.ds(*CHUNKS[k])]))
            _weave(_gate(*chunk, upd_ref, hot_ref, xp_ref, work_ref, s_ref, ds_ref, o_ref),
                   down, DOWN_RATE)
        outs.append(fetch(o_ref.at[pl.ds(*chunk)], o_hbm.at[pl.ds(*chunk)]))
        for cp in outs:
            cp.wait()


@jax.jit
def pallas_recurrent_scan__ssm_conv_s4__moe_arch_mod__prompt_kernel(
    A_u: jax.Array,
    A_A_re: jax.Array,
    A_A_im: jax.Array,
    A_B_re: jax.Array,
    A_B_im: jax.Array,
    A_C_re: jax.Array,
    A_C_im: jax.Array,
    A_log_dt: jax.Array,
    A_Dskip: jax.Array,
    B_x: jax.Array,
    B_w_r: jax.Array,
    B_w_gate: jax.Array,
    B_w_up: jax.Array,
    B_w_down: jax.Array,
):
    del B_x
    assert A_u.shape == (1, L, D) and A_A_re.shape == (D, N) and B_w_gate.shape == (D, F)
    assert A_A_re.dtype == BF16
    vmem = pltpu.VMEM
    nh = 2 * NG
    scratch = [
        vmem((D, L), BF16), vmem((6, D, N), BF16),
        vmem((D,), BF16), vmem((D,), BF16), vmem((D,), BF16),
        vmem((D, F), BF16), vmem((D, F), BF16), vmem((D, F), BF16), vmem((D, L), BF16),
        vmem((4, 2, 64, 128), I32), vmem((4, 128, 128), I32),
        vmem((4, 2, 64, 128), I32), vmem((4, 2, 64, 128), I32),
        vmem((D, 128), F32), vmem((D, 128), F32),
        vmem((4, 2, 144, 128), F32), vmem((4, 192, 128), F32),
        vmem((nh + 4, 5, 2, 8, 128), F32), vmem((nh, 4, 8, 8, 128), F32),
        vmem((16, D // 2, 128), I32), vmem((32, 8, 128), F32),
        vmem((16, D // 2, 256), BF16),
        vmem((nh, XN + 16, 8, 128), F32), vmem((nh, 4, 8, 8, 128), F32),
        vmem((nh, 16, 8, 128), F32),
        vmem((16, 8, 128), F32), vmem((8, D), F32), vmem((8, 128), F32), vmem((8, F), F32),
        vmem((D, TOPK), F32),
        pltpu.SemaphoreType.DMA((20 + 2 * len(CHUNKS),)),
    ]
    out = pl.pallas_call(
        _kernel,
        out_shape=jax.ShapeDtypeStruct((D, L), BF16),
        in_specs=[pl.BlockSpec(memory_space=pl.ANY)] * 13,
        out_specs=pl.BlockSpec(memory_space=pl.ANY),
        scratch_shapes=scratch,
        compiler_params=pltpu.CompilerParams(vmem_limit_bytes=100 * 1024 * 1024, flags=FLAGS),
    )(A_u[0].T, A_A_re, A_A_im, A_B_re, A_B_im, A_C_re, A_C_im, A_log_dt, A_Dskip,
      B_w_r, B_w_gate, B_w_up, B_w_down.T)
    return out.T[None]
```

```python
import itertools
import math

import jax
import jax.numpy as jnp
from jax import lax
import jax.experimental.pallas as pl
import jax.experimental.pallas.tpu as pltpu

F32, BF16, I32 = jnp.float32, jnp.bfloat16, jnp.int32
L, D, N, F, TOPK = 2048, 576, 128, 4608, 8
G = 16
NG = D // G
EPS = 1e-5
NN = (((1,), (0,)), ((), ()))
NT = (((1,), (1,)), ((), ()))
CHUNKS = ((0, 128), (128, 128), (256, 128), (384, 128), (512, 64))
FLAGS = None
RA = 6
PIECE = 3
PIECE2 = 6
BATCH = (2, 3, 3)
SPLIT = (24, 30, 18)
CUTS = (22, 34)
SEND = {1: (0, 128), 2: (128, 128), 3: (256, 128), 4: (384, 128)}
DOWN_RATE = 1.8
DOWN_COPIES = ((0, 256), (256, 272), (528, 48))
WAITS = {1: 1, 3: 2}
ORDER_C = "eob01"


def _iota(shape, dim):
    return lax.broadcasted_iota(I32, shape, dim)


def _cmul(a, b):
    return a[0] * b[0] - a[1] * b[1], a[0] * b[1] + a[1] * b[0]


def _csq(a):
    return a[0] * a[0] - a[1] * a[1], (a[0] + a[0]) * a[1]


def _cadd(a, b):
    return a[0] + b[0], a[1] + b[1]


def _csub(a, b):
    return a[0] - b[0], a[1] - b[1]


def _cadd_i(a, b):
    return a[0] - b[1], a[1] + b[0]


def _csub_i(a, b):
    return a[0] + b[1], a[1] - b[0]


def _dft4(v, sign):
    s02, d02 = _cadd(v[0], v[2]), _csub(v[0], v[2])
    s13, d13 = _cadd(v[1], v[3]), _csub(v[1], v[3])
    a, b = _cadd_i(d02, d13), _csub_i(d02, d13)
    if sign < 0:
        a, b = b, a
    return [_cadd(s02, s13), a, _csub(s02, s13), b]


def _root(n):
    ang = (((n + 1024) & 2047) - 1024).astype(F32) * (2.0 * math.pi / 2048)
    return jnp.cos(ang), jnp.sin(ang)


def _pack(x):
    return pltpu.bitcast(x.astype(BF16), I32)


def _bf(x):
    return pltpu.bitcast(x, BF16)


def _round_bf16(x):
    return x.astype(BF16).astype(F32)


def _silu(x):
    h = 0.5 * x
    return h + h * jnp.tanh(h)


def _skew(r):
    lane = _iota(r[0].shape, 1)
    b0, b1 = (lane & 1) != 0, (lane & 2) != 0
    t = [jnp.where(b0, r[(k + 1) % 4], r[k]) for k in range(4)]
    u = [jnp.where(b1, t[(k + 2) % 4], t[k]) for k in range(4)]
    return [u[(-j) % 4] for j in range(4)]


def _x_time(j, m):
    q = (m - j) & 3
    return 128 * q + ((m - q) & 127)


def _mm(a, b, dims=NN):
    return lax.dot_general(a, b, dims, precision=lax.Precision.DEFAULT,
                           preferred_element_type=F32)


def _rows(i, n):
    return pl.ds(i * n if isinstance(i, int) else pl.multiple_of(i * n, n), n)


def _weave(main, side, rate=1.0):
    credit = 0.0
    for _ in main:
        credit += rate
        while credit >= 1.0:
            credit -= 1.0
            next(side, None)
    for _ in side:
        pass


def _column(v_ref, out_ref, fn):
    v = fn(v_ref[...].astype(F32).reshape(1, D))
    for lo in range(0, D, 128):
        n = min(128, D - lo)
        out_ref[pl.ds(lo, n), :] = jnp.broadcast_to(v[:, lo:lo + n], (128, n)).T


def _make_transforms(fx_ref, fxt_ref, fk_ref, fd_ref):
    freq = 4 * _iota((8, 128), 1) + 1
    row = _iota((8, 128), 0)
    step1 = _root(freq)
    step8 = _csq(_csq(_csq(step1)))
    step32 = _csq(_csq(step8))
    step128 = _csq(_csq(step32))

    def stack(vals, part):
        return jnp.concatenate([v[part] for v in vals], axis=0)

    def component(j, kbase):
        start = _root((_x_time(j, row + 8) - 8) * freq)
        wrapped = _cmul(start, step128)
        wraps = row < ((row - j) & 3)
        vals = [start]
        for _ in range(15):
            vals.append(_cmul(vals[-1], step8))
        vals[0] = tuple(jnp.where(wraps, a, b) for a, b in zip(wrapped, start))
        for part in range(2):
            fx_ref[j, part] = _pack(stack(vals, part))
            fxt_ref[j, pl.ds(64 * part, 64), :] = _pack(stack(vals, part).T)
        vals = [kbase]
        for _ in range(15):
            vals.append(_cmul(vals[-1], step32))
        for part in range(2):
            fk_ref[j, part] = _pack(stack(vals, part))
        return _cmul(kbase, step1)

    lax.fori_loop(0, 4, component, _root(4 * row * freq), unroll=True)

    rows = [_root((256 * (row & 1) + 8 * (row >> 1)) * freq)]
    for _ in range(7):
        rows.append(_cmul(rows[-1], step32))
    zero = jnp.zeros((8, 128), F32)
    rho = step1
    for k in range(4):
        p2 = _csq(rho)
        s3 = _cadd(_cadd(rho, p2), _cmul(p2, rho))
        s4 = _cadd(s3, _csq(p2))
        box = 1.0 + 2.0 * jnp.where((row & 2) == 0, s4[0], s3[0])
        vals = [(r[0] * box, r[1] * box) for r in rows]
        first = row == 0
        vals[0] = (jnp.where(first, 1.0 + s4[0], vals[0][0]),
                   jnp.where(first, s4[1], vals[0][1]))
        vals.append((jnp.where(first, s4[1], 0.0), jnp.where(first, s4[0], 0.0)))
        vals += [(zero, zero)] * 7
        for part in range(2):
            fd_ref[k, part] = _pack(stack(vals, part))
        rho = (-rho[1], rho[0])


def _ssm_bases(g, h, par_ref, dt_ref, base_ref):
    rows = _rows(g, G)
    a_re, a_im, b_re, b_im, c_re, c_im = (
        par_ref[k, rows, :].astype(F32) for k in range(6))
    dt = dt_ref[rows, :]
    decay, phase = dt * a_re, dt * a_im
    dts = dt * (2.0 / 512)
    w = _cmul((c_re, c_im), (dts * b_re, dts * b_im))
    row = _iota((8, 128), 0)

    def deal(v):
        return jnp.concatenate(
            [jnp.take_along_axis(v[lo:lo + 8], (row >> 1) + 4 * (row & 1), axis=0,
                                 mode="promise_in_bounds") for lo in (0, 8)], axis=0)

    decay, phase, w = deal(decay), deal(phase), (deal(w[0]), deal(w[1]))
    z, unit = {}, (jnp.cos(phase), jnp.sin(phase))
    for e in (1, 2, 4, 8, 16, 32, 64, 128, 256, 512, 1024):
        if e in (1, 4, 8, 16, 256, 1024):
            mag = jnp.exp2(decay * (e * math.log2(math.e)))
            z[e] = (mag * unit[0], mag * unit[1])
        if e < 1024:
            unit = _csq(unit)
    w8, w1024 = _cmul(w, z[8]), _cmul(w, z[1024])
    seq = [(jnp.ones_like(dt), jnp.zeros_like(dt)), z[8], z[16], z[16], _cmul(z[16], z[8]),
           z[1], z[1], z[256], z[256], w, _cmul(w, z[4]), w, w8, w1024, w8,
           w1024, _cmul(w1024, z[1024]), w1024]
    for k, v in enumerate(seq):
        for t in range(2):
            for part in range(2):
                base_ref[h + t, part, pl.ds(8 * k, 8), :] = v[part][8 * t:8 * t + 8]


_OFFSETS = ((0, 4), (1, 5), (2, 6), (3, 7), (256, 260), (512, 516), (768, 772),
            (258, 262), (264, 1280), (520, 1536), (776, 1792), (1024, 2048))


def _ssm_values(h, base_ref, kv_ref):
    for quad in range(2):
        def pair(k):
            return tuple(base_ref[h, part, pl.ds(8 * k + quad, 8, stride=2), :]
                         for part in range(2))
        v, z16 = [pair(0), pair(3)], pair(2)
        for _ in range(14):
            v.append(_cmul(v[-1], z16))
        z1, z256 = pair(5), pair(7)
        w = [pair(9 + quad)]
        for _ in range(3):
            w.append(_cmul(w[-1], z1))
        w.append(_cmul(w[0], z256))
        for _ in range(2):
            w.append(_cmul(w[-1], z256))
        w.append(_cmul(w[2], z256))
        w.append(_cmul(pair(12 + quad), z256))
        for _ in range(2):
            w.append(_cmul(w[-1], z256))
        w.append(pair(15 + quad))
        re, im = (_mm(jnp.concatenate([t[part] for t in w], axis=0),
                      jnp.concatenate([t[part] for t in v[::-1]], axis=0), NT)
                  for part in range(2))
        out = re - im
        for u in range(12):
            kv_ref[h, pl.ds(16 * u + 8 * quad, 8), :] = out[8 * u:8 * u + 8]


def _ssm_arrange(h, slot, kv_ref, kr_ref):
    lane, row = _iota((8, 128), 1), _iota((8, 128), 0)
    src = 4 * (((lane >> 1) & 31) ^ 30) + (row & 3)

    def even(a, b):
        return jnp.where((lane & 1) == 0, a, b)

    def low(a, b):
        return jnp.where(lane < 64, a, b)

    val = {}
    for u, pair in enumerate(_OFFSETS):
        a, b = kv_ref[h, pl.ds(16 * u, 8), :], kv_ref[h, pl.ds(16 * u + 8, 8), :]
        for e, x in zip(pair, (jnp.where(row < 4, a, b),
                               pltpu.roll(jnp.where(row < 4, b, a), 4, 0))):
            val[e] = jnp.take_along_axis(x, src, axis=1, mode="promise_in_bounds")
    mid = even(val[256], val[260])
    blk0 = [low(even(val[0], val[4]), mid), low(even(val[1], val[5]), mid),
            low(even(val[2], val[6]), even(val[258], val[262])),
            low(even(val[3], val[7]), even(val[260], val[264])),
            low(even(val[1024], val[1280]), val[1536])]
    q0, q4, q8 = low(val[512], val[768]), low(val[516], val[772]), low(val[520], val[776])
    blk1 = [even(q0, q4), even(q0, q4), even(q0, q8), even(q4, q8),
            low(even(val[1536], val[1792]), jnp.where(lane == 64, val[2048], 0.0))]
    for j in range(5):
        kr_ref[slot, j, 0] = blk0[j]
        kr_ref[slot, j, 1] = blk1[j]


def _ssm_kernel(wait_rest, par_ref, dt_ref, base_ref, kv_ref, kr_ref):
    def body(n, zero):
        pl.when(n == 1)(wait_rest)
        for r in range(RA):
            g, slot = n * RA + r, 2 * (r % 2)
            for t in range(2):
                _ssm_arrange(slot + t, 2 * g + t, kv_ref, kr_ref)
                _ssm_values(slot + t, base_ref, kv_ref)
            ahead = g + 2 if r + 2 < RA else jnp.minimum(g + 2, NG - 1)
            _ssm_bases(ahead, slot, par_ref, dt_ref, base_ref)
        return jnp.minimum(zero, n * L)

    for g in range(2):
        _ssm_bases(g, 2 * g, par_ref, dt_ref, base_ref)
    kv_ref[...] = jnp.zeros_like(kv_ref)
    zero = lax.fori_loop(0, NG // RA, body, L)
    for h in range(4):
        _ssm_arrange(h, 2 * NG + h, kv_ref, kr_ref)
    return zero


def _ssm_spectrum(first, count, HB, fine, kr_ref, fk_ref, fd_ref, kf_ref):
    for h0 in range(0, count, HB):
        near, far = [], []
        for n in range(4):
            lhs = {j: [] for j in ((0, 1, 2, 3) if n < 2 else (4,))}
            for h in range(HB):
                for p in range(2):
                    for j, rows in lhs.items():
                        rows.append(kr_ref[4 + first + h0 + h, j, p])
                if fine:
                    yield
            lhs = {j: jnp.concatenate(rows, axis=0) for j, rows in lhs.items()}
            if n < 2:
                near.append([_mm(lhs[j], _bf(fk_ref[j, n])) for j in range(4)])
            else:
                far += [[_mm(lhs[4], _bf(fd_ref[k, part])) for part in range(2)]
                        for k in (2 * n - 4, 2 * n - 3)]
            if not fine:
                yield
        for h in range(HB):
            r = [slice(8 * (2 * h + p), 8 * (2 * h + p + 1)) for p in range(2)]
            spec = [_dft4([(near[0][j][r[p]], near[1][j][r[p]]) for j in range(4)], 1)
                    for p in range(2)]
            spec += [[(far[k][0][r[p]], far[k][1][r[p]]) for k in range(4)]
                     for p in range(2)]
            for p in range(4):
                for k in range(4):
                    v = spec[p][k] if p == 0 else _csub_i(spec[p][k], spec[p - 1][k])
                    for part in range(2):
                        kf_ref[first + h0 + h, k, 2 * p + part] = v[part]


XN = 32


def _norm_mean(x_ref, xp_ref, tally):
    for p in range(4):
        acc = [None] * 4
        for g in range(NG):
            r = [pltpu.bitcast(x_ref[_rows(g, G), _rows(4 * p + q, 128)], I32)
                 for q in range(4)]
            r = _skew([r[0]] + [pltpu.roll(r[q], q, 1) for q in range(1, 4)])
            for j in range(4):
                xp_ref[4 * p + j, _rows(g, 8), :] = r[j]
                x = _bf(r[j]).astype(F32)
                acc[j] = x[:8] + x[8:] if g % PIECE == 0 else acc[j] + (x[:8] + x[8:])
                if g % PIECE == PIECE - 1:
                    tally(p, j, 0, acc[j], g < PIECE)
            yield


def _norm_centre(xp_ref, cen_ref, stat_ref, tally):
    for lo in range(0, NG, PIECE2):
        for c in range(16):
            m, acc = stat_ref[16 + c], None
            for g in range(lo, lo + PIECE2):
                x = _bf(xp_ref[c, _rows(g, 8), :]).astype(F32)
                d = [x[:8] - m, x[8:] - m]
                sq = d[0] * d[0] + d[1] * d[1]
                acc = sq if g == lo else acc + sq
                cen_ref[c, _rows(g, 8), :] = jnp.concatenate(d, axis=1).astype(BF16)
            tally(c // 4, c % 4, 1, acc, lo == 0)
            yield


def _average(v):
    return jnp.broadcast_to(jnp.sum(v, axis=0, keepdims=True), v.shape) / D


def _norm_factor(squares, mean):
    shift = mean - _round_bf16(mean)
    var = _round_bf16(jnp.maximum(_average(squares) - shift * shift, 0.0))
    eps = _round_bf16(jnp.full_like(var, EPS))
    return 0.5 / _round_bf16(jnp.sqrt(_round_bf16(var + eps)))


def _norm_scale(wr_ref, cen_ref, stat_ref, work_ref):
    wr = jnp.broadcast_to(2.0 * wr_ref[...].astype(F32).reshape(1, D), (8, D))
    for p in range(4):
        cols = range(4 * p, 4 * p + 4)
        inv, score = {c: stat_ref[c] for c in cols}, {}
        for lo in range(0, NG, 8):
            for c in cols:
                vals = []
                for g in reversed(range(lo, min(lo + 8, NG))):
                    d = cen_ref[c, _rows(g, 8), :].astype(F32)
                    for t in (1, 0):
                        vals.insert(0, d[:, 128 * t:128 * t + 128] * inv[c])
                        work_ref[2 * g + t, XN + c] = vals[0]
                part = _mm(wr[:, G * lo:G * lo + 8 * len(vals)],
                           jnp.concatenate(vals, axis=0))
                score[c] = part if lo == 0 else score[c] + part
            yield
        for c in cols:
            stat_ref[c] = score[c]


def _route(stat_ref, work_ref, hot_ref, xs_ref, gate_ref):
    row = _iota((8, 128), 0)
    halves = []
    for lo in (0, 8):
        dense = stat_ref[lo]
        for c in range(1, 8):
            dense = jnp.where(row == c, stat_ref[lo + c], dense)
        halves.append(dense)
    score = _round_bf16(jnp.concatenate(halves, axis=0))
    blk = _iota((16, 128), 0)
    bits = pltpu.bitcast(jnp.where(score == 0.0, 0.0, score), I32) >> 16
    order = jnp.where(bits < 0, bits ^ 0x7FFF, bits) + 0x8000
    time = 512 * (blk >> 2) + _x_time(blk & 3, _iota((16, 128), 1))
    key = pltpu.bitcast((1 << 29) + (order << 11) + (L - 1 - time), F32)
    rank = jnp.full((16, 128), TOPK, I32)
    best = jnp.zeros((8, 128), F32)
    for i in range(TOPK):
        top = jnp.max(jnp.max(key, axis=0, keepdims=True), axis=1, keepdims=True)
        hit = key == top
        rank = jnp.where(hit, i, rank)
        key = jnp.where(hit, 0.0, key)
        best = jnp.where(row == i, top, best)
        yield
        yield
    order = ((pltpu.bitcast(best, I32) >> 11) & 0xFFFF) - 0x8000
    best = pltpu.bitcast(jnp.where(order < 0, order ^ 0x7FFF, order) << 16, F32)
    gate_ref[...] = 0.5 * _round_bf16(jax.nn.sigmoid(best))
    for c in range(16):
        hot_ref[c] = jnp.where(jnp.broadcast_to(rank[c:c + 1], (8, 128)) == row, 1.0, 0.0)
    for lo in range(0, D, 128):
        n, picked = min(128, D - lo), None
        for c in range(16):
            tokens = work_ref[pl.ds(lo // 8, n // 8), XN + c].reshape(n, 128)
            part = _mm(hot_ref[c], tokens, NT)
            picked = part if c == 0 else picked + part
            if c % 4 == 3:
                yield
        xs_ref[:, pl.ds(lo, n)] = 2.0 * picked
    yield
    yield


def _ffn_up(second, xs_ref, w_ref, h_ref):
    for col in range(0, F, 512):
        acc = None
        for lo in range(0, D, 128):
            rows = pl.ds(lo, min(128, D - lo))
            part = _mm(xs_ref[:, rows], w_ref[rows, pl.ds(col, 512)])
            acc = part if lo == 0 else acc + part
            yield
        acc = _round_bf16(acc)
        h_ref[:, pl.ds(col, 512)] = (
            h_ref[:, pl.ds(col, 512)] * acc if second else _round_bf16(_silu(acc)))


def _conv_step(i, same, live, later, kf_ref, fx_ref, fxt_ref, xf_ref, work_ref, s_ref):
    def products():
        for t in range(2):
            h = 2 * (i - 2) + t
            for k in range(4):
                kf = [(kf_ref[h, k, 2 * p], kf_ref[h, k, 2 * p + 1]) for p in range(4)]
                x = [(xf_ref[h, k, 2 * p], xf_ref[h, k, 2 * p + 1]) for p in range(4)]
                for c in (3, 0, 2, 1):
                    acc = _cmul(kf[0], x[c])
                    for p in range(1, c + 1):
                        acc = _cadd(acc, _cmul(kf[p], x[c - p]))
                    for part in range(2):
                        work_ref[2 * (same - 2) + t, 8 * c + 2 * k + part] = acc[part]
                    if c < 2:
                        yield

    fill = products() if live[2] else iter(())
    comp = [None] * 2

    def forward(part):
        lhs = [[] for _ in range(4)]
        for t in range(2):
            for p in range(4):
                for j in range(4):
                    lhs[j].append(work_ref[2 * i + t, XN + 4 * p + j])
                if p % 2:
                    next(fill, None)
        comp[part] = [_mm(jnp.concatenate(lhs[j], axis=0), _bf(fx_ref[j, part]))
                      for j in range(4)]

    def butterflies():
        for t in range(2):
            for p in range(4):
                r = slice(8 * (4 * t + p), 8 * (4 * t + p + 1))
                spec = _dft4([(comp[0][j][r], comp[1][j][r]) for j in range(4)], 1)
                for k in range(4):
                    for part in range(2):
                        xf_ref[2 * same + t, k, 2 * p + part] = spec[k][part]

    def inverse(odd):
        lhs = [[], []]
        for t in range(2):
            h = 2 * (i - 3) + t
            for c in range(4):
                v = [(work_ref[h, 8 * c + 2 * k], work_ref[h, 8 * c + 2 * k + 1])
                     for k in range(4)]
                if odd:
                    a, b = _csub(v[0], v[2]), _csub(v[1], v[3])
                    back = _csub_i(a, b), _cadd_i(a, b)
                else:
                    a, b = _cadd(v[0], v[2]), _cadd(v[1], v[3])
                    back = _cadd(a, b), _csub(a, b)
                for n in range(2):
                    lhs[n].append(jnp.concatenate(back[n], axis=1))
                if c % 2:
                    next(fill, None)
        y = [_mm(jnp.concatenate(lhs[n], axis=0), _bf(fxt_ref[odd + 2 * n]))
             for n in range(2)]
        for t in range(2):
            for c in range(4):
                for n in range(2):
                    s_ref[2 * (i - 3) + t, 4 * c + odd + 2 * n] = (
                        y[n][32 * t + 8 * c:32 * t + 8 * c + 8])

    for op in ORDER_C:
        if op in "01" and live[0]:
            forward(int(op))
        if op in "eo" and live[3]:
            inverse(int(op == "o"))
        while op == "b" and later:
            later.pop()()
        if op != "b":
            yield
    for _ in fill:
        pass
    if live[0]:
        later.append(butterflies)


def _ffn_down(lo, n, h_ref, wd_ref, gate_ref, upd_ref):
    ffn = None
    for k in range(0, F, 512):
        part = _mm(h_ref[:, pl.ds(k, 512)], wd_ref[pl.ds(lo, n), pl.ds(k, 512)], NT)
        ffn = part if ffn is None else ffn + part
        if k + 512 < F:
            yield
    upd_ref[pl.ds(lo, n), :] = (_round_bf16(ffn) * gate_ref[:, :n]).T


def _gate(lo, n, upd_ref, hot_ref, xp_ref, work_ref, s_ref, ds_ref, o_ref):
    for h0 in range(lo // 8, (lo + n) // 8, 8):
        nh = min(8, (lo + n) // 8 - h0)
        for p in range(4):
            scattered = [_mm(upd_ref[pl.ds(8 * h0, 8 * nh), :], hot_ref[4 * p + j])
                         for j in range(4)]
            for h in range(h0, h0 + nh):
                r = []
                for j in range(4):
                    x = _bf(xp_ref[4 * p + j, _rows(h // 2, 8), :]).astype(F32)
                    half = work_ref[h, XN + 4 * p + j]
                    s = s_ref[h, 4 * p + j] + half * ds_ref[_rows(h, 8), :]
                    half = half + scattered[j][8 * (h - h0):8 * (h - h0) + 8]
                    r.append(x[8 * (h % 2):8 * (h % 2) + 8]
                             + s * (half + half * jnp.tanh(half)))
                r = _skew(r)
                r = [r[0]] + [pltpu.roll(r[q], 128 - q, 1) for q in range(1, 4)]
                o_ref[_rows(h, 8), pl.ds(512 * p, 512)] = (
                    jnp.concatenate(r, axis=1).astype(BF16))
            yield


def _kernel(x_hbm, are_hbm, aim_hbm, bre_hbm, bim_hbm, cre_hbm, cim_hbm, ldt_hbm, dsk_hbm,
            wr_hbm, wg_hbm, wu_hbm, wd_hbm, o_hbm,
            x_ref, par_ref, ldt_ref, dsk_ref, wr_ref, wg_ref, wu_ref, wd_ref, o_ref,
            fx_ref, fxt_ref, fk_ref, fd_ref, dt_ref, ds_ref, base_ref, kv_ref, kr_ref, kf_ref,
            xp_ref, stat_ref, cen_ref, work_ref, xf_ref, s_ref,
            hot_ref, xs_ref, gate_ref, h_ref, upd_ref, sems):
    copies = []

    def fetch(src, dst, priority=0):
        cp = pltpu.make_async_copy(src, dst, sems.at[len(copies)])
        copies.append(cp)
        cp.start(priority=priority)
        return cp

    def fetch_params(rows):
        return [fetch(src.at[rows], par_ref.at[i, rows]) for i, src in
                enumerate((are_hbm, aim_hbm, bre_hbm, bim_hbm, cre_hbm, cim_hbm))]

    head = [fetch(ldt_hbm, ldt_ref)] + fetch_params(pl.ds(0, (RA + 2) * G))
    rest = fetch_params(pl.ds((RA + 2) * G, D - (RA + 2) * G)) + [fetch(dsk_hbm, dsk_ref)]
    x_copies = [fetch(x_hbm, x_ref), fetch(wr_hbm, wr_ref)]

    with jax.named_scope("setup"):
        _make_transforms(fx_ref, fxt_ref, fk_ref, fd_ref)
        for cp in head:
            cp.wait()
        ups = [fetch(wg_hbm, wg_ref), fetch(wu_hbm, wu_ref)]
        _column(ldt_ref, dt_ref, lambda v: _round_bf16(jnp.exp(v)))

    def wait_rest():
        for cp in rest:
            cp.wait()

    with jax.named_scope("ssm_kernel"):
        zero = _ssm_kernel(wait_rest, par_ref, dt_ref, base_ref, kv_ref, kr_ref)

    with jax.named_scope("layernorm"):
        for cp in x_copies:
            cp.wait()
        downs = [fetch(wd_hbm.at[pl.ds(*c)], wd_ref.at[pl.ds(*c)]) for c in DOWN_COPIES]

        def tally(p, j, n, value, first):
            kr_ref[p + zero, j, n] = value if first else kr_ref[p, j, n] + value

        def norm_pass(n, job, pieces, fine):
            @pl.when(zero < NG)
            def _():
                batches = 4 * SPLIT[n] // (1 if fine else BATCH[n])
                _weave(_ssm_spectrum(sum(SPLIT[:n]), SPLIT[n], BATCH[n], fine, kr_ref,
                                     fk_ref, fd_ref, kf_ref), job, pieces / (batches - 1))

        norm_pass(0, _norm_mean(x_ref, xp_ref, tally), 4 * NG, True)
        for c in range(16):
            stat_ref[c] = _average(kr_ref[c // 4, c % 4, 0])
            stat_ref[16 + c] = _round_bf16(stat_ref[c])
        norm_pass(1, _norm_centre(xp_ref, cen_ref, stat_ref, tally), 16 * NG // PIECE2, True)
        for c in range(16):
            stat_ref[c] = _norm_factor(kr_ref[c // 4, c % 4, 1], stat_ref[c])
        norm_pass(2, _norm_scale(wr_ref, cen_ref, stat_ref, work_ref), 20, False)

    with jax.named_scope("convolve"):
        def convolve(lo, hi):
            later = []
            for i in range(lo, hi):
                yield from _conv_step(i, i + zero, [0 <= i - k < NG for k in range(4)], later,
                                      kf_ref, fx_ref, fxt_ref, xf_ref, work_ref, s_ref)
            while later:
                later.pop()()

        ups[0].wait()
        _weave(convolve(0, CUTS[0]), itertools.chain(
            _route(stat_ref, work_ref, hot_ref, xs_ref, gate_ref),
            _ffn_up(False, xs_ref, wg_ref, h_ref)))
        ups[1].wait()
        _weave(convolve(CUTS[0], CUTS[1]), _ffn_up(True, xs_ref, wu_ref, h_ref))
        downs[0].wait()
        _column(dsk_ref, ds_ref, lambda v: 2.0 * v)
        _weave(convolve(CUTS[1], NG + 3),
               _ffn_down(*CHUNKS[0], h_ref, wd_ref, gate_ref, upd_ref))

    with jax.named_scope("finish"):
        outs = []
        for i, chunk in enumerate(CHUNKS):
            down = iter(())
            if i + 1 < len(CHUNKS):
                if i in WAITS:
                    downs[WAITS[i]].wait()
                down = _ffn_down(*CHUNKS[i + 1], h_ref, wd_ref, gate_ref, upd_ref)
            if i in SEND:
                outs.append(fetch(o_ref.at[pl.ds(*SEND[i])], o_hbm.at[pl.ds(*SEND[i])]))
            _weave(_gate(*chunk, upd_ref, hot_ref, xp_ref, work_ref, s_ref, ds_ref, o_ref),
                   down, DOWN_RATE)
        outs.append(fetch(o_ref.at[pl.ds(*chunk)], o_hbm.at[pl.ds(*chunk)]))
        for cp in outs:
            cp.wait()


@jax.jit
def pallas_recurrent_scan__ssm_conv_s4__moe_arch_mod__prompt_kernel(
    A_u: jax.Array,
    A_A_re: jax.Array,
    A_A_im: jax.Array,
    A_B_re: jax.Array,
    A_B_im: jax.Array,
    A_C_re: jax.Array,
    A_C_im: jax.Array,
    A_log_dt: jax.Array,
    A_Dskip: jax.Array,
    B_x: jax.Array,
    B_w_r: jax.Array,
    B_w_gate: jax.Array,
    B_w_up: jax.Array,
    B_w_down: jax.Array,
):
    del B_x
    assert A_u.shape == (1, L, D) and A_A_re.shape == (D, N) and B_w_gate.shape == (D, F)
    assert A_A_re.dtype == BF16
    vmem = pltpu.VMEM
    nh = 2 * NG
    scratch = [
        vmem((D, L), BF16), vmem((6, D, N), BF16),
        vmem((D,), BF16), vmem((D,), BF16), vmem((D,), BF16),
        vmem((D, F), BF16), vmem((D, F), BF16), vmem((D, F), BF16), vmem((D, L), BF16),
        vmem((4, 2, 64, 128), I32), vmem((4, 128, 128), I32),
        vmem((4, 2, 64, 128), I32), vmem((4, 2, 64, 128), I32),
        vmem((D, 128), F32), vmem((D, 128), F32),
        vmem((4, 2, 144, 128), F32), vmem((4, 192, 128), F32),
        vmem((nh + 4, 5, 2, 8, 128), F32), vmem((nh, 4, 8, 8, 128), F32),
        vmem((16, D // 2, 128), I32), vmem((32, 8, 128), F32),
        vmem((16, D // 2, 256), BF16),
        vmem((nh, XN + 16, 8, 128), F32), vmem((nh, 4, 8, 8, 128), F32),
        vmem((nh, 16, 8, 128), F32),
        vmem((16, 8, 128), F32), vmem((8, D), F32), vmem((8, 128), F32), vmem((8, F), F32),
        vmem((D, TOPK), F32),
        pltpu.SemaphoreType.DMA((18 + len(CHUNKS) + len(DOWN_COPIES),)),
    ]
    out = pl.pallas_call(
        _kernel,
        out_shape=jax.ShapeDtypeStruct((D, L), BF16),
        in_specs=[pl.BlockSpec(memory_space=pl.ANY)] * 13,
        out_specs=pl.BlockSpec(memory_space=pl.ANY),
        scratch_shapes=scratch,
        compiler_params=pltpu.CompilerParams(vmem_limit_bytes=100 * 1024 * 1024, flags=FLAGS),
    )(A_u[0].T, A_A_re, A_A_im, A_B_re, A_B_im, A_C_re, A_C_im, A_log_dt, A_Dskip,
      B_w_r, B_w_gate, B_w_up, B_w_down.T)
    return out.T[None]
```

```python
import itertools
import math

import jax
import jax.numpy as jnp
from jax import lax
import jax.experimental.pallas as pl
import jax.experimental.pallas.tpu as pltpu

F32, BF16, I32 = jnp.float32, jnp.bfloat16, jnp.int32
L, D, N, F, TOPK = 2048, 576, 128, 4608, 8
EPS = 1e-5
G = 16
NG = D // G
NH = D // 8
NN = (((1,), (0,)), ((), ()))
NT = (((1,), (1,)), ((), ()))

SSM_UNROLL = 6
NORM_SHARE = ((24, 2), (30, 3), (18, 3))
MEAN_GROUPS, VAR_GROUPS = 3, 6
CONV_CUTS = (22, 34)
CHUNKS = ((0, 128), (128, 128), (256, 128), (384, 128), (512, 64))
DOWN_COPIES = ((0, 256), (256, 272), (528, 48))
DOWN_WAITS = {1: 1, 3: 2}


def _iota(shape, dim):
    return lax.broadcasted_iota(I32, shape, dim)


def _rows(i, n):
    return pl.ds(i * n if isinstance(i, int) else pl.multiple_of(i * n, n), n)


def _cat(xs, axis=0):
    return jnp.concatenate(xs, axis=axis)


def _cmul(a, b):
    return a[0] * b[0] - a[1] * b[1], a[0] * b[1] + a[1] * b[0]


def _csq(a):
    return a[0] * a[0] - a[1] * a[1], (a[0] + a[0]) * a[1]


def _cadd(a, b):
    return a[0] + b[0], a[1] + b[1]


def _csub(a, b):
    return a[0] - b[0], a[1] - b[1]


def _cadd_i(a, b):
    return a[0] - b[1], a[1] + b[0]


def _csub_i(a, b):
    return a[0] + b[1], a[1] - b[0]


def _dft4(v):
    s02, d02 = _cadd(v[0], v[2]), _csub(v[0], v[2])
    s13, d13 = _cadd(v[1], v[3]), _csub(v[1], v[3])
    return [_cadd(s02, s13), _cadd_i(d02, d13), _csub(s02, s13), _csub_i(d02, d13)]


def _root(n):
    ang = (((n + 1024) & 2047) - 1024).astype(F32) * (2.0 * math.pi / 2048)
    return jnp.cos(ang), jnp.sin(ang)


def _powers(start, step, count):
    vals = [start]
    for _ in range(count - 1):
        vals.append(_cmul(vals[-1], step))
    return vals


def _pack(x):
    return pltpu.bitcast(x.astype(BF16), I32)


def _bf(x):
    return pltpu.bitcast(x, BF16)


def _round_bf16(x):
    return x.astype(BF16).astype(F32)


def _silu_of_twice(h):
    return h + h * jnp.tanh(h)


def _mm(a, b, dims=NN):
    return lax.dot_general(a, b, dims, precision=lax.Precision.DEFAULT,
                           preferred_element_type=F32)


def _skew(r):
    lane = _iota(r[0].shape, 1)
    b0, b1 = (lane & 1) != 0, (lane & 2) != 0
    t = [lax.select(b0, r[(k + 1) % 4], r[k]) for k in range(4)]
    u = [lax.select(b1, t[(k + 2) % 4], t[k]) for k in range(4)]
    return [u[(-j) % 4] for j in range(4)]


def _x_time(j, m):
    q = (m - j) & 3
    return 128 * q + ((m - q) & 127)


def _weave(main, side, rate=1.0):
    credit = 0.0
    for _ in main:
        credit += rate
        while credit >= 1.0:
            credit -= 1.0
            next(side, None)
    for _ in side:
        pass


def _column(v_ref, out_ref, fn):
    v = fn(v_ref[...].astype(F32).reshape(1, D))
    for lo in range(0, D, 128):
        n = min(128, D - lo)
        out_ref[pl.ds(lo, n), :] = jnp.broadcast_to(v[:, lo:lo + n], (128, n)).T


def _input_transform(fx_ref, fxt_ref):
    freq, row = 4 * _iota((8, 128), 1) + 1, _iota((8, 128), 0)
    step8 = _root(8 * freq)
    step128 = _csq(_csq(_csq(_csq(step8))))
    for j in range(4):
        start = _root((_x_time(j, row + 8) - 8) * freq)
        vals = _powers(start, step8, 16)
        wraps = row < ((row - j) & 3)
        vals[0] = tuple(jnp.where(wraps, a, b) for a, b in zip(_cmul(start, step128), start))
        for part in range(2):
            m = _cat([v[part] for v in vals])
            fx_ref[j, part] = _pack(m)
            fxt_ref[j, pl.ds(64 * part, 64), :] = _pack(m.T)


def _kernel_transform(fk_ref, fd_ref):
    freq, row = 4 * _iota((8, 128), 1) + 1, _iota((8, 128), 0)
    rho = _root(freq)
    step32 = _csq(_csq(_csq(_csq(_csq(rho)))))
    for j, start in enumerate(_powers(_root(4 * row * freq), rho, 4)):
        vals = _powers(start, step32, 16)
        for part in range(2):
            fk_ref[j, part] = _pack(_cat([v[part] for v in vals]))
    rows = _powers(_root((256 * (row & 1) + 8 * (row >> 1)) * freq), step32, 8)
    first = row == 0
    for k in range(4):
        p2 = _csq(rho)
        s3 = _cadd(_cadd(rho, p2), _cmul(p2, rho))
        s4 = _cadd(s3, _csq(p2))
        box = 1.0 + 2.0 * jnp.where((row & 2) == 0, s4[0], s3[0])
        vals = [(r[0] * box, r[1] * box) for r in rows]
        vals[0] = (jnp.where(first, 1.0 + s4[0], vals[0][0]),
                   jnp.where(first, s4[1], vals[0][1]))
        vals.append((jnp.where(first, s4[1], 0.0), jnp.where(first, s4[0], 0.0)))
        for part in range(2):
            fd_ref[k, part, pl.ds(0, 40), :] = _pack(
                _cat([v[part] for v in vals] + [jnp.zeros((8, 128), F32)]))
            fd_ref[k, part, pl.ds(40, 24), :] = jnp.zeros((24, 128), I32)
        rho = (-rho[1], rho[0])


def _ssm_bases(g, h, par_ref, dt_ref, base_ref):
    a_re, a_im, b_re, b_im, c_re, c_im = (
        par_ref[k, _rows(g, G), :].astype(F32) for k in range(6))
    dt = dt_ref[_rows(g, G), :]
    dts = dt * (2.0 / 512)
    row = _iota((8, 128), 0)

    def deal(v):
        return _cat([jnp.take_along_axis(v[lo:lo + 8], (row >> 1) + 4 * (row & 1), axis=0,
                                         mode="promise_in_bounds") for lo in (0, 8)])

    decay, phase = deal(dt * a_re), deal(dt * a_im)
    w = tuple(deal(v) for v in _cmul((c_re, c_im), (dts * b_re, dts * b_im)))
    z, unit = {}, (jnp.cos(phase), jnp.sin(phase))
    for e in (1, 2, 4, 8, 16, 32, 64, 128, 256):
        if e in (1, 4, 8, 16, 256):
            mag = jnp.exp2(decay * (e * math.log2(math.e)))
            z[e] = (mag * unit[0], mag * unit[1])
        if e < 256:
            unit = _csq(unit)
    z1024 = _csq(_csq(z[256]))
    w8, w1024 = _cmul(w, z[8]), _cmul(w, z1024)
    seq = [(jnp.ones_like(dt), jnp.zeros_like(dt)), z[8], z[16], z[16], _cmul(z[16], z[8]),
           z[1], z[1], z[256], z[256], w, _cmul(w, z[4]), w,
           w8, w1024, w8, w1024, _cmul(w1024, z1024), w1024]
    for k, v in enumerate(seq):
        for t in range(2):
            for part in range(2):
                base_ref[h + t, part, pl.ds(8 * k, 8), :] = v[part][8 * t:8 * t + 8]


_OFFSETS = ((0, 4), (1, 5), (2, 6), (3, 7), (258, 262), (256, 260), (512, 516), (768, 772),
            (264, 1280), (520, 1536), (776, 1792), (1024, 2048))


def _ssm_values(h, base_ref, kv_ref):
    for quad in range(2):
        def pair(k):
            return tuple(base_ref[h, part, pl.ds(8 * k + quad, 8, stride=2), :]
                         for part in range(2))

        v = [pair(0)] + _powers(pair(3), pair(2), 15)
        z256 = pair(7)
        w = _powers(pair(9 + quad), pair(5), 4)
        w += [_cmul(w[2], z256)] + _powers(w[0], z256, 4)[1:]
        w += _powers(pair(12 + quad), z256, 4)[1:] + [pair(15 + quad)]
        re, im = (_mm(_cat([t[part] for t in w]), _cat([t[part] for t in v[::-1]]), NT)
                  for part in range(2))
        kv_ref[h, quad] = re - im


def _ssm_arrange(h, slot, kv_ref, kr_ref):
    lane, row = _iota((8, 128), 1), _iota((8, 128), 0)
    src = 4 * (((lane >> 1) & 31) ^ 30) + (row & 3)
    top = row < 4

    def spread(x):
        return jnp.take_along_axis(x, src, axis=1, mode="promise_in_bounds")

    def even(a, b):
        return jnp.where((lane & 1) == 0, a, b)

    def low(a, b):
        return jnp.where(lane < 64, a, b)

    val = {}
    for u, (e0, e1) in enumerate(_OFFSETS):
        a, b = (kv_ref[h, quad, pl.ds(8 * u, 8), :] for quad in range(2))
        val[e0] = spread(jnp.where(top, a, b))
        val[e1] = spread(pltpu.roll(jnp.where(top, b, a), 4, 0))
    mid = even(val[256], val[260])
    q0, q4, q8 = low(val[512], val[768]), low(val[516], val[772]), low(val[520], val[776])
    blocks = [
        (low(even(val[0], val[4]), mid), even(q0, q4)),
        (low(even(val[1], val[5]), mid), even(q0, q4)),
        (low(even(val[2], val[6]), even(val[258], val[262])), even(q0, q8)),
        (low(even(val[3], val[7]), even(val[260], val[264])), even(q4, q8)),
        (low(even(val[1024], val[1280]), val[1536]),
         low(even(val[1536], val[1792]), jnp.where(lane == 64, val[2048], 0.0)))]
    for j, pair in enumerate(blocks):
        kr_ref[slot, j] = _cat(pair)


def _ssm_kernel(wait_rest, par_ref, dt_ref, base_ref, kv_ref, kr_ref):
    def body(n, zero):
        pl.when(n == 1)(wait_rest)
        for r in range(SSM_UNROLL):
            g, slot = n * SSM_UNROLL + r, 2 * (r % 2)
            for t in range(2):
                _ssm_arrange(slot + t, 2 * g + t, kv_ref, kr_ref)
                _ssm_values(slot + t, base_ref, kv_ref)
            ahead = g + 2 if r + 2 < SSM_UNROLL else jnp.minimum(g + 2, NG - 1)
            _ssm_bases(ahead, slot, par_ref, dt_ref, base_ref)
        return jnp.minimum(zero, n * L)

    for g in range(2):
        _ssm_bases(g, 2 * g, par_ref, dt_ref, base_ref)
    kv_ref[...] = jnp.zeros_like(kv_ref)
    zero = lax.fori_loop(0, NG // SSM_UNROLL, body, L)
    for h in range(4):
        _ssm_arrange(h, NH + h, kv_ref, kr_ref)
    return zero


def _ssm_spectrum(first, count, batch, fine, kr_ref, fk_ref, fd_ref, kf_ref):
    def blocks(x):
        x = x.reshape(batch, 2, 1, 8, 128)
        return x[:, :1], x[:, 1:]

    for h0 in range(first, first + count, batch):
        near, far = [], []
        for n in range(4):
            lhs = {j: [] for j in ((0, 1, 2, 3) if n < 2 else (4,))}
            for h in range(h0, h0 + batch):
                for j, rows in lhs.items():
                    rows.append(kr_ref[4 + h, j])
                if fine:
                    yield
            if n < 2:
                near.append([_mm(_cat(lhs[j]), _bf(fk_ref[j, n])) for j in range(4)])
            else:
                far += [[_mm(_cat(lhs[4]), _bf(fd_ref[k, part])) for part in range(2)]
                        for k in (2 * n - 4, 2 * n - 3)]
            if not fine:
                yield
        out = []
        for a, b in zip(_dft4(list(zip(*near))), far):
            spec = list(zip(*(blocks(a[part]) + blocks(b[part]) for part in range(2))))
            spec = spec[:1] + [_csub_i(spec[p], spec[p - 1]) for p in range(1, 4)]
            out += [_cat(v, 1) for v in zip(*spec)]
        kf_ref[pl.ds(4 * h0, 4 * batch)] = _cat(out, 2).reshape(4 * batch, 8, 8, 128)


XN = 8


def _fold(x):
    x = x.reshape(3, -1, 8, 128)
    x = x[0] + x[1] + x[2]
    while x.shape[0] > 1:
        x = x[:x.shape[0] // 2] + x[x.shape[0] // 2:]
    return x[0]


def _norm_mean(x_ref, xp_ref, tally):
    for p in range(4):
        for i in range(NG // MEAN_GROUPS):
            r = [pltpu.bitcast(x_ref[_rows(i, MEAN_GROUPS * G), _rows(4 * p + q, 128)], I32)
                 for q in range(4)]
            r = _skew([r[0]] + [pltpu.roll(r[q], q, 1) for q in range(1, 4)])
            for j in range(4):
                xp_ref[p, j, _rows(i, MEAN_GROUPS * 8), :] = r[j]
                tally(p, j, 0, _fold(_bf(r[j]).astype(F32)), i == 0)
            yield


def _norm_centre(xp_ref, cen_ref, stat_ref, tally):
    for i in range(NG // VAR_GROUPS):
        for p, j in itertools.product(range(4), range(4)):
            x = _bf(xp_ref[p, j, _rows(i, VAR_GROUPS * 8), :]).astype(F32)
            d = x.reshape(VAR_GROUPS, G, 128) - _cat([stat_ref[1, p, j]] * 2)
            cen_ref[p, j, _rows(i, VAR_GROUPS)] = _cat([d[:, :8], d[:, 8:]], 2).astype(BF16)
            tally(p, j, 1, _fold(d * d), i == 0)
            yield


def _average(v):
    return jnp.broadcast_to(jnp.sum(v, axis=0, keepdims=True), v.shape) / D


def _norm_factor(squares, mean):
    shift = mean - _round_bf16(mean)
    var = _round_bf16(jnp.maximum(_average(squares) - shift * shift, 0.0))
    eps = _round_bf16(jnp.full_like(var, EPS))
    return 0.5 / _round_bf16(jnp.sqrt(_round_bf16(var + eps)))


def _norm_scale(wr_ref, cen_ref, stat_ref, work_ref):
    wr = jnp.broadcast_to(2.0 * wr_ref[...].astype(F32).reshape(1, D), (8, D))
    for p in range(4):
        score = [None] * 4
        for lo in range(0, D, 128):
            n = min(128, D - lo)
            for j in range(4):
                d = cen_ref[p, j, pl.ds(lo // G, n // G)].astype(F32)
                half = _cat([d[:, :, :128], d[:, :, 128:]], 1).reshape(n // 8, 8, 128)
                half = half * stat_ref[0, p, j]
                work_ref[pl.ds(lo // 8, n // 8), p, XN + j] = half
                part = _mm(wr[:, lo:lo + n], half.reshape(n, 128))
                score[j] = part if lo == 0 else score[j] + part
            yield
        for j in range(4):
            stat_ref[1, p, j] = score[j]


def _route(stat_ref, work_ref, hot_ref, xs_ref, gate_ref):
    row, blk = _iota((8, 128), 0), _iota((16, 128), 0)
    halves = []
    for lo in (0, 2):
        dense = stat_ref[1, lo, 0]
        for c in range(1, 8):
            dense = jnp.where(row == c, stat_ref[1, lo + c // 4, c % 4], dense)
        halves.append(dense)
    score = _round_bf16(_cat(halves))
    bits = pltpu.bitcast(jnp.where(score == 0.0, 0.0, score), I32) >> 16
    order = jnp.where(bits < 0, bits ^ 0x7FFF, bits) + 0x8000
    time = 512 * (blk >> 2) + _x_time(blk & 3, _iota((16, 128), 1))
    key = pltpu.bitcast((1 << 29) + (order << 11) + (L - 1 - time), F32)
    rank = jnp.full((16, 128), TOPK, I32)
    best = jnp.zeros((8, 128), F32)
    for i in range(TOPK):
        top = jnp.max(jnp.max(key, axis=0, keepdims=True), axis=1, keepdims=True)
        hit = key == top
        rank = jnp.where(hit, i, rank)
        key = jnp.where(hit, 0.0, key)
        best = jnp.where(row == i, top, best)
        yield from range(2)
    order = ((pltpu.bitcast(best, I32) >> 11) & 0xFFFF) - 0x8000
    best = pltpu.bitcast(jnp.where(order < 0, order ^ 0x7FFF, order) << 16, F32)
    gate_ref[...] = 0.5 * _round_bf16(jax.nn.sigmoid(best))
    for c in range(16):
        hot_ref[c] = jnp.where(jnp.broadcast_to(rank[c:c + 1], (8, 128)) == row, 1.0, 0.0)
    for lo in range(0, D, 128):
        n, picked = min(128, D - lo), None
        for p in range(4):
            for j in range(4):
                tokens = work_ref[pl.ds(lo // 8, n // 8), p, XN + j]
                part = _mm(hot_ref[4 * p + j], tokens.reshape(n, 128), NT)
                picked = part if picked is None else picked + part
            yield
        xs_ref[:, pl.ds(lo, n)] = 2.0 * picked
    yield from range(2)


def _ffn_up(second, xs_ref, w_ref, h_ref):
    for col in range(0, F, 512):
        acc = None
        for lo in range(0, D, 128):
            rows = pl.ds(lo, min(128, D - lo))
            part = _mm(xs_ref[:, rows], w_ref[rows, pl.ds(col, 512)])
            acc = part if lo == 0 else acc + part
            yield
        acc = _round_bf16(acc)
        h_ref[:, pl.ds(col, 512)] = (h_ref[:, pl.ds(col, 512)] * acc if second
                                     else _round_bf16(_silu_of_twice(0.5 * acc)))


def _ffn_down(lo, n, h_ref, wd_ref, gate_ref, upd_ref):
    ffn = None
    for k in range(0, F, 512):
        part = _mm(h_ref[:, pl.ds(k, 512)], wd_ref[pl.ds(lo, n), pl.ds(k, 512)], NT)
        ffn = part if ffn is None else ffn + part
        if k + 512 < F:
            yield
    upd_ref[pl.ds(lo, n), :] = (_round_bf16(ffn) * gate_ref[:, :n]).T


def _convolve(start, stop, zero, kf_ref, fx_ref, fxt_ref, xf_ref, work_ref, y_ref):
    def products(g):
        for h, k in itertools.product((2 * g, 2 * g + 1), range(4)):
            kf, x = ([tuple(ref[4 * h + p, 2 * k + part] for part in range(2))
                      for p in range(4)] for ref in (kf_ref, xf_ref))
            for c in (3, 0, 2, 1):
                acc = _cmul(kf[0], x[c])
                for p in range(1, c + 1):
                    acc = _cadd(acc, _cmul(kf[p], x[c - p]))
                for part in range(2):
                    work_ref[h + zero, c, 2 * k + part] = acc[part]
                if c < 2:
                    yield

    def operands(g, slots, fill):
        rows = []
        for h, p in itertools.product((2 * g, 2 * g + 1), range(4)):
            rows.append(work_ref[h, pl.ds(p, 1), slots])
            if p % 2:
                next(fill, None)
        rows = _cat(rows)
        return [rows[:, s].reshape(64, 128) for s in range(slots.size)]

    def butterflies(g, comp):
        spec = [v.reshape(8, 1, 8, 128) for pair in _dft4(list(zip(*comp))) for v in pair]
        xf_ref[pl.ds(8 * g + zero, 8)] = _cat(spec, 1)

    pending = None
    for i in range(start, stop):
        fill = products(i - 2) if 0 <= i - 2 < NG else iter(())
        for odd in range(2):
            if 0 <= i - 3:
                v = operands(i - 3, pl.ds(0, XN), fill)
                v = list(zip(v[0::2], v[1::2]))
                if odd:
                    a, b = _csub(v[0], v[2]), _csub(v[1], v[3])
                    back = _csub_i(a, b), _cadd_i(a, b)
                else:
                    a, b = _cadd(v[0], v[2]), _cadd(v[1], v[3])
                    back = _cadd(a, b), _csub(a, b)
                for j, spec in zip((odd, odd + 2), back):
                    y = _mm(_cat(spec, 1), _bf(fxt_ref[j]))
                    y_ref[_rows(i - 3, 2), :, j] = y.reshape(2, 4, 8, 128)
            yield
        if pending:
            butterflies(*pending)
        pending = (i, []) if i < NG else None
        for part in range(2):
            if pending:
                x = operands(i, pl.ds(XN, 4), fill)
                pending[1].append([_mm(x[j], _bf(fx_ref[j, part])) for j in range(4)])
            yield
        for _ in fill:
            pass
    if pending:
        butterflies(*pending)


def _gate(lo, n, upd_ref, hot_ref, xp_ref, work_ref, y_ref, skip_ref, o_ref):
    for i in range(lo // 64, (lo + n) // 64):
        for p in range(4):
            r = []
            for j in range(4):
                x = _bf(xp_ref[p, j, _rows(i, 32), :]).astype(F32)
                half = work_ref[_rows(i, 8), p, XN + j].reshape(64, 128)
                s = (y_ref[_rows(i, 8), p, j].reshape(64, 128)
                     + half * skip_ref[_rows(i, 64), :])
                routed = _mm(upd_ref[_rows(i, 64), :], hot_ref[4 * p + j])
                r.append(x + s * _silu_of_twice(half + routed))
            r = _skew(r)
            r = [r[0]] + [pltpu.roll(r[q], 128 - q, 1) for q in range(1, 4)]
            o_ref[_rows(i, 64), _rows(p, 512)] = _cat(r, 1).astype(BF16)
            yield


def _kernel(x_hbm, are_hbm, aim_hbm, bre_hbm, bim_hbm, cre_hbm, cim_hbm, ldt_hbm, dsk_hbm,
            wr_hbm, wg_hbm, wu_hbm, wd_hbm, o_hbm,
            x_ref, par_ref, ldt_ref, dsk_ref, wr_ref, wg_ref, wu_ref, wd_ref, o_ref,
            fx_ref, fxt_ref, fk_ref, fd_ref, dt_ref, skip_ref, base_ref, kv_ref, kr_ref,
            kf_ref, xp_ref, stat_ref, cen_ref, work_ref, xf_ref, y_ref,
            hot_ref, xs_ref, gate_ref, h_ref, upd_ref, sems):
    copies = []

    def fetch(src, dst):
        copies.append(pltpu.make_async_copy(src, dst, sems.at[len(copies)]))
        copies[-1].start()
        return copies[-1]

    def fetch_params(rows):
        return [fetch(src.at[rows], par_ref.at[i, rows]) for i, src in
                enumerate((are_hbm, aim_hbm, bre_hbm, bim_hbm, cre_hbm, cim_hbm))]

    def wait(pending):
        for cp in pending:
            cp.wait()

    early = (SSM_UNROLL + 2) * G
    head = [fetch(ldt_hbm, ldt_ref)] + fetch_params(pl.ds(0, early))
    rest = fetch_params(pl.ds(early, D - early))
    inputs = [fetch(x_hbm, x_ref), fetch(wr_hbm, wr_ref), fetch(dsk_hbm, dsk_ref)]
    _kernel_transform(fk_ref, fd_ref)
    _input_transform(fx_ref, fxt_ref)
    wait(head)
    ups = [fetch(wg_hbm, wg_ref), fetch(wu_hbm, wu_ref)]
    downs = [fetch(wd_hbm.at[pl.ds(*c)], wd_ref.at[pl.ds(*c)]) for c in DOWN_COPIES]
    _column(ldt_ref, dt_ref, lambda v: _round_bf16(jnp.exp(v)))
    zero = _ssm_kernel(lambda: wait(rest), par_ref, dt_ref, base_ref, kv_ref, kr_ref)

    def tally(p, j, n, value, first):
        kr_ref[p + zero, j, _rows(n, 8), :] = (
            value if first else kr_ref[p, j, _rows(n, 8), :] + value)

    def norm_pass(n, job, pieces, fine):
        count, batch = NORM_SHARE[n]
        first = sum(share[0] for share in NORM_SHARE[:n])

        @pl.when(zero < NG)
        def _():
            _weave(_ssm_spectrum(first, count, batch, fine, kr_ref, fk_ref, fd_ref, kf_ref),
                   job, pieces / (4 * count // (1 if fine else batch) - 1))

    wait(inputs)
    norm_pass(0, _norm_mean(x_ref, xp_ref, tally), 4 * NG // MEAN_GROUPS, True)
    for p, j in itertools.product(range(4), range(4)):
        stat_ref[0, p, j] = _average(kr_ref[p, j, _rows(0, 8), :])
        stat_ref[1, p, j] = _round_bf16(stat_ref[0, p, j])
    norm_pass(1, _norm_centre(xp_ref, cen_ref, stat_ref, tally), 16 * NG // VAR_GROUPS, True)
    for p, j in itertools.product(range(4), range(4)):
        stat_ref[0, p, j] = _norm_factor(kr_ref[p, j, _rows(1, 8), :], stat_ref[0, p, j])
    norm_pass(2, _norm_scale(wr_ref, cen_ref, stat_ref, work_ref), 20, False)

    def convolve(start, stop):
        return _convolve(start, stop, zero, kf_ref, fx_ref, fxt_ref, xf_ref, work_ref, y_ref)

    def ffn_down(i):
        return _ffn_down(*CHUNKS[i], h_ref, wd_ref, gate_ref, upd_ref)

    ups[0].wait()
    _weave(convolve(0, CONV_CUTS[0]), itertools.chain(
        _route(stat_ref, work_ref, hot_ref, xs_ref, gate_ref),
        _ffn_up(False, xs_ref, wg_ref, h_ref)))
    ups[1].wait()
    _weave(convolve(*CONV_CUTS), _ffn_up(True, xs_ref, wu_ref, h_ref))
    downs[0].wait()
    _column(dsk_ref, skip_ref, lambda v: 2.0 * v)
    _weave(convolve(CONV_CUTS[1], NG + 3), ffn_down(0))

    outs = []
    for i, chunk in enumerate(CHUNKS):
        _weave(_gate(*chunk, upd_ref, hot_ref, xp_ref, work_ref, y_ref, skip_ref, o_ref),
               ffn_down(i + 1) if i + 1 < len(CHUNKS) else iter(()), 1.8)
        if i + 1 in DOWN_WAITS:
            downs[DOWN_WAITS[i + 1]].wait()
        outs.append(fetch(o_ref.at[pl.ds(*chunk)], o_hbm.at[pl.ds(*chunk)]))
    wait(outs)


@jax.jit
def pallas_recurrent_scan__ssm_conv_s4__moe_arch_mod__prompt_kernel(
    A_u: jax.Array,
    A_A_re: jax.Array,
    A_A_im: jax.Array,
    A_B_re: jax.Array,
    A_B_im: jax.Array,
    A_C_re: jax.Array,
    A_C_im: jax.Array,
    A_log_dt: jax.Array,
    A_Dskip: jax.Array,
    B_x: jax.Array,
    B_w_r: jax.Array,
    B_w_gate: jax.Array,
    B_w_up: jax.Array,
    B_w_down: jax.Array,
):
    del B_x
    assert A_u.shape == (1, L, D) and A_A_re.shape == (D, N) and B_w_gate.shape == (D, F)
    assert A_A_re.dtype == BF16
    vmem = pltpu.VMEM
    scratch = [
        vmem((D, L), BF16), vmem((6, D, N), BF16),
        vmem((D,), BF16), vmem((D,), BF16), vmem((D,), BF16),
        vmem((D, F), BF16), vmem((D, F), BF16), vmem((D, F), BF16), vmem((D, L), BF16),
        vmem((4, 2, 64, 128), I32), vmem((4, 128, 128), I32),
        vmem((4, 2, 64, 128), I32), vmem((4, 2, 64, 128), I32),
        vmem((D, 128), F32), vmem((D, 128), F32),
        vmem((4, 2, 144, 128), F32), vmem((4, 2, 96, 128), F32),
        vmem((NH + 4, 5, 16, 128), F32), vmem((4 * NH, 8, 8, 128), F32),
        vmem((4, 4, D // 2, 128), I32), vmem((2, 4, 4, 8, 128), F32),
        vmem((4, 4, NG, 8, 256), BF16),
        vmem((NH, 4, XN + 4, 8, 128), F32), vmem((4 * NH, 8, 8, 128), F32),
        vmem((NH, 4, 4, 8, 128), F32),
        vmem((16, 8, 128), F32), vmem((8, D), F32), vmem((8, 128), F32), vmem((8, F), F32),
        vmem((D, TOPK), F32),
        pltpu.SemaphoreType.DMA((18 + len(DOWN_COPIES) + len(CHUNKS),)),
    ]
    out = pl.pallas_call(
        _kernel,
        out_shape=jax.ShapeDtypeStruct((D, L), BF16),
        in_specs=[pl.BlockSpec(memory_space=pl.ANY)] * 13,
        out_specs=pl.BlockSpec(memory_space=pl.ANY),
        scratch_shapes=scratch,
        compiler_params=pltpu.CompilerParams(vmem_limit_bytes=100 * 1024 * 1024),
    )(A_u[0].T, A_A_re, A_A_im, A_B_re, A_B_im, A_C_re, A_C_im, A_log_dt, A_Dskip,
      B_w_r, B_w_gate, B_w_up, B_w_down.T)
    return out.T[None]
```

```python
import itertools
import math

import jax
import jax.numpy as jnp
from jax import lax
import jax.experimental.pallas as pl
import jax.experimental.pallas.tpu as pltpu

F32, BF16, I32 = jnp.float32, jnp.bfloat16, jnp.int32
L, D, N, F, TOPK = 2048, 576, 128, 4608, 8
EPS = 1e-5
G = 16
NG = D // G
NH = D // 8
NN = (((1,), (0,)), ((), ()))
NT = (((1,), (1,)), ((), ()))

SSM_UNROLL = 6
NORM_SHARE = ((24, 2), (30, 3), (18, 3))
MEAN_GROUPS, VAR_GROUPS = 3, 6
CONV_CUTS = (22, 34)
CHUNKS = ((0, 128), (128, 128), (256, 128), (384, 128), (512, 64))
DOWN_COPIES = ((0, 256), (256, 272), (528, 48))
DOWN_WAITS = {1: 1, 3: 2}


def _iota(shape, dim):
    return lax.broadcasted_iota(I32, shape, dim)


def _rows(i, n):
    return pl.ds(i * n if isinstance(i, int) else pl.multiple_of(i * n, n), n)


def _cat(xs, axis=0):
    return jnp.concatenate(xs, axis=axis)


def _cmul(a, b):
    return a[0] * b[0] - a[1] * b[1], a[0] * b[1] + a[1] * b[0]


def _csq(a):
    return a[0] * a[0] - a[1] * a[1], (a[0] + a[0]) * a[1]


def _cadd(a, b):
    return a[0] + b[0], a[1] + b[1]


def _csub(a, b):
    return a[0] - b[0], a[1] - b[1]


def _cadd_i(a, b):
    return a[0] - b[1], a[1] + b[0]


def _csub_i(a, b):
    return a[0] + b[1], a[1] - b[0]


def _dft4(v):
    s02, d02 = _cadd(v[0], v[2]), _csub(v[0], v[2])
    s13, d13 = _cadd(v[1], v[3]), _csub(v[1], v[3])
    return [_cadd(s02, s13), _cadd_i(d02, d13), _csub(s02, s13), _csub_i(d02, d13)]


def _root(n):
    ang = (((n + 1024) & 2047) - 1024).astype(F32) * (2.0 * math.pi / 2048)
    return jnp.cos(ang), jnp.sin(ang)


def _powers(start, step, count):
    vals = [start]
    for _ in range(count - 1):
        vals.append(_cmul(vals[-1], step))
    return vals


def _pack(x):
    return pltpu.bitcast(x.astype(BF16), I32)


def _bf(x):
    return pltpu.bitcast(x, BF16)


def _round_bf16(x):
    return x.astype(BF16).astype(F32)


def _silu_of_twice(h):
    return h + h * jnp.tanh(h)


def _mm(a, b, dims=NN):
    return lax.dot_general(a, b, dims, precision=lax.Precision.DEFAULT,
                           preferred_element_type=F32)


def _skew(r):
    lane = _iota(r[0].shape, 1)
    b0, b1 = (lane & 1) != 0, (lane & 2) != 0
    t = [lax.select(b0, r[(k + 1) % 4], r[k]) for k in range(4)]
    u = [lax.select(b1, t[(k + 2) % 4], t[k]) for k in range(4)]
    return [u[(-j) % 4] for j in range(4)]


def _x_time(j, m):
    q = (m - j) & 3
    return 128 * q + ((m - q) & 127)


def _weave(main, side, rate=1.0):
    credit = 0.0
    for _ in main:
        credit += rate
        while credit >= 1.0:
            credit -= 1.0
            next(side, None)
    for _ in side:
        pass


def _column(v_ref, out_ref, fn):
    v = fn(v_ref[...].astype(F32).reshape(1, D))
    for lo in range(0, D, 128):
        n = min(128, D - lo)
        out_ref[pl.ds(lo, n), :] = jnp.broadcast_to(v[:, lo:lo + n], (128, n)).T


def _input_transform(fx_ref, fxt_ref):
    freq, row = 4 * _iota((8, 128), 1) + 1, _iota((8, 128), 0)
    step8 = _root(8 * freq)
    step128 = _csq(_csq(_csq(_csq(step8))))
    for j in range(4):
        start = _root((_x_time(j, row + 8) - 8) * freq)
        vals = _powers(start, step8, 16)
        wraps = row < ((row - j) & 3)
        vals[0] = tuple(jnp.where(wraps, a, b) for a, b in zip(_cmul(start, step128), start))
        for part in range(2):
            m = _cat([v[part] for v in vals])
            fx_ref[j, part] = _pack(m)
            fxt_ref[j, pl.ds(64 * part, 64), :] = _pack(m.T)


def _kernel_transform(fk_ref, fd_ref):
    freq, row = 4 * _iota((8, 128), 1) + 1, _iota((8, 128), 0)
    rho = _root(freq)
    step32 = _csq(_csq(_csq(_csq(_csq(rho)))))
    for j, start in enumerate(_powers(_root(4 * row * freq), rho, 4)):
        vals = _powers(start, step32, 16)
        for part in range(2):
            fk_ref[j, part] = _pack(_cat([v[part] for v in vals]))
    rows = _powers(_root((256 * (row & 1) + 8 * (row >> 1)) * freq), step32, 8)
    first = row == 0
    for k in range(4):
        p2 = _csq(rho)
        s3 = _cadd(_cadd(rho, p2), _cmul(p2, rho))
        s4 = _cadd(s3, _csq(p2))
        box = 1.0 + 2.0 * jnp.where((row & 2) == 0, s4[0], s3[0])
        vals = [(r[0] * box, r[1] * box) for r in rows]
        vals[0] = (jnp.where(first, 1.0 + s4[0], vals[0][0]),
                   jnp.where(first, s4[1], vals[0][1]))
        vals.append((jnp.where(first, s4[1], 0.0), jnp.where(first, s4[0], 0.0)))
        for part in range(2):
            fd_ref[k, part, pl.ds(0, 40), :] = _pack(
                _cat([v[part] for v in vals] + [jnp.zeros((8, 128), F32)]))
            fd_ref[k, part, pl.ds(40, 24), :] = jnp.zeros((24, 128), I32)
        rho = (-rho[1], rho[0])


def _ssm_bases(g, h, par_ref, dt_ref, base_ref):
    a_re, a_im, b_re, b_im, c_re, c_im = (
        par_ref[k, _rows(g, G), :].astype(F32) for k in range(6))
    dt = dt_ref[_rows(g, G), :]
    dts = dt * (2.0 / 512)
    row = _iota((8, 128), 0)

    def deal(v):
        return _cat([jnp.take_along_axis(v[lo:lo + 8], (row >> 1) + 4 * (row & 1), axis=0,
                                         mode="promise_in_bounds") for lo in (0, 8)])

    decay, phase = deal(dt * a_re), deal(dt * a_im)
    w = tuple(deal(v) for v in _cmul((c_re, c_im), (dts * b_re, dts * b_im)))
    z, unit = {}, (jnp.cos(phase), jnp.sin(phase))
    for e in (1, 2, 4, 8, 16, 32, 64, 128, 256):
        if e in (1, 4, 8, 16, 256):
            mag = jnp.exp2(decay * (e * math.log2(math.e)))
            z[e] = (mag * unit[0], mag * unit[1])
        if e < 256:
            unit = _csq(unit)
    z1024 = _csq(_csq(z[256]))
    w8, w1024 = _cmul(w, z[8]), _cmul(w, z1024)
    seq = [(jnp.ones_like(dt), jnp.zeros_like(dt)), z[8], z[16], z[16], _cmul(z[16], z[8]),
           z[1], z[1], z[256], z[256], w, _cmul(w, z[4]), w,
           w8, w1024, w8, w1024, _cmul(w1024, z1024), w1024]
    for k, v in enumerate(seq):
        for t in range(2):
            for part in range(2):
                base_ref[h + t, part, pl.ds(8 * k, 8), :] = v[part][8 * t:8 * t + 8]


_OFFSETS = ((0, 4), (1, 5), (2, 6), (3, 7), (258, 262), (256, 260), (512, 516), (768, 772),
            (264, 1280), (520, 1536), (776, 1792), (1024, 2048))


def _ssm_values(h, base_ref, kv_ref):
    for quad in range(2):
        def pair(k):
            return tuple(base_ref[h, part, pl.ds(8 * k + quad, 8, stride=2), :]
                         for part in range(2))

        v = [pair(0)] + _powers(pair(3), pair(2), 15)
        z256 = pair(7)
        w = _powers(pair(9 + quad), pair(5), 4)
        w += [_cmul(w[2], z256)] + _powers(w[0], z256, 4)[1:]
        w += _powers(pair(12 + quad), z256, 4)[1:] + [pair(15 + quad)]
        re, im = (_mm(_cat([t[part] for t in w]), _cat([t[part] for t in v[::-1]]), NT)
                  for part in range(2))
        kv_ref[h, quad] = re - im


def _ssm_arrange(h, slot, kv_ref, kr_ref):
    lane, row = _iota((8, 128), 1), _iota((8, 128), 0)
    src = 4 * (((lane >> 1) & 31) ^ 30) + (row & 3)
    top = row < 4

    def spread(x):
        return jnp.take_along_axis(x, src, axis=1, mode="promise_in_bounds")

    def even(a, b):
        return jnp.where((lane & 1) == 0, a, b)

    def low(a, b):
        return jnp.where(lane < 64, a, b)

    val = {}
    for u, (e0, e1) in enumerate(_OFFSETS):
        a, b = (kv_ref[h, quad, pl.ds(8 * u, 8), :] for quad in range(2))
        val[e0] = spread(jnp.where(top, a, b))
        val[e1] = spread(pltpu.roll(jnp.where(top, b, a), 4, 0))
    mid = even(val[256], val[260])
    q0, q4, q8 = low(val[512], val[768]), low(val[516], val[772]), low(val[520], val[776])
    blocks = [
        (low(even(val[0], val[4]), mid), even(q0, q4)),
        (low(even(val[1], val[5]), mid), even(q0, q4)),
        (low(even(val[2], val[6]), even(val[258], val[262])), even(q0, q8)),
        (low(even(val[3], val[7]), even(val[260], val[264])), even(q4, q8)),
        (low(even(val[1024], val[1280]), val[1536]),
         low(even(val[1536], val[1792]), jnp.where(lane == 64, val[2048], 0.0)))]
    for j, pair in enumerate(blocks):
        kr_ref[slot, j] = _cat(pair)


def _ssm_kernel(wait_rest, par_ref, dt_ref, base_ref, kv_ref, kr_ref):
    def body(n, zero):
        pl.when(n == 1)(wait_rest)
        for r in range(SSM_UNROLL):
            g, slot = n * SSM_UNROLL + r, 2 * (r % 2)
            for t in range(2):
                _ssm_arrange(slot + t, 2 * g + t, kv_ref, kr_ref)
                _ssm_values(slot + t, base_ref, kv_ref)
            ahead = g + 2 if r + 2 < SSM_UNROLL else jnp.minimum(g + 2, NG - 1)
            _ssm_bases(ahead, slot, par_ref, dt_ref, base_ref)
        return jnp.minimum(zero, n * L)

    for g in range(2):
        _ssm_bases(g, 2 * g, par_ref, dt_ref, base_ref)
    kv_ref[...] = jnp.zeros_like(kv_ref)
    zero = lax.fori_loop(0, NG // SSM_UNROLL, body, L)
    for h in range(4):
        _ssm_arrange(h, NH + h, kv_ref, kr_ref)
    return zero


def _ssm_spectrum(first, count, batch, fine, kr_ref, fk_ref, fd_ref, kf_ref):
    def blocks(x):
        x = x.reshape(batch, 2, 1, 8, 128)
        return x[:, :1], x[:, 1:]

    for h0 in range(first, first + count, batch):
        near, far = [], []
        for n in range(4):
            lhs = {j: [] for j in ((0, 1, 2, 3) if n < 2 else (4,))}
            for h in range(h0, h0 + batch):
                for j, rows in lhs.items():
                    rows.append(kr_ref[4 + h, j])
                if fine:
                    yield
            if n < 2:
                near.append([_mm(_cat(lhs[j]), _bf(fk_ref[j, n])) for j in range(4)])
            else:
                far += [[_mm(_cat(lhs[4]), _bf(fd_ref[k, part])) for part in range(2)]
                        for k in (2 * n - 4, 2 * n - 3)]
            if not fine:
                yield
        out = []
        for a, b in zip(_dft4(list(zip(*near))), far):
            spec = list(zip(*(blocks(a[part]) + blocks(b[part]) for part in range(2))))
            spec = spec[:1] + [_csub_i(spec[p], spec[p - 1]) for p in range(1, 4)]
            out += [_cat(v, 1) for v in zip(*spec)]
        kf_ref[pl.ds(4 * h0, 4 * batch)] = _cat(out, 2).reshape(4 * batch, 8, 8, 128)


XN = 8


def _fold(x):
    x = x.reshape(3, -1, 8, 128)
    x = x[0] + x[1] + x[2]
    while x.shape[0] > 1:
        x = x[:x.shape[0] // 2] + x[x.shape[0] // 2:]
    return x[0]


def _norm_mean(x_ref, xp_ref, tally):
    for p in range(4):
        for i in range(NG // MEAN_GROUPS):
            r = [pltpu.bitcast(x_ref[_rows(i, MEAN_GROUPS * G), _rows(4 * p + q, 128)], I32)
                 for q in range(4)]
            r = _skew([r[0]] + [pltpu.roll(r[q], q, 1) for q in range(1, 4)])
            for j in range(4):
                xp_ref[p, j, _rows(i, MEAN_GROUPS * 8), :] = r[j]
                tally(p, j, 0, _fold(_bf(r[j]).astype(F32)), i == 0)
            yield


def _norm_centre(xp_ref, cen_ref, stat_ref, tally):
    for i in range(NG // VAR_GROUPS):
        for p, j in itertools.product(range(4), range(4)):
            x = _bf(xp_ref[p, j, _rows(i, VAR_GROUPS * 8), :]).astype(F32)
            d = x.reshape(VAR_GROUPS, G, 128) - _cat([stat_ref[1, p, j]] * 2)
            cen_ref[p, j, _rows(i, VAR_GROUPS)] = _cat([d[:, :8], d[:, 8:]], 2).astype(BF16)
            tally(p, j, 1, _fold(d * d), i == 0)
            yield


def _average(v):
    return jnp.broadcast_to(jnp.sum(v, axis=0, keepdims=True), v.shape) / D


def _norm_factor(squares, mean):
    shift = mean - _round_bf16(mean)
    var = _round_bf16(jnp.maximum(_average(squares) - shift * shift, 0.0))
    eps = _round_bf16(jnp.full_like(var, EPS))
    return 0.5 / _round_bf16(jnp.sqrt(_round_bf16(var + eps)))


def _norm_scale(wr_ref, cen_ref, stat_ref, work_ref):
    wr = jnp.broadcast_to(2.0 * wr_ref[...].astype(F32).reshape(1, D), (8, D))
    for p in range(4):
        score = [None] * 4
        for lo in range(0, D, 128):
            n = min(128, D - lo)
            for j in range(4):
                d = cen_ref[p, j, pl.ds(lo // G, n // G)].astype(F32)
                half = _cat([d[:, :, :128], d[:, :, 128:]], 1).reshape(n // 8, 8, 128)
                half = half * stat_ref[0, p, j]
                work_ref[pl.ds(lo // 8, n // 8), p, XN + j] = half
                part = _mm(wr[:, lo:lo + n], half.reshape(n, 128))
                score[j] = part if lo == 0 else score[j] + part
            yield
        for j in range(4):
            stat_ref[1, p, j] = score[j]


def _route(stat_ref, work_ref, hot_ref, xs_ref, gate_ref):
    row, blk = _iota((8, 128), 0), _iota((16, 128), 0)
    halves = []
    for lo in (0, 2):
        dense = stat_ref[1, lo, 0]
        for c in range(1, 8):
            dense = jnp.where(row == c, stat_ref[1, lo + c // 4, c % 4], dense)
        halves.append(dense)
    score = _round_bf16(_cat(halves))
    bits = pltpu.bitcast(jnp.where(score == 0.0, 0.0, score), I32) >> 16
    order = jnp.where(bits < 0, bits ^ 0x7FFF, bits) + 0x8000
    time = 512 * (blk >> 2) + _x_time(blk & 3, _iota((16, 128), 1))
    key = pltpu.bitcast((1 << 29) + (order << 11) + (L - 1 - time), F32)
    rank = jnp.full((16, 128), TOPK, I32)
    best = jnp.zeros((8, 128), F32)
    for i in range(TOPK):
        top = jnp.max(jnp.max(key, axis=0, keepdims=True), axis=1, keepdims=True)
        hit = key == top
        rank = jnp.where(hit, i, rank)
        key = jnp.where(hit, 0.0, key)
        best = jnp.where(row == i, top, best)
        yield from range(2)
    order = ((pltpu.bitcast(best, I32) >> 11) & 0xFFFF) - 0x8000
    best = pltpu.bitcast(jnp.where(order < 0, order ^ 0x7FFF, order) << 16, F32)
    gate_ref[...] = 0.5 * _round_bf16(jax.nn.sigmoid(best))
    for c in range(16):
        hot_ref[c] = jnp.where(jnp.broadcast_to(rank[c:c + 1], (8, 128)) == row, 1.0, 0.0)
    for lo in range(0, D, 128):
        n, picked = min(128, D - lo), None
        for p in range(4):
            for j in range(4):
                tokens = work_ref[pl.ds(lo // 8, n // 8), p, XN + j]
                part = _mm(hot_ref[4 * p + j], tokens.reshape(n, 128), NT)
                picked = part if picked is None else picked + part
            yield
        xs_ref[:, pl.ds(lo, n)] = 2.0 * picked
    yield from range(2)


def _ffn_up(second, xs_ref, w_ref, h_ref):
    for col in range(0, F, 512):
        acc = None
        for lo in range(0, D, 128):
            rows = pl.ds(lo, min(128, D - lo))
            part = _mm(xs_ref[:, rows], w_ref[rows, pl.ds(col, 512)])
            acc = part if lo == 0 else acc + part
            yield
        acc = _round_bf16(acc)
        h_ref[:, pl.ds(col, 512)] = (h_ref[:, pl.ds(col, 512)] * acc if second
                                     else _round_bf16(_silu_of_twice(0.5 * acc)))


def _ffn_down(lo, n, h_ref, wd_ref, gate_ref, upd_ref):
    ffn = None
    for k in range(0, F, 512):
        part = _mm(h_ref[:, pl.ds(k, 512)], wd_ref[pl.ds(lo, n), pl.ds(k, 512)], NT)
        ffn = part if ffn is None else ffn + part
        if k + 512 < F:
            yield
    upd_ref[pl.ds(lo, n), :] = (_round_bf16(ffn) * gate_ref[:, :n]).T


def _convolve(start, stop, zero, kf_ref, fx_ref, fxt_ref, xf_ref, work_ref, y_ref):
    def products(g):
        for h, k in itertools.product((2 * g, 2 * g + 1), range(4)):
            kf, x = ([tuple(ref[4 * h + p, 2 * k + part] for part in range(2))
                      for p in range(4)] for ref in (kf_ref, xf_ref))
            for c in (3, 0, 2, 1):
                acc = _cmul(kf[0], x[c])
                for p in range(1, c + 1):
                    acc = _cadd(acc, _cmul(kf[p], x[c - p]))
                for part in range(2):
                    work_ref[h + zero, c, 2 * k + part] = acc[part]
                if c < 2:
                    yield

    def operands(g, slots, fill):
        rows = []
        for h, p in itertools.product((2 * g, 2 * g + 1), range(4)):
            rows.append(work_ref[h, pl.ds(p, 1), slots])
            if p % 2:
                next(fill, None)
        rows = _cat(rows)
        return [rows[:, s].reshape(64, 128) for s in range(slots.size)]

    def butterflies(g, comp):
        spec = [v.reshape(8, 1, 8, 128) for pair in _dft4(list(zip(*comp))) for v in pair]
        xf_ref[pl.ds(8 * g + zero, 8)] = _cat(spec, 1)

    pending = None
    for i in range(start, stop):
        fill = products(i - 2) if 0 <= i - 2 < NG else iter(())
        for odd in range(2):
            if 0 <= i - 3:
                v = operands(i - 3, pl.ds(0, XN), fill)
                v = list(zip(v[0::2], v[1::2]))
                if odd:
                    a, b = _csub(v[0], v[2]), _csub(v[1], v[3])
                    back = _csub_i(a, b), _cadd_i(a, b)
                else:
                    a, b = _cadd(v[0], v[2]), _cadd(v[1], v[3])
                    back = _cadd(a, b), _csub(a, b)
                for j, spec in zip((odd, odd + 2), back):
                    y = _mm(_cat(spec, 1), _bf(fxt_ref[j]))
                    y_ref[_rows(i - 3, 2), :, j] = y.reshape(2, 4, 8, 128)
            yield
        if pending:
            butterflies(*pending)
        pending = (i, []) if i < NG else None
        for part in range(2):
            if pending:
                x = operands(i, pl.ds(XN, 4), fill)
                pending[1].append([_mm(x[j], _bf(fx_ref[j, part])) for j in range(4)])
            yield
        for _ in fill:
            pass
    if pending:
        butterflies(*pending)


def _gate(lo, n, upd_ref, hot_ref, xp_ref, work_ref, y_ref, skip_ref, o_ref):
    for i in range(lo // 64, (lo + n) // 64):
        for p in range(4):
            r = []
            for j in range(4):
                x = _bf(xp_ref[p, j, _rows(i, 32), :]).astype(F32)
                half = work_ref[_rows(i, 8), p, XN + j].reshape(64, 128)
                s = (y_ref[_rows(i, 8), p, j].reshape(64, 128)
                     + half * skip_ref[_rows(i, 64), :])
                routed = _mm(upd_ref[_rows(i, 64), :], hot_ref[4 * p + j])
                r.append(x + s * _silu_of_twice(half + routed))
            r = _skew(r)
            r = [r[0]] + [pltpu.roll(r[q], 128 - q, 1) for q in range(1, 4)]
            o_ref[_rows(i, 64), _rows(p, 512)] = _cat(r, 1).astype(BF16)
            yield


def _kernel(x_hbm, are_hbm, aim_hbm, bre_hbm, bim_hbm, cre_hbm, cim_hbm, ldt_hbm, dsk_hbm,
            wr_hbm, wg_hbm, wu_hbm, wd_hbm, o_hbm,
            x_ref, par_ref, ldt_ref, dsk_ref, wr_ref, wg_ref, wu_ref, wd_ref, o_ref,
            fx_ref, fxt_ref, fk_ref, fd_ref, dt_ref, skip_ref, base_ref, kv_ref, kr_ref,
            kf_ref, xp_ref, stat_ref, cen_ref, work_ref, xf_ref, y_ref,
            hot_ref, xs_ref, gate_ref, h_ref, upd_ref, sems):
    def batch(sem, *pairs):
        return [pltpu.make_async_copy(src, dst, sems.at[sem]) for src, dst in pairs]

    def start(copies):
        for cp in copies:
            cp.start()

    def wait(copies):
        for cp in copies:
            cp.wait()

    def params(rows):
        return [(src.at[rows], par_ref.at[i, rows]) for i, src in
                enumerate((are_hbm, aim_hbm, bre_hbm, bim_hbm, cre_hbm, cim_hbm))]

    early = (SSM_UNROLL + 2) * G
    head = batch(0, (ldt_hbm, ldt_ref), *params(pl.ds(0, early)))
    rest = batch(1, *params(pl.ds(early, D - early)))
    inputs = batch(2, (x_hbm, x_ref), (wr_hbm, wr_ref), (dsk_hbm, dsk_ref))
    w_gate, w_up = batch(0, (wg_hbm, wg_ref)), batch(1, (wu_hbm, wu_ref))
    w_down = [batch(sem, (wd_hbm.at[pl.ds(*rows)], wd_ref.at[pl.ds(*rows)]))
              for sem, rows in zip((2, 0, 1), DOWN_COPIES)]
    outs = batch(2, *[(o_ref.at[pl.ds(*rows)], o_hbm.at[pl.ds(*rows)]) for rows in CHUNKS])

    def wait_rest():
        wait(rest)
        start(w_up)

    start(head + rest + inputs)
    _kernel_transform(fk_ref, fd_ref)
    _input_transform(fx_ref, fxt_ref)
    wait(head)
    start(w_gate)
    _column(ldt_ref, dt_ref, lambda v: _round_bf16(jnp.exp(v)))
    zero = _ssm_kernel(wait_rest, par_ref, dt_ref, base_ref, kv_ref, kr_ref)

    def tally(p, j, n, value, first):
        kr_ref[p + zero, j, _rows(n, 8), :] = (
            value if first else kr_ref[p, j, _rows(n, 8), :] + value)

    def norm_pass(n, job, pieces, fine):
        count, batch = NORM_SHARE[n]
        first = sum(share[0] for share in NORM_SHARE[:n])

        @pl.when(zero < NG)
        def _():
            _weave(_ssm_spectrum(first, count, batch, fine, kr_ref, fk_ref, fd_ref, kf_ref),
                   job, pieces / (4 * count // (1 if fine else batch) - 1))

    wait(inputs)
    start(w_down[0])
    norm_pass(0, _norm_mean(x_ref, xp_ref, tally), 4 * NG // MEAN_GROUPS, True)
    for p, j in itertools.product(range(4), range(4)):
        stat_ref[0, p, j] = _average(kr_ref[p, j, _rows(0, 8), :])
        stat_ref[1, p, j] = _round_bf16(stat_ref[0, p, j])
    norm_pass(1, _norm_centre(xp_ref, cen_ref, stat_ref, tally), 16 * NG // VAR_GROUPS, True)
    for p, j in itertools.product(range(4), range(4)):
        stat_ref[0, p, j] = _norm_factor(kr_ref[p, j, _rows(1, 8), :], stat_ref[0, p, j])
    norm_pass(2, _norm_scale(wr_ref, cen_ref, stat_ref, work_ref), 20, False)

    def convolve(first, stop):
        return _convolve(first, stop, zero, kf_ref, fx_ref, fxt_ref, xf_ref, work_ref, y_ref)

    def ffn_down(i):
        return _ffn_down(*CHUNKS[i], h_ref, wd_ref, gate_ref, upd_ref)

    wait(w_gate)
    start(w_down[1])
    _weave(convolve(0, CONV_CUTS[0]), itertools.chain(
        _route(stat_ref, work_ref, hot_ref, xs_ref, gate_ref),
        _ffn_up(False, xs_ref, wg_ref, h_ref)))
    wait(w_up)
    start(w_down[2])
    _weave(convolve(*CONV_CUTS), _ffn_up(True, xs_ref, wu_ref, h_ref))
    wait(w_down[0])
    _column(dsk_ref, skip_ref, lambda v: 2.0 * v)
    _weave(convolve(CONV_CUTS[1], NG + 3), ffn_down(0))

    for i, chunk in enumerate(CHUNKS):
        _weave(_gate(*chunk, upd_ref, hot_ref, xp_ref, work_ref, y_ref, skip_ref, o_ref),
               ffn_down(i + 1) if i + 1 < len(CHUNKS) else iter(()), 1.8)
        if i + 1 in DOWN_WAITS:
            wait(w_down[DOWN_WAITS[i + 1]])
        outs[i].start()
    wait(outs)


@jax.jit
def pallas_recurrent_scan__ssm_conv_s4__moe_arch_mod__prompt_kernel(
    A_u: jax.Array,
    A_A_re: jax.Array,
    A_A_im: jax.Array,
    A_B_re: jax.Array,
    A_B_im: jax.Array,
    A_C_re: jax.Array,
    A_C_im: jax.Array,
    A_log_dt: jax.Array,
    A_Dskip: jax.Array,
    B_x: jax.Array,
    B_w_r: jax.Array,
    B_w_gate: jax.Array,
    B_w_up: jax.Array,
    B_w_down: jax.Array,
):
    del B_x
    assert A_u.shape == (1, L, D) and A_A_re.shape == (D, N) and B_w_gate.shape == (D, F)
    assert A_A_re.dtype == BF16
    vmem = pltpu.VMEM
    scratch = [
        vmem((D, L), BF16), vmem((6, D, N), BF16),
        vmem((D,), BF16), vmem((D,), BF16), vmem((D,), BF16),
        vmem((D, F), BF16), vmem((D, F), BF16), vmem((D, F), BF16), vmem((D, L), BF16),
        vmem((4, 2, 64, 128), I32), vmem((4, 128, 128), I32),
        vmem((4, 2, 64, 128), I32), vmem((4, 2, 64, 128), I32),
        vmem((D, 128), F32), vmem((D, 128), F32),
        vmem((4, 2, 144, 128), F32), vmem((4, 2, 96, 128), F32),
        vmem((NH + 4, 5, 16, 128), F32), vmem((4 * NH, 8, 8, 128), F32),
        vmem((4, 4, D // 2, 128), I32), vmem((2, 4, 4, 8, 128), F32),
        vmem((4, 4, NG, 8, 256), BF16),
        vmem((NH, 4, XN + 4, 8, 128), F32), vmem((4 * NH, 8, 8, 128), F32),
        vmem((NH, 4, 4, 8, 128), F32),
        vmem((16, 8, 128), F32), vmem((8, D), F32), vmem((8, 128), F32), vmem((8, F), F32),
        vmem((D, TOPK), F32),
        pltpu.SemaphoreType.DMA((3,)),
    ]
    out = pl.pallas_call(
        _kernel,
        out_shape=jax.ShapeDtypeStruct((D, L), BF16),
        in_specs=[pl.BlockSpec(memory_space=pl.ANY)] * 13,
        out_specs=pl.BlockSpec(memory_space=pl.ANY),
        scratch_shapes=scratch,
        compiler_params=pltpu.CompilerParams(vmem_limit_bytes=100 * 1024 * 1024),
    )(A_u[0].T, A_A_re, A_A_im, A_B_re, A_B_im, A_C_re, A_C_im, A_log_dt, A_Dskip,
      B_w_r, B_w_gate, B_w_up, B_w_down.T)
    return out.T[None]
```

```python
import itertools
import math

import jax
import jax.numpy as jnp
from jax import lax
import jax.experimental.pallas as pl
import jax.experimental.pallas.tpu as pltpu

F32, BF16, I32 = jnp.float32, jnp.bfloat16, jnp.int32
L, D, N, F, TOPK = 2048, 576, 128, 4608, 8
EPS = 1e-5
G = 16
NG = D // G
NH = D // 8
NN = (((1,), (0,)), ((), ()))
NT = (((1,), (1,)), ((), ()))

SSM_UNROLL = 6
NORM_SHARE = ((24, 2), (30, 3), (18, 3))
MEAN_GROUPS, VAR_GROUPS = 3, 6
CONV_CUTS = (0, 21, 33, NG + 3)
CHUNKS = ((0, 128), (128, 128), (256, 128), (384, 128), (512, 64))
SHORT_PER_WEIGHT = (45, 28, 13, 5)
SHORT_PER_PHASE = (7, 7, 6, 22, 13, 0)
assert sum(SHORT_PER_WEIGHT) == NG + sum(SHORT_PER_PHASE)
FINE_ROWS = (0, 448, 512)
DOWN_RATE, PAUSE = 2.0, 3


def _iota(shape, dim):
    return lax.broadcasted_iota(I32, shape, dim)


def _rows(i, n):
    return pl.ds(i * n if isinstance(i, int) else pl.multiple_of(i * n, n), n)


def _cat(xs, axis=0):
    return jnp.concatenate(xs, axis=axis)


def _cmul(a, b):
    return a[0] * b[0] - a[1] * b[1], a[0] * b[1] + a[1] * b[0]


def _csq(a):
    return a[0] * a[0] - a[1] * a[1], (a[0] + a[0]) * a[1]


def _cadd(a, b):
    return a[0] + b[0], a[1] + b[1]


def _csub(a, b):
    return a[0] - b[0], a[1] - b[1]


def _cadd_i(a, b):
    return a[0] - b[1], a[1] + b[0]


def _csub_i(a, b):
    return a[0] + b[1], a[1] - b[0]


def _dft4(v):
    s02, d02 = _cadd(v[0], v[2]), _csub(v[0], v[2])
    s13, d13 = _cadd(v[1], v[3]), _csub(v[1], v[3])
    return [_cadd(s02, s13), _cadd_i(d02, d13), _csub(s02, s13), _csub_i(d02, d13)]


def _root(n):
    ang = (((n + 1024) & 2047) - 1024).astype(F32) * (2.0 * math.pi / 2048)
    return jnp.cos(ang), jnp.sin(ang)


def _powers(start, step, count):
    vals = [start]
    for _ in range(count - 1):
        vals.append(_cmul(vals[-1], step))
    return vals


def _pack(x):
    return pltpu.bitcast(x.astype(BF16), I32)


def _bf(x):
    return pltpu.bitcast(x, BF16)


def _round_bf16(x):
    return x.astype(BF16).astype(F32)


def _silu_of_twice(h):
    return h + h * jnp.tanh(h)


def _mm(a, b, dims=NN):
    return lax.dot_general(a, b, dims, precision=lax.Precision.DEFAULT,
                           preferred_element_type=F32)


def _skew(r):
    lane = _iota(r[0].shape, 1)
    b0, b1 = (lane & 1) != 0, (lane & 2) != 0
    t = [lax.select(b0, r[(k + 1) % 4], r[k]) for k in range(4)]
    u = [lax.select(b1, t[(k + 2) % 4], t[k]) for k in range(4)]
    return [u[(-j) % 4] for j in range(4)]


def _x_time(j, m):
    q = (m - j) & 3
    return 128 * q + ((m - q) & 127)


def _weave(main, side, rate=1.0):
    credit = 0.0
    for _ in main:
        credit += rate
        while credit >= 1.0:
            credit -= 1.0
            next(side, None)
    for _ in side:
        pass


def _column(v_ref, out_ref, fn):
    v = fn(v_ref[...].astype(F32).reshape(1, D))
    for lo in range(0, D, 128):
        n = min(128, D - lo)
        out_ref[pl.ds(lo, n), :] = jnp.broadcast_to(v[:, lo:lo + n], (128, n)).T


def _input_transform(fx_ref, fxt_ref):
    freq, row = 4 * _iota((8, 128), 1) + 1, _iota((8, 128), 0)
    step8 = _root(8 * freq)
    step128 = _csq(_csq(_csq(_csq(step8))))
    for j in range(4):
        start = _root((_x_time(j, row + 8) - 8) * freq)
        vals = _powers(start, step8, 16)
        wraps = row < ((row - j) & 3)
        vals[0] = tuple(jnp.where(wraps, a, b) for a, b in zip(_cmul(start, step128), start))
        for part in range(2):
            m = _cat([v[part] for v in vals])
            fx_ref[j, part] = _pack(m)
            fxt_ref[j, pl.ds(64 * part, 64), :] = _pack(m.T)


def _kernel_transform(fk_ref, fd_ref):
    freq, row = 4 * _iota((8, 128), 1) + 1, _iota((8, 128), 0)
    rho = _root(freq)
    step32 = _csq(_csq(_csq(_csq(_csq(rho)))))
    for j, start in enumerate(_powers(_root(4 * row * freq), rho, 4)):
        vals = _powers(start, step32, 16)
        for part in range(2):
            fk_ref[j, part] = _pack(_cat([v[part] for v in vals]))
    rows = _powers(_root((256 * (row & 1) + 8 * (row >> 1)) * freq), step32, 8)
    first = row == 0
    for k in range(4):
        p2 = _csq(rho)
        s3 = _cadd(_cadd(rho, p2), _cmul(p2, rho))
        s4 = _cadd(s3, _csq(p2))
        box = 1.0 + 2.0 * jnp.where((row & 2) == 0, s4[0], s3[0])
        vals = [(r[0] * box, r[1] * box) for r in rows]
        vals[0] = (jnp.where(first, 1.0 + s4[0], vals[0][0]),
                   jnp.where(first, s4[1], vals[0][1]))
        vals.append((jnp.where(first, s4[1], 0.0), jnp.where(first, s4[0], 0.0)))
        for part in range(2):
            fd_ref[k, part, pl.ds(0, 40), :] = _pack(
                _cat([v[part] for v in vals] + [jnp.zeros((8, 128), F32)]))
            fd_ref[k, part, pl.ds(40, 24), :] = jnp.zeros((24, 128), I32)
        rho = (-rho[1], rho[0])


def _ssm_bases(g, h, par_ref, dt_ref, base_ref):
    a_re, a_im, b_re, b_im, c_re, c_im = (
        par_ref[k, _rows(g, G), :].astype(F32) for k in range(6))
    dt = dt_ref[_rows(g, G), :]
    dts = dt * (2.0 / 512)
    row = _iota((8, 128), 0)

    def deal(v):
        return _cat([jnp.take_along_axis(v[lo:lo + 8], (row >> 1) + 4 * (row & 1), axis=0,
                                         mode="promise_in_bounds") for lo in (0, 8)])

    decay, phase = deal(dt * a_re), deal(dt * a_im)
    w = tuple(deal(v) for v in _cmul((c_re, c_im), (dts * b_re, dts * b_im)))
    z, unit = {}, (jnp.cos(phase), jnp.sin(phase))
    for e in (1, 2, 4, 8, 16, 32, 64, 128, 256):
        if e in (1, 4, 8, 16, 256):
            mag = jnp.exp2(decay * (e * math.log2(math.e)))
            z[e] = (mag * unit[0], mag * unit[1])
        if e < 256:
            unit = _csq(unit)
    z1024 = _csq(_csq(z[256]))
    w8, w1024 = _cmul(w, z[8]), _cmul(w, z1024)
    seq = [(jnp.ones_like(dt), jnp.zeros_like(dt)), z[8], z[16], z[16], _cmul(z[16], z[8]),
           z[1], z[1], z[256], z[256], w, _cmul(w, z[4]), w,
           w8, w1024, w8, w1024, _cmul(w1024, z1024), w1024]
    for k, v in enumerate(seq):
        for t in range(2):
            for part in range(2):
                base_ref[h + t, part, pl.ds(8 * k, 8), :] = v[part][8 * t:8 * t + 8]


_OFFSETS = ((0, 4), (1, 5), (2, 6), (3, 7), (258, 262), (256, 260), (512, 516), (768, 772),
            (264, 1280), (520, 1536), (776, 1792), (1024, 2048))


def _ssm_values(h, base_ref, kv_ref):
    for quad in range(2):
        def pair(k):
            return tuple(base_ref[h, part, pl.ds(8 * k + quad, 8, stride=2), :]
                         for part in range(2))

        v = [pair(0)] + _powers(pair(3), pair(2), 15)
        z256 = pair(7)
        w = _powers(pair(9 + quad), pair(5), 4)
        w += [_cmul(w[2], z256)] + _powers(w[0], z256, 4)[1:]
        w += _powers(pair(12 + quad), z256, 4)[1:] + [pair(15 + quad)]
        re, im = (_mm(_cat([t[part] for t in w]), _cat([t[part] for t in v[::-1]]), NT)
                  for part in range(2))
        kv_ref[h, quad] = re - im


def _ssm_arrange(h, slot, kv_ref, kr_ref):
    lane, row = _iota((8, 128), 1), _iota((8, 128), 0)
    src = 4 * (((lane >> 1) & 31) ^ 30) + (row & 3)
    top = row < 4

    def spread(x):
        return jnp.take_along_axis(x, src, axis=1, mode="promise_in_bounds")

    def even(a, b):
        return jnp.where((lane & 1) == 0, a, b)

    def low(a, b):
        return jnp.where(lane < 64, a, b)

    val = {}
    for u, (e0, e1) in enumerate(_OFFSETS):
        a, b = (kv_ref[h, quad, pl.ds(8 * u, 8), :] for quad in range(2))
        val[e0] = spread(jnp.where(top, a, b))
        val[e1] = spread(pltpu.roll(jnp.where(top, b, a), 4, 0))
    mid = even(val[256], val[260])
    q0, q4, q8 = low(val[512], val[768]), low(val[516], val[772]), low(val[520], val[776])
    blocks = [
        (low(even(val[0], val[4]), mid), even(q0, q4)),
        (low(even(val[1], val[5]), mid), even(q0, q4)),
        (low(even(val[2], val[6]), even(val[258], val[262])), even(q0, q8)),
        (low(even(val[3], val[7]), even(val[260], val[264])), even(q4, q8)),
        (low(even(val[1024], val[1280]), val[1536]),
         low(even(val[1536], val[1792]), jnp.where(lane == 64, val[2048], 0.0)))]
    for j, pair in enumerate(blocks):
        kr_ref[slot, j] = _cat(pair)


def _ssm_kernel(wait_rest, every_group, par_ref, dt_ref, base_ref, kv_ref, kr_ref):
    def body(n, zero):
        pl.when(n == 1)(wait_rest)
        for r in range(SSM_UNROLL):
            g, slot = n * SSM_UNROLL + r, 2 * (r % 2)
            for t in range(2):
                _ssm_arrange(slot + t, 2 * g + t, kv_ref, kr_ref)
                _ssm_values(slot + t, base_ref, kv_ref)
            every_group(g, kv_ref[slot, 0, pl.ds(0, 8), :])
            ahead = g + 2 if r + 2 < SSM_UNROLL else jnp.minimum(g + 2, NG - 1)
            _ssm_bases(ahead, slot, par_ref, dt_ref, base_ref)
        return jnp.minimum(zero, n * L)

    for g in range(2):
        _ssm_bases(g, 2 * g, par_ref, dt_ref, base_ref)
    kv_ref[...] = jnp.zeros_like(kv_ref)
    zero = lax.fori_loop(0, NG // SSM_UNROLL, body, L)
    for h in range(4):
        _ssm_arrange(h, NH + h, kv_ref, kr_ref)
    return zero


def _ssm_spectrum(first, count, batch, fine, kr_ref, fk_ref, fd_ref, kf_ref):
    def blocks(x):
        x = x.reshape(batch, 2, 1, 8, 128)
        return x[:, :1], x[:, 1:]

    recent = jnp.zeros((8, 128), F32)
    for h0 in range(first, first + count, batch):
        near, far = [], []
        for n in range(4):
            lhs = {j: [] for j in ((0, 1, 2, 3) if n < 2 else (4,))}
            for h in range(h0, h0 + batch):
                for j, rows in lhs.items():
                    rows.append(kr_ref[4 + h, j])
                if fine:
                    yield recent
            if n < 2:
                near.append([_mm(_cat(lhs[j]), _bf(fk_ref[j, n])) for j in range(4)])
            else:
                far += [[_mm(_cat(lhs[4]), _bf(fd_ref[k, part])) for part in range(2)]
                        for k in (2 * n - 4, 2 * n - 3)]
            recent = (far or near)[-1][0]
            if not fine:
                yield recent
        out = []
        for a, b in zip(_dft4(list(zip(*near))), far):
            spec = list(zip(*(blocks(a[part]) + blocks(b[part]) for part in range(2))))
            spec = spec[:1] + [_csub_i(spec[p], spec[p - 1]) for p in range(1, 4)]
            out += [_cat(v, 1) for v in zip(*spec)]
        kf_ref[pl.ds(4 * h0, 4 * batch)] = _cat(out, 2).reshape(4 * batch, 8, 8, 128)


XN = 8


def _fold(x):
    x = x.reshape(3, -1, 8, 128)
    x = x[0] + x[1] + x[2]
    while x.shape[0] > 1:
        x = x[:x.shape[0] // 2] + x[x.shape[0] // 2:]
    return x[0]


def _norm_mean(x_ref, xp_ref, tally):
    for p in range(4):
        for i in range(NG // MEAN_GROUPS):
            r = [pltpu.bitcast(x_ref[_rows(i, MEAN_GROUPS * G), _rows(4 * p + q, 128)], I32)
                 for q in range(4)]
            r = _skew([r[0]] + [pltpu.roll(r[q], q, 1) for q in range(1, 4)])
            for j in range(4):
                xp_ref[p, j, _rows(i, MEAN_GROUPS * 8), :] = r[j]
                tally(p, j, 0, _fold(_bf(r[j]).astype(F32)), i == 0)
            yield


def _norm_centre(xp_ref, cen_ref, stat_ref, tally):
    for i in range(NG // VAR_GROUPS):
        for p, j in itertools.product(range(4), range(4)):
            x = _bf(xp_ref[p, j, _rows(i, VAR_GROUPS * 8), :]).astype(F32)
            d = x.reshape(VAR_GROUPS, G, 128) - _cat([stat_ref[1, p, j]] * 2)
            cen_ref[p, j, _rows(i, VAR_GROUPS)] = _cat([d[:, :8], d[:, 8:]], 2).astype(BF16)
            tally(p, j, 1, _fold(d * d), i == 0)
            yield


def _average(v):
    return jnp.broadcast_to(jnp.sum(v, axis=0, keepdims=True), v.shape) / D


def _norm_factor(squares, mean):
    shift = mean - _round_bf16(mean)
    var = _round_bf16(jnp.maximum(_average(squares) - shift * shift, 0.0))
    eps = _round_bf16(jnp.full_like(var, EPS))
    return 0.5 / _round_bf16(jnp.sqrt(_round_bf16(var + eps)))


def _norm_scale(wr_ref, cen_ref, stat_ref, work_ref):
    wr = jnp.broadcast_to(2.0 * wr_ref[...].astype(F32).reshape(1, D), (8, D))
    for p in range(4):
        score = [None] * 4
        for lo in range(0, D, 128):
            n = min(128, D - lo)
            for j in range(4):
                d = cen_ref[p, j, pl.ds(lo // G, n // G)].astype(F32)
                half = _cat([d[:, :, :128], d[:, :, 128:]], 1).reshape(n // 8, 8, 128)
                half = half * stat_ref[0, p, j]
                work_ref[pl.ds(lo // 8, n // 8), p, XN + j] = half
                part = _mm(wr[:, lo:lo + n], half.reshape(n, 128))
                score[j] = part if lo == 0 else score[j] + part
            yield
        for j in range(4):
            stat_ref[1, p, j] = score[j]


def _route(stat_ref, work_ref, hot_ref, xs_ref, gate_ref):
    row, blk = _iota((8, 128), 0), _iota((16, 128), 0)
    halves = []
    for lo in (0, 2):
        dense = stat_ref[1, lo, 0]
        for c in range(1, 8):
            dense = jnp.where(row == c, stat_ref[1, lo + c // 4, c % 4], dense)
        halves.append(dense)
    score = _round_bf16(_cat(halves))
    bits = pltpu.bitcast(jnp.where(score == 0.0, 0.0, score), I32) >> 16
    order = jnp.where(bits < 0, bits ^ 0x7FFF, bits) + 0x8000
    time = 512 * (blk >> 2) + _x_time(blk & 3, _iota((16, 128), 1))
    key = pltpu.bitcast((1 << 29) + (order << 11) + (L - 1 - time), F32)
    rank = jnp.full((16, 128), TOPK, I32)
    best = jnp.zeros((8, 128), F32)
    for i in range(TOPK):
        top = jnp.max(jnp.max(key, axis=0, keepdims=True), axis=1, keepdims=True)
        hit = key == top
        rank = jnp.where(hit, i, rank)
        key = jnp.where(hit, 0.0, key)
        best = jnp.where(row == i, top, best)
        yield from range(2)
    order = ((pltpu.bitcast(best, I32) >> 11) & 0xFFFF) - 0x8000
    best = pltpu.bitcast(jnp.where(order < 0, order ^ 0x7FFF, order) << 16, F32)
    gate_ref[...] = 0.5 * _round_bf16(jax.nn.sigmoid(best))
    for c in range(16):
        hot_ref[c] = jnp.where(jnp.broadcast_to(rank[c:c + 1], (8, 128)) == row, 1.0, 0.0)
    for lo in range(0, D, 128):
        n, picked = min(128, D - lo), None
        for p in range(4):
            for j in range(4):
                tokens = work_ref[pl.ds(lo // 8, n // 8), p, XN + j]
                part = _mm(hot_ref[4 * p + j], tokens.reshape(n, 128), NT)
                picked = part if picked is None else picked + part
            yield
        xs_ref[:, pl.ds(lo, n)] = 2.0 * picked
    yield from range(2)


def _ffn_up(second, xs_ref, w_ref, h_ref):
    for col in range(0, F, 512):
        acc = None
        for lo in range(0, D, 128):
            rows = pl.ds(lo, min(128, D - lo))
            part = _mm(xs_ref[:, rows], w_ref[rows, pl.ds(col, 512)])
            acc = part if lo == 0 else acc + part
            yield
        acc = _round_bf16(acc)
        h_ref[:, pl.ds(col, 512)] = (h_ref[:, pl.ds(col, 512)] * acc if second
                                     else _round_bf16(_silu_of_twice(0.5 * acc)))


def _ffn_down(lo, n, h_ref, wd_ref, gate_ref, upd_ref):
    ffn = None
    for k in range(0, F, 512):
        part = _mm(h_ref[:, pl.ds(k, 512)], wd_ref[pl.ds(lo, n), pl.ds(k, 512)], NT)
        ffn = part if ffn is None else ffn + part
        yield
    yield from range(PAUSE)
    eye = jnp.where(_iota((n, n), 0) == _iota((n, n), 1), 1.0, 0.0)
    upd_ref[pl.ds(lo, n), :] = _mm(eye, _round_bf16(ffn) * gate_ref[:, :n], NT)


def _convolve(start, stop, zero, kf_ref, fx_ref, fxt_ref, xf_ref, work_ref, y_ref):
    def products(g):
        for h, k in itertools.product((2 * g, 2 * g + 1), range(4)):
            kf, x = ([tuple(ref[4 * h + p, 2 * k + part] for part in range(2))
                      for p in range(4)] for ref in (kf_ref, xf_ref))
            for c in (3, 0, 2, 1):
                acc = _cmul(kf[0], x[c])
                for p in range(1, c + 1):
                    acc = _cadd(acc, _cmul(kf[p], x[c - p]))
                for part in range(2):
                    work_ref[h + zero, c, 2 * k + part] = acc[part]
                if c < 2:
                    yield

    def operands(g, slots, fill):
        rows = []
        for h, p in itertools.product((2 * g, 2 * g + 1), range(4)):
            rows.append(work_ref[h, pl.ds(p, 1), slots])
            if p % 2:
                next(fill, None)
        rows = _cat(rows)
        return [rows[:, s].reshape(64, 128) for s in range(slots.size)]

    def butterflies(g, comp):
        spec = [v.reshape(8, 1, 8, 128) for pair in _dft4(list(zip(*comp))) for v in pair]
        xf_ref[pl.ds(8 * g + zero, 8)] = _cat(spec, 1)

    pending, recent = None, jnp.zeros((8, 128), F32)
    for i in range(start, stop):
        fill = products(i - 2) if 0 <= i - 2 < NG else iter(())
        for odd in range(2):
            if 0 <= i - 3:
                v = operands(i - 3, pl.ds(0, XN), fill)
                v = list(zip(v[0::2], v[1::2]))
                if odd:
                    a, b = _csub(v[0], v[2]), _csub(v[1], v[3])
                    back = _csub_i(a, b), _cadd_i(a, b)
                else:
                    a, b = _cadd(v[0], v[2]), _cadd(v[1], v[3])
                    back = _cadd(a, b), _csub(a, b)
                for j, spec in zip((odd, odd + 2), back):
                    recent = _mm(_cat(spec, 1), _bf(fxt_ref[j]))
                    y_ref[_rows(i - 3, 2), :, j] = recent.reshape(2, 4, 8, 128)
            yield recent
        if pending:
            butterflies(*pending)
        pending = (i, []) if i < NG else None
        for part in range(2):
            if pending:
                x = operands(i, pl.ds(XN, 4), fill)
                pending[1].append([_mm(x[j], _bf(fx_ref[j, part])) for j in range(4)])
                recent = pending[1][-1][0]
            yield recent
        for _ in fill:
            pass
    if pending:
        butterflies(*pending)


def _gate(lo, n, upd_ref, hot_ref, xp_ref, work_ref, y_ref, skip_ref, o_ref):
    for i in range(lo // 64, (lo + n) // 64):
        for p in range(4):
            r = []
            for j in range(4):
                x = _bf(xp_ref[p, j, _rows(i, 32), :]).astype(F32)
                half = work_ref[_rows(i, 8), p, XN + j].reshape(64, 128)
                s = (y_ref[_rows(i, 8), p, j].reshape(64, 128)
                     + half * skip_ref[_rows(i, 64), :])
                routed = _mm(upd_ref[_rows(i, 64), :], hot_ref[4 * p + j])
                r.append(x + s * _silu_of_twice(half + routed))
            r = _skew(r)
            r = [r[0]] + [pltpu.roll(r[q], 128 - q, 1) for q in range(1, 4)]
            o_ref[_rows(i, 64), _rows(p, 512)] = _cat(r, 1).astype(BF16)
            yield 64 * i, 512 * p


def _kernel(x_hbm, are_hbm, aim_hbm, bre_hbm, bim_hbm, cre_hbm, cim_hbm, ldt_hbm, dsk_hbm,
            wr_hbm, wg_hbm, wu_hbm, wd_hbm, o_hbm,
            x_ref, par_ref, ldt_ref, dsk_ref, wr_ref, wg_ref, wu_ref, wd_ref, o_ref,
            fx_ref, fxt_ref, fk_ref, fd_ref, dt_ref, skip_ref, base_ref, kv_ref, kr_ref,
            kf_ref, xp_ref, stat_ref, cen_ref, work_ref, xf_ref, y_ref,
            hot_ref, xs_ref, gate_ref, h_ref, upd_ref, sems):
    def copy(src, dst, sem, *part):
        if part:
            part = tuple(pl.ds(*p) for p in part)
            src, dst = src.at[part], dst.at[part]
        return pltpu.make_async_copy(src, dst, sems.at[sem])

    def params(sem, rows):
        return [copy(src, par_ref.at[i], sem, rows) for i, src in
                enumerate((are_hbm, aim_hbm, bre_hbm, bim_hbm, cre_hbm, cim_hbm))]

    def stream(*copies):
        for cp in copies:
            cp.start(priority=1)

    def wait(*copies):
        for cp in copies:
            cp.wait()

    def trickle(src, dst, sem, i, recent):
        dst[_rows(i, 8), pl.ds(0, 128)] = recent[:8].astype(BF16)
        copy(src.at[_rows(i, 8)], dst.at[_rows(i, 8)], sem).start()

    def with_trickle(jobs, count, pieces):
        due = [k * count // pieces for k in range(pieces)]
        for n, recent in enumerate(jobs):
            if n in due:
                trickle(*next(short), recent)
            yield

    def bulk(src, dst, sem, lo, hi, pieces):
        return copy(src, dst, sem, (lo + 8 * pieces, hi - lo - 8 * pieces))

    def whole(src, dst, sem, lo, hi, pieces):
        return copy(src, dst, sem, (lo, hi - lo))

    early, late = (SSM_UNROLL + 2) * G, CHUNKS[3][0]
    w_gate, w_up, w_down, w_last = weights = [w + (n,) for w, n in zip(
        ((wg_hbm, wg_ref, 0, 0, D), (wu_hbm, wu_ref, 1, 0, D),
         (wd_hbm, wd_ref, 2, 0, late), (wd_hbm, wd_ref, 0, late, D)), SHORT_PER_WEIGHT)]
    short = iter([(*w[:3], w[3] // 8 + i) for w in weights for i in range(w[5])][NG:])
    head = [copy(ldt_hbm, ldt_ref, 0)] + params(0, (0, early))
    rest = params(1, (early, D - early))
    inputs = [copy(x_hbm, x_ref, 2), copy(wr_hbm, wr_ref, 2), copy(dsk_hbm, dsk_ref, 2)]

    def wait_rest():
        wait(*rest)
        stream(bulk(*w_up))

    stream(*head, *rest, *inputs)
    _kernel_transform(fk_ref, fd_ref)
    _input_transform(fx_ref, fxt_ref)
    wait(*head)
    stream(bulk(*w_gate))
    _column(ldt_ref, dt_ref, lambda v: _round_bf16(jnp.exp(v)))
    zero = _ssm_kernel(wait_rest, lambda *a: trickle(*w_gate[:3], *a),
                       par_ref, dt_ref, base_ref, kv_ref, kr_ref)

    def tally(p, j, n, value, first):
        kr_ref[p + zero, j, _rows(n, 8), :] = (
            value if first else kr_ref[p, j, _rows(n, 8), :] + value)

    def norm_pass(n, job, pieces, fine):
        count, batch = NORM_SHARE[n]
        first = sum(share[0] for share in NORM_SHARE[:n])
        steps = 4 * count // (1 if fine else batch)

        @pl.when(zero < NG)
        def _():
            main = _ssm_spectrum(first, count, batch, fine, kr_ref, fk_ref, fd_ref, kf_ref)
            _weave(with_trickle(main, steps, SHORT_PER_PHASE[n]), job, pieces / (steps - 1))

    wait(*inputs)
    stream(bulk(*w_down))
    norm_pass(0, _norm_mean(x_ref, xp_ref, tally), 4 * NG // MEAN_GROUPS, True)
    for p, j in itertools.product(range(4), range(4)):
        stat_ref[0, p, j] = _average(kr_ref[p, j, _rows(0, 8), :])
        stat_ref[1, p, j] = _round_bf16(stat_ref[0, p, j])
    norm_pass(1, _norm_centre(xp_ref, cen_ref, stat_ref, tally), 16 * NG // VAR_GROUPS, True)
    for p, j in itertools.product(range(4), range(4)):
        stat_ref[0, p, j] = _norm_factor(kr_ref[p, j, _rows(1, 8), :], stat_ref[0, p, j])
    wait(whole(*w_gate))
    stream(bulk(*w_last))
    norm_pass(2, _norm_scale(wr_ref, cen_ref, stat_ref, work_ref), 20, False)

    def convolve(n):
        first, stop = CONV_CUTS[n:n + 2]
        steps = _convolve(first, stop, zero, kf_ref, fx_ref, fxt_ref, xf_ref, work_ref, y_ref)
        return with_trickle(steps, 4 * (stop - first), SHORT_PER_PHASE[3 + n])

    def ffn_down(i):
        return _ffn_down(*CHUNKS[i], h_ref, wd_ref, gate_ref, upd_ref)

    def gate_and_send(chunk):
        for row, col in _gate(*chunk, upd_ref, hot_ref, xp_ref, work_ref, y_ref, skip_ref,
                              o_ref):
            if row in FINE_ROWS:
                copy(o_ref, o_hbm, 1, (row, 64), (col, 512)).start()
            elif col + 512 == L:
                copy(o_ref, o_hbm, 1, (row, 64)).start()
            yield

    _weave(convolve(0), itertools.chain(
        _route(stat_ref, work_ref, hot_ref, xs_ref, gate_ref),
        _ffn_up(False, xs_ref, wg_ref, h_ref)))
    wait(whole(*w_up))
    _column(dsk_ref, skip_ref, lambda v: 2.0 * v)
    _weave(convolve(1), _ffn_up(True, xs_ref, wu_ref, h_ref))
    wait(whole(*w_down))
    _weave(convolve(2), ffn_down(0))
    for i, chunk in enumerate(CHUNKS):
        if chunk[0] + chunk[1] == late:
            wait(whole(*w_last))
        _weave(gate_and_send(chunk),
               ffn_down(i + 1) if i + 1 < len(CHUNKS) else iter(()), DOWN_RATE)
    wait(copy(o_ref, o_hbm, 1))


@jax.jit
def pallas_recurrent_scan__ssm_conv_s4__moe_arch_mod__prompt_kernel(
    A_u: jax.Array,
    A_A_re: jax.Array,
    A_A_im: jax.Array,
    A_B_re: jax.Array,
    A_B_im: jax.Array,
    A_C_re: jax.Array,
    A_C_im: jax.Array,
    A_log_dt: jax.Array,
    A_Dskip: jax.Array,
    B_x: jax.Array,
    B_w_r: jax.Array,
    B_w_gate: jax.Array,
    B_w_up: jax.Array,
    B_w_down: jax.Array,
):
    del B_x
    assert A_u.shape == (1, L, D) and A_A_re.shape == (D, N) and B_w_gate.shape == (D, F)
    assert A_A_re.dtype == BF16
    vmem = pltpu.VMEM
    scratch = [
        vmem((D, L), BF16), vmem((6, D, N), BF16),
        vmem((D,), BF16), vmem((D,), BF16), vmem((D,), BF16),
        vmem((D, F), BF16), vmem((D, F), BF16), vmem((D, F), BF16), vmem((D, L), BF16),
        vmem((4, 2, 64, 128), I32), vmem((4, 128, 128), I32),
        vmem((4, 2, 64, 128), I32), vmem((4, 2, 64, 128), I32),
        vmem((D, 128), F32), vmem((D, 128), F32),
        vmem((4, 2, 144, 128), F32), vmem((4, 2, 96, 128), F32),
        vmem((NH + 4, 5, 16, 128), F32), vmem((4 * NH, 8, 8, 128), F32),
        vmem((4, 4, D // 2, 128), I32), vmem((2, 4, 4, 8, 128), F32),
        vmem((4, 4, NG, 8, 256), BF16),
        vmem((NH, 4, XN + 4, 8, 128), F32), vmem((4 * NH, 8, 8, 128), F32),
        vmem((NH, 4, 4, 8, 128), F32),
        vmem((16, 8, 128), F32), vmem((8, D), F32), vmem((8, 128), F32), vmem((8, F), F32),
        vmem((D, TOPK), F32),
        pltpu.SemaphoreType.DMA((3,)),
    ]
    out = pl.pallas_call(
        _kernel,
        out_shape=jax.ShapeDtypeStruct((D, L), BF16),
        in_specs=[pl.BlockSpec(memory_space=pl.ANY)] * 13,
        out_specs=pl.BlockSpec(memory_space=pl.ANY),
        scratch_shapes=scratch,
        compiler_params=pltpu.CompilerParams(vmem_limit_bytes=100 * 1024 * 1024),
    )(A_u[0].T, A_A_re, A_A_im, A_B_re, A_B_im, A_C_re, A_C_im, A_log_dt, A_Dskip,
      B_w_r, B_w_gate, B_w_up, B_w_down.T)
    return out.T[None]
```

```python
import itertools
import math

import jax
import jax.numpy as jnp
from jax import lax
import jax.experimental.pallas as pl
import jax.experimental.pallas.tpu as pltpu

F32, BF16, I32 = jnp.float32, jnp.bfloat16, jnp.int32
L, D, N, F, TOPK = 2048, 576, 128, 4608, 8
EPS = 1e-5
G = 16
NG = D // G
NH = D // 8
NN = (((1,), (0,)), ((), ()))
NT = (((1,), (1,)), ((), ()))

SSM_UNROLL = 8
NORM_SHARE = ((24, 2), (30, 3), (18, 3))
MEAN_GROUPS, VAR_GROUPS = 3, 6
CONV_CUTS = (0, 21, 33, NG + 3)
CHUNKS = ((0, 128), (128, 128), (256, 128), (384, 128), (512, 64))
SHORT_PER_WEIGHT = (43, 22, 10, 4)
SHORT_PER_PHASE = (5, 6, 5, 17, 10, 0)
assert sum(SHORT_PER_WEIGHT) == NG + sum(SHORT_PER_PHASE)
DOWN_RATE, PAUSE = 2.0, 3


def _iota(shape, dim):
    return lax.broadcasted_iota(I32, shape, dim)


def _rows(i, n):
    return pl.ds(i * n if isinstance(i, int) else pl.multiple_of(i * n, n), n)


def _cat(xs, axis=0):
    return jnp.concatenate(xs, axis=axis)


def _cmul(a, b):
    return a[0] * b[0] - a[1] * b[1], a[0] * b[1] + a[1] * b[0]


def _csq(a):
    return a[0] * a[0] - a[1] * a[1], (a[0] + a[0]) * a[1]


def _cadd(a, b):
    return a[0] + b[0], a[1] + b[1]


def _csub(a, b):
    return a[0] - b[0], a[1] - b[1]


def _cadd_i(a, b):
    return a[0] - b[1], a[1] + b[0]


def _csub_i(a, b):
    return a[0] + b[1], a[1] - b[0]


def _dft4(v):
    s02, d02 = _cadd(v[0], v[2]), _csub(v[0], v[2])
    s13, d13 = _cadd(v[1], v[3]), _csub(v[1], v[3])
    return [_cadd(s02, s13), _cadd_i(d02, d13), _csub(s02, s13), _csub_i(d02, d13)]


def _root(n):
    ang = (((n + 1024) & 2047) - 1024).astype(F32) * (2.0 * math.pi / 2048)
    return jnp.cos(ang), jnp.sin(ang)


def _powers(start, step, count):
    vals = [start]
    for _ in range(count - 1):
        vals.append(_cmul(vals[-1], step))
    return vals


def _pack(x):
    return pltpu.bitcast(x.astype(BF16), I32)


def _bf(x):
    return pltpu.bitcast(x, BF16)


def _round_bf16(x):
    return x.astype(BF16).astype(F32)


def _silu_of_twice(h):
    return h + h * jnp.tanh(h)


def _mm(a, b, dims=NN):
    return lax.dot_general(a, b, dims, precision=lax.Precision.DEFAULT,
                           preferred_element_type=F32)


def _skew(r):
    lane = _iota(r[0].shape, 1)
    b0, b1 = (lane & 1) != 0, (lane & 2) != 0
    t = [lax.select(b0, r[(k + 1) % 4], r[k]) for k in range(4)]
    u = [lax.select(b1, t[(k + 2) % 4], t[k]) for k in range(4)]
    return [u[(-j) % 4] for j in range(4)]


def _x_time(j, m):
    q = (m - j) & 3
    return 128 * q + ((m - q) & 127)


def _weave(main, side, rate=1.0):
    credit = 0.0
    for _ in main:
        credit += rate
        while credit >= 1.0:
            credit -= 1.0
            next(side, None)
    for _ in side:
        pass


def _column(v_ref, out_ref, fn):
    v = fn(v_ref[...].astype(F32).reshape(1, D))
    for lo in range(0, D, 128):
        n = min(128, D - lo)
        out_ref[pl.ds(lo, n), :] = jnp.broadcast_to(v[:, lo:lo + n], (128, n)).T


def _input_transform(fx_ref, fxt_ref):
    freq, row = 4 * _iota((8, 128), 1) + 1, _iota((8, 128), 0)
    step8 = _root(8 * freq)
    step128 = _csq(_csq(_csq(_csq(step8))))
    for j in range(4):
        start = _root((_x_time(j, row + 8) - 8) * freq)
        vals = _powers(start, step8, 16)
        wraps = row < ((row - j) & 3)
        vals[0] = tuple(jnp.where(wraps, a, b) for a, b in zip(_cmul(start, step128), start))
        for part in range(2):
            m = _cat([v[part] for v in vals])
            fx_ref[j, part] = _pack(m)
            fxt_ref[j, pl.ds(64 * part, 64), :] = _pack(m.T)


def _kernel_transform(fk_ref, fd_ref):
    freq, row = 4 * _iota((8, 128), 1) + 1, _iota((8, 128), 0)
    rho = _root(freq)
    step32 = _csq(_csq(_csq(_csq(_csq(rho)))))
    for j, start in enumerate(_powers(_root(4 * row * freq), rho, 4)):
        vals = _powers(start, step32, 16)
        for part in range(2):
            fk_ref[j, part] = _pack(_cat([v[part] for v in vals]))
    rows = _powers(_root((256 * (row & 1) + 8 * (row >> 1)) * freq), step32, 8)
    first = row == 0
    for k in range(4):
        p2 = _csq(rho)
        s3 = _cadd(_cadd(rho, p2), _cmul(p2, rho))
        s4 = _cadd(s3, _csq(p2))
        box = 1.0 + 2.0 * jnp.where((row & 2) == 0, s4[0], s3[0])
        vals = [(r[0] * box, r[1] * box) for r in rows]
        vals[0] = (jnp.where(first, 1.0 + s4[0], vals[0][0]),
                   jnp.where(first, s4[1], vals[0][1]))
        vals.append((jnp.where(first, s4[1], 0.0), jnp.where(first, s4[0], 0.0)))
        for part in range(2):
            fd_ref[k, part, pl.ds(0, 40), :] = _pack(
                _cat([v[part] for v in vals] + [jnp.zeros((8, 128), F32)]))
            fd_ref[k, part, pl.ds(40, 24), :] = jnp.zeros((24, 128), I32)
        rho = (-rho[1], rho[0])


def _ssm_bases(g, h, par_ref, dt_ref, base_ref):
    a_re, a_im, b_re, b_im, c_re, c_im = (
        par_ref[k, _rows(g, G), :].astype(F32) for k in range(6))
    dt = dt_ref[_rows(g, G), :]
    dts = dt * (2.0 / 512)
    row = _iota((8, 128), 0)

    def deal(v):
        return _cat([jnp.take_along_axis(v[lo:lo + 8], (row >> 1) + 4 * (row & 1), axis=0,
                                         mode="promise_in_bounds") for lo in (0, 8)])

    decay, phase = deal(dt * a_re), deal(dt * a_im)
    w = tuple(deal(v) for v in _cmul((c_re, c_im), (dts * b_re, dts * b_im)))
    z, unit = {}, (jnp.cos(phase), jnp.sin(phase))
    for e in (1, 2, 4, 8, 16, 32, 64, 128, 256):
        if e in (1, 4, 8, 16, 256):
            mag = jnp.exp2(decay * (e * math.log2(math.e)))
            z[e] = (mag * unit[0], mag * unit[1])
        if e < 256:
            unit = _csq(unit)
    z1024 = _csq(_csq(z[256]))
    w8, w1024 = _cmul(w, z[8]), _cmul(w, z1024)
    seq = [(jnp.ones_like(dt), jnp.zeros_like(dt)), z[8], z[16], z[16], _cmul(z[16], z[8]),
           z[1], z[1], z[256], z[256], w, _cmul(w, z[4]), w,
           w8, w1024, w8, w1024, _cmul(w1024, z1024), w1024]
    for k, v in enumerate(seq):
        for t in range(2):
            for part in range(2):
                base_ref[h + t, part, pl.ds(8 * k, 8), :] = v[part][8 * t:8 * t + 8]


_OFFSETS = ((0, 4), (1, 5), (2, 6), (3, 7), (258, 262), (256, 260), (512, 516), (768, 772),
            (264, 1280), (520, 1536), (776, 1792), (1024, 2048))


def _ssm_values(h, base_ref, kv_ref):
    for quad in range(2):
        def pair(k):
            return tuple(base_ref[h, part, pl.ds(8 * k + quad, 8, stride=2), :]
                         for part in range(2))

        v = [pair(0)] + _powers(pair(3), pair(2), 15)
        z256 = pair(7)
        w = _powers(pair(9 + quad), pair(5), 4)
        w += [_cmul(w[2], z256)] + _powers(w[0], z256, 4)[1:]
        w += _powers(pair(12 + quad), z256, 4)[1:] + [pair(15 + quad)]
        re, im = (_mm(_cat([t[part] for t in w]), _cat([t[part] for t in v[::-1]]), NT)
                  for part in range(2))
        kv_ref[h, quad] = re - im


def _ssm_arrange(h, slot, kv_ref, kr_ref):
    lane, row = _iota((8, 128), 1), _iota((8, 128), 0)
    src = 4 * (((lane >> 1) & 31) ^ 30) + (row & 3)
    top = row < 4

    def spread(x):
        return jnp.take_along_axis(x, src, axis=1, mode="promise_in_bounds")

    def even(a, b):
        return jnp.where((lane & 1) == 0, a, b)

    def low(a, b):
        return jnp.where(lane < 64, a, b)

    val = {}
    for u, (e0, e1) in enumerate(_OFFSETS):
        a, b = (kv_ref[h, quad, pl.ds(8 * u, 8), :] for quad in range(2))
        val[e0] = spread(jnp.where(top, a, b))
        val[e1] = spread(pltpu.roll(jnp.where(top, b, a), 4, 0))
    mid = even(val[256], val[260])
    q0, q4, q8 = low(val[512], val[768]), low(val[516], val[772]), low(val[520], val[776])
    blocks = [
        (low(even(val[0], val[4]), mid), even(q0, q4)),
        (low(even(val[1], val[5]), mid), even(q0, q4)),
        (low(even(val[2], val[6]), even(val[258], val[262])), even(q0, q8)),
        (low(even(val[3], val[7]), even(val[260], val[264])), even(q4, q8)),
        (low(even(val[1024], val[1280]), val[1536]),
         low(even(val[1536], val[1792]), jnp.where(lane == 64, val[2048], 0.0)))]
    for j, pair in enumerate(blocks):
        kr_ref[slot, j] = _cat(pair)


def _ssm_kernel(waits, every_group, par_ref, dt_ref, base_ref, kv_ref, kr_ref):
    def step(g, slot, ahead=True):
        for t in range(2):
            _ssm_arrange(slot + t, 2 * g + t, kv_ref, kr_ref)
            _ssm_values(slot + t, base_ref, kv_ref)
        every_group(g, kv_ref[slot, 0, pl.ds(0, 8), :])
        if ahead:
            _ssm_bases(g + 2, slot, par_ref, dt_ref, base_ref)

    def body(n, zero):
        pl.when(n == 1)(waits[0])
        for r in range(SSM_UNROLL):
            step(n * SSM_UNROLL + r, 2 * (r % 2))
        return jnp.minimum(zero, n * L)

    for g in range(2):
        _ssm_bases(g, 2 * g, par_ref, dt_ref, base_ref)
    kv_ref[...] = jnp.zeros_like(kv_ref)
    trips = (NG - 2) // SSM_UNROLL
    zero = lax.fori_loop(0, trips, body, L)
    waits[1]()
    for g in range(trips * SSM_UNROLL, NG):
        step(g, 2 * (g % 2), g + 2 < NG)
    for h in range(4):
        _ssm_arrange(h, NH + h, kv_ref, kr_ref)
    return zero


def _ssm_spectrum(first, count, batch, fine, kr_ref, fk_ref, fd_ref, kf_ref):
    def blocks(x):
        x = x.reshape(batch, 2, 1, 8, 128)
        return x[:, :1], x[:, 1:]

    recent = jnp.zeros((8, 128), F32)
    for h0 in range(first, first + count, batch):
        near, far = [], []
        for n in range(4):
            lhs = {j: [] for j in ((0, 1, 2, 3) if n < 2 else (4,))}
            for h in range(h0, h0 + batch):
                for j, rows in lhs.items():
                    rows.append(kr_ref[4 + h, j])
                if fine:
                    yield recent
            if n < 2:
                near.append([_mm(_cat(lhs[j]), _bf(fk_ref[j, n])) for j in range(4)])
            else:
                far += [[_mm(_cat(lhs[4]), _bf(fd_ref[k, part])) for part in range(2)]
                        for k in (2 * n - 4, 2 * n - 3)]
            recent = (far or near)[-1][0]
            if not fine:
                yield recent
        out = []
        for a, b in zip(_dft4(list(zip(*near))), far):
            spec = list(zip(*(blocks(a[part]) + blocks(b[part]) for part in range(2))))
            spec = spec[:1] + [_csub_i(spec[p], spec[p - 1]) for p in range(1, 4)]
            out += [_cat(v, 1) for v in zip(*spec)]
        kf_ref[pl.ds(4 * h0, 4 * batch)] = _cat(out, 2).reshape(4 * batch, 8, 8, 128)


XN = 8


def _fold(x):
    x = x.reshape(3, -1, 8, 128)
    x = x[0] + x[1] + x[2]
    while x.shape[0] > 1:
        x = x[:x.shape[0] // 2] + x[x.shape[0] // 2:]
    return x[0]


def _norm_mean(x_ref, xp_ref, tally):
    for p in range(4):
        for i in range(NG // MEAN_GROUPS):
            r = [pltpu.bitcast(x_ref[_rows(i, MEAN_GROUPS * G), _rows(4 * p + q, 128)], I32)
                 for q in range(4)]
            r = _skew([r[0]] + [pltpu.roll(r[q], q, 1) for q in range(1, 4)])
            for j in range(4):
                xp_ref[p, j, _rows(i, MEAN_GROUPS * 8), :] = r[j]
                tally(p, j, 0, _fold(_bf(r[j]).astype(F32)), i == 0)
            yield


def _norm_centre(xp_ref, cen_ref, stat_ref, tally):
    for i in range(NG // VAR_GROUPS):
        for p, j in itertools.product(range(4), range(4)):
            x = _bf(xp_ref[p, j, _rows(i, VAR_GROUPS * 8), :]).astype(F32)
            d = x.reshape(VAR_GROUPS, G, 128) - _cat([stat_ref[1, p, j]] * 2)
            cen_ref[p, j, _rows(i, VAR_GROUPS)] = _cat([d[:, :8], d[:, 8:]], 2).astype(BF16)
            tally(p, j, 1, _fold(d * d), i == 0)
            yield


def _average(v):
    return jnp.broadcast_to(jnp.sum(v, axis=0, keepdims=True), v.shape) / D


def _norm_factor(squares, mean):
    shift = mean - _round_bf16(mean)
    var = _round_bf16(jnp.maximum(_average(squares) - shift * shift, 0.0))
    eps = _round_bf16(jnp.full_like(var, EPS))
    return 0.5 / _round_bf16(jnp.sqrt(_round_bf16(var + eps)))


def _norm_scale(wr_ref, cen_ref, stat_ref, work_ref):
    wr = jnp.broadcast_to(2.0 * wr_ref[...].astype(F32).reshape(1, D), (8, D))
    for p in range(4):
        score = [None] * 4
        for lo in range(0, D, 128):
            n = min(128, D - lo)
            for j in range(4):
                d = cen_ref[p, j, pl.ds(lo // G, n // G)].astype(F32)
                half = _cat([d[:, :, :128], d[:, :, 128:]], 1).reshape(n // 8, 8, 128)
                half = half * stat_ref[0, p, j]
                work_ref[pl.ds(lo // 8, n // 8), p, XN + j] = half
                part = _mm(wr[:, lo:lo + n], half.reshape(n, 128))
                score[j] = part if lo == 0 else score[j] + part
            yield
        for j in range(4):
            stat_ref[1, p, j] = score[j]


def _route(stat_ref, work_ref, hot_ref, xs_ref, gate_ref):
    row, blk = _iota((8, 128), 0), _iota((16, 128), 0)
    halves = []
    for lo in (0, 2):
        dense = stat_ref[1, lo, 0]
        for c in range(1, 8):
            dense = jnp.where(row == c, stat_ref[1, lo + c // 4, c % 4], dense)
        halves.append(dense)
    score = _round_bf16(_cat(halves))
    bits = pltpu.bitcast(jnp.where(score == 0.0, 0.0, score), I32) >> 16
    order = jnp.where(bits < 0, bits ^ 0x7FFF, bits) + 0x8000
    time = 512 * (blk >> 2) + _x_time(blk & 3, _iota((16, 128), 1))
    key = pltpu.bitcast((1 << 29) + (order << 11) + (L - 1 - time), F32)
    rank = jnp.full((16, 128), TOPK, I32)
    best = jnp.zeros((8, 128), F32)
    for i in range(TOPK):
        top = jnp.max(jnp.max(key, axis=0, keepdims=True), axis=1, keepdims=True)
        hit = key == top
        rank = jnp.where(hit, i, rank)
        key = jnp.where(hit, 0.0, key)
        best = jnp.where(row == i, top, best)
        yield from range(2)
    order = ((pltpu.bitcast(best, I32) >> 11) & 0xFFFF) - 0x8000
    best = pltpu.bitcast(jnp.where(order < 0, order ^ 0x7FFF, order) << 16, F32)
    gate_ref[...] = 0.5 * _round_bf16(jax.nn.sigmoid(best))
    for c in range(16):
        hot_ref[c] = jnp.where(jnp.broadcast_to(rank[c:c + 1], (8, 128)) == row, 1.0, 0.0)
    for lo in range(0, D, 128):
        n, picked = min(128, D - lo), None
        for p in range(4):
            for j in range(4):
                tokens = work_ref[pl.ds(lo // 8, n // 8), p, XN + j]
                part = _mm(hot_ref[4 * p + j], tokens.reshape(n, 128), NT)
                picked = part if picked is None else picked + part
            yield
        xs_ref[:, pl.ds(lo, n)] = 2.0 * picked
    yield from range(2)


def _ffn_up(second, xs_ref, w_ref, h_ref):
    for col in range(0, F, 512):
        acc = None
        for lo in range(0, D, 128):
            rows = pl.ds(lo, min(128, D - lo))
            part = _mm(xs_ref[:, rows], w_ref[rows, pl.ds(col, 512)])
            acc = part if lo == 0 else acc + part
            yield
        acc = _round_bf16(acc)
        h_ref[:, pl.ds(col, 512)] = (h_ref[:, pl.ds(col, 512)] * acc if second
                                     else _round_bf16(_silu_of_twice(0.5 * acc)))


def _ffn_down(lo, n, h_ref, wd_ref, gate_ref, upd_ref):
    ffn = None
    for k in range(0, F, 512):
        part = _mm(h_ref[:, pl.ds(k, 512)], wd_ref[pl.ds(lo, n), pl.ds(k, 512)], NT)
        ffn = part if ffn is None else ffn + part
        yield
    yield from range(PAUSE)
    eye = jnp.where(_iota((n, n), 0) == _iota((n, n), 1), 1.0, 0.0)
    upd_ref[pl.ds(lo, n), :] = _mm(eye, _round_bf16(ffn) * gate_ref[:, :n], NT)


def _convolve(start, stop, zero, kf_ref, fx_ref, fxt_ref, xf_ref, work_ref, y_ref):
    def products(g):
        for h, k in itertools.product((2 * g, 2 * g + 1), range(4)):
            kf, x = ([tuple(ref[4 * h + p, 2 * k + part] for part in range(2))
                      for p in range(4)] for ref in (kf_ref, xf_ref))
            for c in (3, 0, 2, 1):
                acc = _cmul(kf[0], x[c])
                for p in range(1, c + 1):
                    acc = _cadd(acc, _cmul(kf[p], x[c - p]))
                for part in range(2):
                    work_ref[h + zero, c, 2 * k + part] = acc[part]
                if c < 2:
                    yield

    def operands(g, slots, fill):
        rows = []
        for h, p in itertools.product((2 * g, 2 * g + 1), range(4)):
            rows.append(work_ref[h, pl.ds(p, 1), slots])
            if p % 2:
                next(fill, None)
        rows = _cat(rows)
        return [rows[:, s].reshape(64, 128) for s in range(slots.size)]

    def butterflies(g, comp):
        spec = [v.reshape(8, 1, 8, 128) for pair in _dft4(list(zip(*comp))) for v in pair]
        xf_ref[pl.ds(8 * g + zero, 8)] = _cat(spec, 1)

    pending, recent = None, jnp.zeros((8, 128), F32)
    for i in range(start, stop):
        fill = products(i - 2) if 0 <= i - 2 < NG else iter(())
        for odd in range(2):
            if 0 <= i - 3:
                v = operands(i - 3, pl.ds(0, XN), fill)
                v = list(zip(v[0::2], v[1::2]))
                if odd:
                    a, b = _csub(v[0], v[2]), _csub(v[1], v[3])
                    back = _csub_i(a, b), _cadd_i(a, b)
                else:
                    a, b = _cadd(v[0], v[2]), _cadd(v[1], v[3])
                    back = _cadd(a, b), _csub(a, b)
                for j, spec in zip((odd, odd + 2), back):
                    recent = _mm(_cat(spec, 1), _bf(fxt_ref[j]))
                    y_ref[_rows(i - 3, 2), :, j] = recent.reshape(2, 4, 8, 128)
            yield recent
        if pending:
            butterflies(*pending)
        pending = (i, []) if i < NG else None
        for part in range(2):
            if pending:
                x = operands(i, pl.ds(XN, 4), fill)
                pending[1].append([_mm(x[j], _bf(fx_ref[j, part])) for j in range(4)])
                recent = pending[1][-1][0]
            yield recent
        for _ in fill:
            pass
    if pending:
        butterflies(*pending)


def _gate(lo, n, upd_ref, hot_ref, xp_ref, work_ref, y_ref, skip_ref, o_ref):
    for i in range(lo // 64, (lo + n) // 64):
        for p in range(4):
            r = []
            for j in range(4):
                x = _bf(xp_ref[p, j, _rows(i, 32), :]).astype(F32)
                half = work_ref[_rows(i, 8), p, XN + j].reshape(64, 128)
                s = (y_ref[_rows(i, 8), p, j].reshape(64, 128)
                     + half * skip_ref[_rows(i, 64), :])
                routed = _mm(upd_ref[_rows(i, 64), :], hot_ref[4 * p + j])
                r.append(x + s * _silu_of_twice(half + routed))
            r = _skew(r)
            r = [r[0]] + [pltpu.roll(r[q], 128 - q, 1) for q in range(1, 4)]
            o_ref[_rows(i, 64), _rows(p, 512)] = _cat(r, 1).astype(BF16)
            yield 64 * i, 512 * p


def _kernel(x_hbm, are_hbm, aim_hbm, bre_hbm, bim_hbm, cre_hbm, cim_hbm, ldt_hbm, dsk_hbm,
            wr_hbm, wg_hbm, wu_hbm, wd_hbm, o_hbm,
            x_ref, par_ref, ldt_ref, dsk_ref, wr_ref, wg_ref, wu_ref, wd_ref, o_ref,
            fx_ref, fxt_ref, fk_ref, fd_ref, dt_ref, skip_ref, base_ref, kv_ref, kr_ref,
            kf_ref, xp_ref, stat_ref, cen_ref, work_ref, xf_ref, y_ref,
            hot_ref, xs_ref, gate_ref, h_ref, upd_ref, sems):
    def copy(src, dst, sem, *part):
        if part:
            part = tuple(pl.ds(*p) for p in part)
            src, dst = src.at[part], dst.at[part]
        return pltpu.make_async_copy(src, dst, sems.at[sem])

    def params(sem, rows):
        return [copy(src, par_ref.at[i], sem, rows) for i, src in
                enumerate((are_hbm, aim_hbm, bre_hbm, bim_hbm, cre_hbm, cim_hbm))]

    def stream(*copies):
        for cp in copies:
            cp.start(priority=1)

    def wait(*copies):
        for cp in copies:
            cp.wait()

    def trickle(src, dst, sem, i, recent):
        dst[_rows(i, 8), pl.ds(0, 128)] = recent[:8].astype(BF16)
        copy(src.at[_rows(i, 8)], dst.at[_rows(i, 8)], sem).start()

    def with_trickle(jobs, count, pieces):
        due = [k * count // pieces for k in range(pieces)]
        for n, recent in enumerate(jobs):
            if n in due:
                trickle(*next(short), recent)
            yield

    def bulk(src, dst, sem, lo, hi, pieces):
        return copy(src, dst, sem, (lo + 8 * pieces, hi - lo - 8 * pieces))

    def whole(src, dst, sem, lo, hi, pieces):
        return copy(src, dst, sem, (lo, hi - lo))

    early, late = (SSM_UNROLL + 2) * G, CHUNKS[3][0]
    w_gate, w_up, w_down, w_last = weights = [w + (n,) for w, n in zip(
        ((wg_hbm, wg_ref, 0, 0, D), (wu_hbm, wu_ref, 1, 0, D),
         (wd_hbm, wd_ref, 2, 0, late), (wd_hbm, wd_ref, 0, late, D)), SHORT_PER_WEIGHT)]
    short = iter([(*w[:3], w[3] // 8 + i) for w in weights for i in range(w[5])][NG:])
    head = [copy(ldt_hbm, ldt_ref, 0)] + params(0, (0, early))
    rest = params(1, (early, D - early))
    inputs = [copy(x_hbm, x_ref, 2), copy(wr_hbm, wr_ref, 2), copy(dsk_hbm, dsk_ref, 2)]

    def wait_rest():
        wait(*rest)
        stream(bulk(*w_up))

    def wait_inputs():
        wait(*inputs)
        stream(bulk(*w_down))

    stream(*head, *rest, *inputs)
    _kernel_transform(fk_ref, fd_ref)
    _input_transform(fx_ref, fxt_ref)
    wait(*head)
    stream(bulk(*w_gate))
    _column(ldt_ref, dt_ref, lambda v: _round_bf16(jnp.exp(v)))
    zero = _ssm_kernel((wait_rest, wait_inputs), lambda *a: trickle(*w_gate[:3], *a),
                       par_ref, dt_ref, base_ref, kv_ref, kr_ref)

    def tally(p, j, n, value, first):
        kr_ref[p + zero, j, _rows(n, 8), :] = (
            value if first else kr_ref[p, j, _rows(n, 8), :] + value)

    def norm_pass(n, job, pieces, fine):
        count, batch = NORM_SHARE[n]
        first = sum(share[0] for share in NORM_SHARE[:n])
        steps = 4 * count // (1 if fine else batch)
        main = _ssm_spectrum(first, count, batch, fine, kr_ref, fk_ref, fd_ref, kf_ref)
        _weave(with_trickle(main, steps, SHORT_PER_PHASE[n]), job, pieces / (steps - 1))

    norm_pass(0, _norm_mean(x_ref, xp_ref, tally), 4 * NG // MEAN_GROUPS, True)
    for p, j in itertools.product(range(4), range(4)):
        stat_ref[0, p, j] = _average(kr_ref[p, j, _rows(0, 8), :])
        stat_ref[1, p, j] = _round_bf16(stat_ref[0, p, j])
    pl.when(zero < NG)(lambda: norm_pass(
        1, _norm_centre(xp_ref, cen_ref, stat_ref, tally), 16 * NG // VAR_GROUPS, True))
    for p, j in itertools.product(range(4), range(4)):
        stat_ref[0, p, j] = _norm_factor(kr_ref[p, j, _rows(1, 8), :], stat_ref[0, p, j])
    wait(whole(*w_gate))
    stream(bulk(*w_last))
    norm_pass(2, _norm_scale(wr_ref, cen_ref, stat_ref, work_ref), 20, False)

    def convolve(n):
        first, stop = CONV_CUTS[n:n + 2]
        steps = _convolve(first, stop, zero, kf_ref, fx_ref, fxt_ref, xf_ref, work_ref, y_ref)
        return with_trickle(steps, 4 * (stop - first), SHORT_PER_PHASE[3 + n])

    def ffn_down(i):
        return _ffn_down(*CHUNKS[i], h_ref, wd_ref, gate_ref, upd_ref)

    def gate_and_send(chunk):
        for row, col in _gate(*chunk, upd_ref, hot_ref, xp_ref, work_ref, y_ref, skip_ref,
                              o_ref):
            stream(copy(o_ref, o_hbm, 1, (row, 64), (col, 512)))
            yield

    _weave(convolve(0), itertools.chain(
        _route(stat_ref, work_ref, hot_ref, xs_ref, gate_ref),
        _ffn_up(False, xs_ref, wg_ref, h_ref)))
    wait(whole(*w_up))
    _column(dsk_ref, skip_ref, lambda v: 2.0 * v)
    _weave(convolve(1), _ffn_up(True, xs_ref, wu_ref, h_ref))
    wait(whole(*w_down))
    _weave(convolve(2), ffn_down(0))
    for i, chunk in enumerate(CHUNKS):
        if chunk[0] + chunk[1] == late:
            wait(whole(*w_last))
        _weave(gate_and_send(chunk),
               ffn_down(i + 1) if i + 1 < len(CHUNKS) else iter(()), DOWN_RATE)
    wait(copy(o_ref, o_hbm, 1))


@jax.jit
def pallas_recurrent_scan__ssm_conv_s4__moe_arch_mod__prompt_kernel(
    A_u: jax.Array,
    A_A_re: jax.Array,
    A_A_im: jax.Array,
    A_B_re: jax.Array,
    A_B_im: jax.Array,
    A_C_re: jax.Array,
    A_C_im: jax.Array,
    A_log_dt: jax.Array,
    A_Dskip: jax.Array,
    B_x: jax.Array,
    B_w_r: jax.Array,
    B_w_gate: jax.Array,
    B_w_up: jax.Array,
    B_w_down: jax.Array,
):
    del B_x
    assert A_u.shape == (1, L, D) and A_A_re.shape == (D, N) and B_w_gate.shape == (D, F)
    assert A_A_re.dtype == BF16
    vmem = pltpu.VMEM
    scratch = [
        vmem((D, L), BF16), vmem((6, D, N), BF16),
        vmem((D,), BF16), vmem((D,), BF16), vmem((D,), BF16),
        vmem((D, F), BF16), vmem((D, F), BF16), vmem((D, F), BF16), vmem((D, L), BF16),
        vmem((4, 2, 64, 128), I32), vmem((4, 128, 128), I32),
        vmem((4, 2, 64, 128), I32), vmem((4, 2, 64, 128), I32),
        vmem((D, 128), F32), vmem((D, 128), F32),
        vmem((4, 2, 144, 128), F32), vmem((4, 2, 96, 128), F32),
        vmem((NH + 4, 5, 16, 128), F32), vmem((4 * NH, 8, 8, 128), F32),
        vmem((4, 4, D // 2, 128), I32), vmem((2, 4, 4, 8, 128), F32),
        vmem((4, 4, NG, 8, 256), BF16),
        vmem((NH, 4, XN + 4, 8, 128), F32), vmem((4 * NH, 8, 8, 128), F32),
        vmem((NH, 4, 4, 8, 128), F32),
        vmem((16, 8, 128), F32), vmem((8, D), F32), vmem((8, 128), F32), vmem((8, F), F32),
        vmem((D, TOPK), F32),
        pltpu.SemaphoreType.DMA((3,)),
    ]
    out = pl.pallas_call(
        _kernel,
        out_shape=jax.ShapeDtypeStruct((D, L), BF16),
        in_specs=[pl.BlockSpec(memory_space=pl.ANY)] * 13,
        out_specs=pl.BlockSpec(memory_space=pl.ANY),
        scratch_shapes=scratch,
        compiler_params=pltpu.CompilerParams(vmem_limit_bytes=100 * 1024 * 1024),
    )(A_u[0].T, A_A_re, A_A_im, A_B_re, A_B_im, A_C_re, A_C_im, A_log_dt, A_Dskip,
      B_w_r, B_w_gate, B_w_up, B_w_down.T)
    return out.T[None]
```

```python
import itertools
import math

import jax
import jax.numpy as jnp
from jax import lax
import jax.experimental.pallas as pl
import jax.experimental.pallas.tpu as pltpu

F32, BF16, I32 = jnp.float32, jnp.bfloat16, jnp.int32
L, D, N, F, TOPK = 2048, 576, 128, 4608, 8
EPS = 1e-5
G = 16
NG = D // G
NH = D // 8
NN = (((1,), (0,)), ((), ()))
NT = (((1,), (1,)), ((), ()))

SSM_UNROLL = 8
NORM_SHARE = ((24, 2), (30, 3), (18, 3))
MEAN_GROUPS, VAR_GROUPS = 3, 6
CONV_CUTS = (0, 21, 33, NG + 3)
CHUNKS = ((0, 128), (128, 128), (256, 128), (384, 128), (512, 64))
SHORT_PER_WEIGHT = (43, 22, 10, 4)
SHORT_PER_PHASE = (5, 6, 5, 17, 10, 0)
assert sum(SHORT_PER_WEIGHT) == NG + sum(SHORT_PER_PHASE)
DOWN_RATE, PAUSE = 2.0, 3


def _iota(shape, dim):
    return lax.broadcasted_iota(I32, shape, dim)


def _rows(i, n):
    return pl.ds(i * n if isinstance(i, int) else pl.multiple_of(i * n, n), n)


def _cat(xs, axis=0):
    return jnp.concatenate(xs, axis=axis)


def _cmul(a, b):
    return a[0] * b[0] - a[1] * b[1], a[0] * b[1] + a[1] * b[0]


def _csq(a):
    return a[0] * a[0] - a[1] * a[1], (a[0] + a[0]) * a[1]


def _cadd(a, b):
    return a[0] + b[0], a[1] + b[1]


def _csub(a, b):
    return a[0] - b[0], a[1] - b[1]


def _cadd_i(a, b):
    return a[0] - b[1], a[1] + b[0]


def _csub_i(a, b):
    return a[0] + b[1], a[1] - b[0]


def _dft4(v):
    s02, d02 = _cadd(v[0], v[2]), _csub(v[0], v[2])
    s13, d13 = _cadd(v[1], v[3]), _csub(v[1], v[3])
    return [_cadd(s02, s13), _cadd_i(d02, d13), _csub(s02, s13), _csub_i(d02, d13)]


def _root(n):
    ang = (((n + 1024) & 2047) - 1024).astype(F32) * (2.0 * math.pi / 2048)
    return jnp.cos(ang), jnp.sin(ang)


def _powers(start, step, count):
    vals = [start]
    for _ in range(count - 1):
        vals.append(_cmul(vals[-1], step))
    return vals


def _pack(x):
    return pltpu.bitcast(x.astype(BF16), I32)


def _bf(x):
    return pltpu.bitcast(x, BF16)


def _round_bf16(x):
    return x.astype(BF16).astype(F32)


def _silu_of_twice(h):
    return h + h * jnp.tanh(h)


def _mm(a, b, dims=NN):
    return lax.dot_general(a, b, dims, precision=lax.Precision.DEFAULT,
                           preferred_element_type=F32)


def _skew(r):
    lane = _iota(r[0].shape, 1)
    b0, b1 = (lane & 1) != 0, (lane & 2) != 0
    t = [lax.select(b0, r[(k + 1) % 4], r[k]) for k in range(4)]
    u = [lax.select(b1, t[(k + 2) % 4], t[k]) for k in range(4)]
    return [u[(-j) % 4] for j in range(4)]


def _x_time(j, m):
    q = (m - j) & 3
    return 128 * q + ((m - q) & 127)


def _weave(main, side, rate=1.0):
    credit = 0.0
    for _ in main:
        credit += rate
        while credit >= 1.0:
            credit -= 1.0
            next(side, None)
    for _ in side:
        pass


def _column(v_ref, out_ref, fn):
    v = fn(v_ref[...].astype(F32).reshape(1, D))
    for lo in range(0, D, 128):
        n = min(128, D - lo)
        out_ref[pl.ds(lo, n), :] = jnp.broadcast_to(v[:, lo:lo + n], (128, n)).T


def _input_transform(fx_ref, fxt_ref):
    freq, row = 4 * _iota((8, 128), 1) + 1, _iota((8, 128), 0)
    step8 = _root(8 * freq)
    step128 = _csq(_csq(_csq(_csq(step8))))
    for j in range(4):
        start = _root((_x_time(j, row + 8) - 8) * freq)
        vals = _powers(start, step8, 16)
        wraps = row < ((row - j) & 3)
        vals[0] = tuple(jnp.where(wraps, a, b) for a, b in zip(_cmul(start, step128), start))
        for part in range(2):
            m = _cat([v[part] for v in vals])
            fx_ref[j, part] = _pack(m)
            fxt_ref[j, pl.ds(64 * part, 64), :] = _pack(m.T)


def _kernel_transform(fk_ref, fd_ref):
    freq, row = 4 * _iota((8, 128), 1) + 1, _iota((8, 128), 0)
    rho = _root(freq)
    step32 = _csq(_csq(_csq(_csq(_csq(rho)))))
    for j, start in enumerate(_powers(_root(4 * row * freq), rho, 4)):
        vals = _powers(start, step32, 16)
        for part in range(2):
            fk_ref[j, part] = _pack(_cat([v[part] for v in vals]))
    rows = _powers(_root((256 * (row & 1) + 8 * (row >> 1)) * freq), step32, 8)
    first = row == 0
    for k in range(4):
        p2 = _csq(rho)
        s3 = _cadd(_cadd(rho, p2), _cmul(p2, rho))
        s4 = _cadd(s3, _csq(p2))
        box = 1.0 + 2.0 * jnp.where((row & 2) == 0, s4[0], s3[0])
        vals = [(r[0] * box, r[1] * box) for r in rows]
        vals[0] = (jnp.where(first, 1.0 + s4[0], vals[0][0]),
                   jnp.where(first, s4[1], vals[0][1]))
        vals.append((jnp.where(first, s4[1], 0.0), jnp.where(first, s4[0], 0.0)))
        for part in range(2):
            fd_ref[k, part, pl.ds(0, 40), :] = _pack(
                _cat([v[part] for v in vals] + [jnp.zeros((8, 128), F32)]))
            fd_ref[k, part, pl.ds(40, 24), :] = jnp.zeros((24, 128), I32)
        rho = (-rho[1], rho[0])


def _ssm_bases(g, h, par_ref, dt_ref, base_ref):
    a_re, a_im, b_re, b_im, c_re, c_im = (
        par_ref[k, _rows(g, G), :].astype(F32) for k in range(6))
    dt = dt_ref[_rows(g, G), :]
    dts = dt * (2.0 / 512)
    row = _iota((8, 128), 0)

    def deal(v):
        return _cat([jnp.take_along_axis(v[lo:lo + 8], (row >> 1) + 4 * (row & 1), axis=0,
                                         mode="promise_in_bounds") for lo in (0, 8)])

    decay, phase = deal(dt * a_re), deal(dt * a_im)
    w = tuple(deal(v) for v in _cmul((c_re, c_im), (dts * b_re, dts * b_im)))
    z, unit = {}, (jnp.cos(phase), jnp.sin(phase))
    for e in (1, 2, 4, 8, 16, 32, 64, 128, 256):
        if e in (1, 4, 8, 16, 256):
            mag = jnp.exp2(decay * (e * math.log2(math.e)))
            z[e] = (mag * unit[0], mag * unit[1])
        if e < 256:
            unit = _csq(unit)
    z1024 = _csq(_csq(z[256]))
    w8, w1024 = _cmul(w, z[8]), _cmul(w, z1024)
    seq = [(jnp.ones_like(dt), jnp.zeros_like(dt)), z[8], z[16], z[16], _cmul(z[16], z[8]),
           z[1], z[1], z[256], z[256], w, _cmul(w, z[4]), w,
           w8, w1024, w8, w1024, _cmul(w1024, z1024), w1024]
    for k, v in enumerate(seq):
        for t in range(2):
            for part in range(2):
                base_ref[h + t, part, pl.ds(8 * k, 8), :] = v[part][8 * t:8 * t + 8]


_OFFSETS = ((0, 4), (1, 5), (2, 6), (3, 7), (258, 262), (256, 260), (512, 516), (768, 772),
            (264, 1280), (520, 1536), (776, 1792), (1024, 2048))


def _ssm_values(h, base_ref, kv_ref):
    for quad in range(2):
        def pair(k):
            return tuple(base_ref[h, part, pl.ds(8 * k + quad, 8, stride=2), :]
                         for part in range(2))

        v = [pair(0)] + _powers(pair(3), pair(2), 15)
        z256 = pair(7)
        w = _powers(pair(9 + quad), pair(5), 4)
        w += [_cmul(w[2], z256)] + _powers(w[0], z256, 4)[1:]
        w += _powers(pair(12 + quad), z256, 4)[1:] + [pair(15 + quad)]
        re, im = (_mm(_cat([t[part] for t in w]), _cat([t[part] for t in v[::-1]]), NT)
                  for part in range(2))
        kv_ref[h, quad] = re - im


def _ssm_arrange(h, slot, kv_ref, kr_ref):
    lane, row = _iota((8, 128), 1), _iota((8, 128), 0)
    src = 4 * (((lane >> 1) & 31) ^ 30) + (row & 3)
    top = row < 4

    def spread(x):
        return jnp.take_along_axis(x, src, axis=1, mode="promise_in_bounds")

    def even(a, b):
        return jnp.where((lane & 1) == 0, a, b)

    def low(a, b):
        return jnp.where(lane < 64, a, b)

    val = {}
    for u, (e0, e1) in enumerate(_OFFSETS):
        a, b = (kv_ref[h, quad, pl.ds(8 * u, 8), :] for quad in range(2))
        val[e0] = spread(jnp.where(top, a, b))
        val[e1] = spread(pltpu.roll(jnp.where(top, b, a), 4, 0))
    mid = even(val[256], val[260])
    q0, q4, q8 = low(val[512], val[768]), low(val[516], val[772]), low(val[520], val[776])
    blocks = [
        (low(even(val[0], val[4]), mid), even(q0, q4)),
        (low(even(val[1], val[5]), mid), even(q0, q4)),
        (low(even(val[2], val[6]), even(val[258], val[262])), even(q0, q8)),
        (low(even(val[3], val[7]), even(val[260], val[264])), even(q4, q8)),
        (low(even(val[1024], val[1280]), val[1536]),
         low(even(val[1536], val[1792]), jnp.where(lane == 64, val[2048], 0.0)))]
    for j, pair in enumerate(blocks):
        kr_ref[slot, j] = _cat(pair)


def _ssm_kernel(waits, every_group, par_ref, dt_ref, base_ref, kv_ref, kr_ref):
    def step(g, slot, ahead=True):
        for t in range(2):
            _ssm_arrange(slot + t, 2 * g + t, kv_ref, kr_ref)
            _ssm_values(slot + t, base_ref, kv_ref)
        every_group(g, kv_ref[slot, 0, pl.ds(0, 8), :])
        if ahead:
            _ssm_bases(g + 2, slot, par_ref, dt_ref, base_ref)

    def body(n, zero):
        pl.when(n == 1)(waits[0])
        for r in range(SSM_UNROLL):
            step(n * SSM_UNROLL + r, 2 * (r % 2))
        return jnp.minimum(zero, n * L)

    for g in range(2):
        _ssm_bases(g, 2 * g, par_ref, dt_ref, base_ref)
    kv_ref[...] = jnp.zeros_like(kv_ref)
    trips = (NG - 2) // SSM_UNROLL
    zero = lax.fori_loop(0, trips, body, L)
    waits[1]()
    for g in range(trips * SSM_UNROLL, NG):
        step(g, 2 * (g % 2), g + 2 < NG)
    for h in range(4):
        _ssm_arrange(h, NH + h, kv_ref, kr_ref)
    return zero


def _ssm_spectrum(first, count, batch, fine, kr_ref, fk_ref, fd_ref, kf_ref):
    def blocks(x):
        x = x.reshape(batch, 2, 1, 8, 128)
        return x[:, :1], x[:, 1:]

    recent = jnp.zeros((8, 128), F32)
    for h0 in range(first, first + count, batch):
        near, far = [], []
        for n in range(4):
            lhs = {j: [] for j in ((0, 1, 2, 3) if n < 2 else (4,))}
            for h in range(h0, h0 + batch):
                for j, rows in lhs.items():
                    rows.append(kr_ref[4 + h, j])
                if fine:
                    yield recent
            if n < 2:
                near.append([_mm(_cat(lhs[j]), _bf(fk_ref[j, n])) for j in range(4)])
            else:
                far += [[_mm(_cat(lhs[4]), _bf(fd_ref[k, part])) for part in range(2)]
                        for k in (2 * n - 4, 2 * n - 3)]
            recent = (far or near)[-1][0]
            if not fine:
                yield recent
        out = []
        for a, b in zip(_dft4(list(zip(*near))), far):
            spec = list(zip(*(blocks(a[part]) + blocks(b[part]) for part in range(2))))
            spec = spec[:1] + [_csub_i(spec[p], spec[p - 1]) for p in range(1, 4)]
            out += [_cat(v, 1) for v in zip(*spec)]
        kf_ref[pl.ds(4 * h0, 4 * batch)] = _cat(out, 2).reshape(4 * batch, 8, 8, 128)


XN = 8


def _fold(x):
    x = x.reshape(3, -1, 8, 128)
    x = x[0] + x[1] + x[2]
    while x.shape[0] > 1:
        x = x[:x.shape[0] // 2] + x[x.shape[0] // 2:]
    return x[0]


def _norm_mean(x_ref, xp_ref, tally):
    for p in range(4):
        for i in range(NG // MEAN_GROUPS):
            r = [pltpu.bitcast(x_ref[_rows(i, MEAN_GROUPS * G), _rows(4 * p + q, 128)], I32)
                 for q in range(4)]
            r = _skew([r[0]] + [pltpu.roll(r[q], q, 1) for q in range(1, 4)])
            for j in range(4):
                xp_ref[p, j, _rows(i, MEAN_GROUPS * 8), :] = r[j]
                tally(p, j, 0, _fold(_bf(r[j]).astype(F32)), i == 0)
            yield


def _norm_centre(xp_ref, cen_ref, stat_ref, tally):
    for i in range(NG // VAR_GROUPS):
        for p, j in itertools.product(range(4), range(4)):
            x = _bf(xp_ref[p, j, _rows(i, VAR_GROUPS * 8), :]).astype(F32)
            d = x.reshape(VAR_GROUPS, G, 128) - _cat([stat_ref[1, p, j]] * 2)
            cen_ref[p, j, _rows(i, VAR_GROUPS)] = _cat([d[:, :8], d[:, 8:]], 2).astype(BF16)
            tally(p, j, 1, _fold(d * d), i == 0)
            yield


def _average(v):
    return jnp.broadcast_to(jnp.sum(v, axis=0, keepdims=True), v.shape) / D


def _norm_factor(squares, mean):
    shift = mean - _round_bf16(mean)
    var = _round_bf16(jnp.maximum(_average(squares) - shift * shift, 0.0))
    eps = _round_bf16(jnp.full_like(var, EPS))
    return 0.5 / _round_bf16(jnp.sqrt(_round_bf16(var + eps)))


def _norm_scale(wr_ref, cen_ref, stat_ref, work_ref):
    wr = jnp.broadcast_to(2.0 * wr_ref[...].astype(F32).reshape(1, D), (8, D))
    for p in range(4):
        score = [None] * 4
        for lo in range(0, D, 128):
            n = min(128, D - lo)
            for j in range(4):
                d = cen_ref[p, j, pl.ds(lo // G, n // G)].astype(F32)
                half = _cat([d[:, :, :128], d[:, :, 128:]], 1).reshape(n // 8, 8, 128)
                half = half * stat_ref[0, p, j]
                work_ref[pl.ds(lo // 8, n // 8), p, XN + j] = half
                part = _mm(wr[:, lo:lo + n], half.reshape(n, 128))
                score[j] = part if lo == 0 else score[j] + part
            yield
        for j in range(4):
            stat_ref[1, p, j] = score[j]


def _route(stat_ref, work_ref, hot_ref, xs_ref, gate_ref):
    row, blk = _iota((8, 128), 0), _iota((16, 128), 0)
    halves = []
    for lo in (0, 2):
        dense = stat_ref[1, lo, 0]
        for c in range(1, 8):
            dense = jnp.where(row == c, stat_ref[1, lo + c // 4, c % 4], dense)
        halves.append(dense)
    score = _round_bf16(_cat(halves))
    bits = pltpu.bitcast(jnp.where(score == 0.0, 0.0, score), I32) >> 16
    order = jnp.where(bits < 0, bits ^ 0x7FFF, bits) + 0x8000
    time = 512 * (blk >> 2) + _x_time(blk & 3, _iota((16, 128), 1))
    key = pltpu.bitcast((1 << 29) + (order << 11) + (L - 1 - time), F32)
    rank = jnp.full((16, 128), TOPK, I32)
    best = jnp.zeros((8, 128), F32)
    for i in range(TOPK):
        top = jnp.max(jnp.max(key, axis=0, keepdims=True), axis=1, keepdims=True)
        hit = key == top
        rank = jnp.where(hit, i, rank)
        key = jnp.where(hit, 0.0, key)
        best = jnp.where(row == i, top, best)
        yield from range(2)
    order = ((pltpu.bitcast(best, I32) >> 11) & 0xFFFF) - 0x8000
    best = pltpu.bitcast(jnp.where(order < 0, order ^ 0x7FFF, order) << 16, F32)
    gate_ref[...] = 0.5 * _round_bf16(jax.nn.sigmoid(best))
    for c in range(16):
        hot_ref[c] = jnp.where(jnp.broadcast_to(rank[c:c + 1], (8, 128)) == row, 1.0, 0.0)
    for lo in range(0, D, 128):
        n, picked = min(128, D - lo), None
        for p in range(4):
            for j in range(4):
                tokens = work_ref[pl.ds(lo // 8, n // 8), p, XN + j]
                part = _mm(hot_ref[4 * p + j], tokens.reshape(n, 128), NT)
                picked = part if picked is None else picked + part
            yield
        xs_ref[:, pl.ds(lo, n)] = 2.0 * picked
    yield from range(2)


def _ffn_up(second, xs_ref, w_ref, h_ref):
    for col in range(0, F, 512):
        acc = None
        for lo in range(0, D, 128):
            rows = pl.ds(lo, min(128, D - lo))
            part = _mm(xs_ref[:, rows], w_ref[rows, pl.ds(col, 512)])
            acc = part if lo == 0 else acc + part
            yield
        acc = _round_bf16(acc)
        h_ref[:, pl.ds(col, 512)] = (h_ref[:, pl.ds(col, 512)] * acc if second
                                     else _round_bf16(_silu_of_twice(0.5 * acc)))


def _ffn_down(lo, n, h_ref, wd_ref, gate_ref, upd_ref):
    ffn = None
    for k in range(0, F, 512):
        part = _mm(h_ref[:, pl.ds(k, 512)], wd_ref[pl.ds(lo, n), pl.ds(k, 512)], NT)
        ffn = part if ffn is None else ffn + part
        yield
    yield from range(PAUSE)
    eye = jnp.where(_iota((n, n), 0) == _iota((n, n), 1), 1.0, 0.0)
    upd_ref[pl.ds(lo, n), :] = _mm(eye, _round_bf16(ffn) * gate_ref[:, :n], NT)


def _convolve(start, stop, zero, kf_ref, fx_ref, fxt_ref, xf_ref, work_ref, y_ref):
    def products(g):
        for h, k in itertools.product((2 * g, 2 * g + 1), range(4)):
            kf, x = ([tuple(ref[4 * h + p, 2 * k + part] for part in range(2))
                      for p in range(4)] for ref in (kf_ref, xf_ref))
            for c in (3, 0, 2, 1):
                acc = _cmul(kf[0], x[c])
                for p in range(1, c + 1):
                    acc = _cadd(acc, _cmul(kf[p], x[c - p]))
                for part in range(2):
                    work_ref[h + zero, c, 2 * k + part] = acc[part]
                if c < 2:
                    yield

    def operands(g, slots, fill):
        rows = []
        for h, p in itertools.product((2 * g, 2 * g + 1), range(4)):
            rows.append(work_ref[h, pl.ds(p, 1), slots])
            if p % 2:
                next(fill, None)
        rows = _cat(rows)
        return [rows[:, s].reshape(64, 128) for s in range(slots.size)]

    def butterflies(g, comp):
        spec = [v.reshape(8, 1, 8, 128) for pair in _dft4(list(zip(*comp))) for v in pair]
        xf_ref[pl.ds(8 * g + zero, 8)] = _cat(spec, 1)

    pending, recent = None, jnp.zeros((8, 128), F32)
    for i in range(start, stop):
        fill = products(i - 2) if 0 <= i - 2 < NG else iter(())
        for odd in range(2):
            if 0 <= i - 3:
                v = operands(i - 3, pl.ds(0, XN), fill)
                v = list(zip(v[0::2], v[1::2]))
                if odd:
                    a, b = _csub(v[0], v[2]), _csub(v[1], v[3])
                    back = _csub_i(a, b), _cadd_i(a, b)
                else:
                    a, b = _cadd(v[0], v[2]), _cadd(v[1], v[3])
                    back = _cadd(a, b), _csub(a, b)
                for j, spec in zip((odd, odd + 2), back):
                    recent = _mm(_cat(spec, 1), _bf(fxt_ref[j]))
                    y_ref[_rows(i - 3, 2), :, j] = recent.reshape(2, 4, 8, 128)
            yield recent
        if pending:
            butterflies(*pending)
        pending = (i, []) if i < NG else None
        for part in range(2):
            if pending:
                x = operands(i, pl.ds(XN, 4), fill)
                pending[1].append([_mm(x[j], _bf(fx_ref[j, part])) for j in range(4)])
                recent = pending[1][-1][0]
            yield recent
        for _ in fill:
            pass
    if pending:
        butterflies(*pending)


def _gate(lo, n, upd_ref, hot_ref, xp_ref, work_ref, y_ref, skip_ref, o_ref):
    for i in range(lo // 64, (lo + n) // 64):
        for p in range(4):
            r = []
            for j in range(4):
                x = _bf(xp_ref[p, j, _rows(i, 32), :]).astype(F32)
                half = work_ref[_rows(i, 8), p, XN + j].reshape(64, 128)
                s = (y_ref[_rows(i, 8), p, j].reshape(64, 128)
                     + half * skip_ref[_rows(i, 64), :])
                routed = _mm(upd_ref[_rows(i, 64), :], hot_ref[4 * p + j])
                r.append(x + s * _silu_of_twice(half + routed))
            r = _skew(r)
            r = [r[0]] + [pltpu.roll(r[q], 128 - q, 1) for q in range(1, 4)]
            o_ref[_rows(i, 64), _rows(p, 512)] = _cat(r, 1).astype(BF16)
            yield 64 * i, 512 * p


def _kernel(x_hbm, are_hbm, aim_hbm, bre_hbm, bim_hbm, cre_hbm, cim_hbm, ldt_hbm, dsk_hbm,
            wr_hbm, wg_hbm, wu_hbm, wd_hbm, o_hbm,
            x_ref, par_ref, ldt_ref, dsk_ref, wr_ref, wg_ref, wu_ref, wd_ref, o_ref,
            fx_ref, fxt_ref, fk_ref, fd_ref, dt_ref, skip_ref, base_ref, kv_ref, kr_ref,
            kf_ref, xp_ref, stat_ref, cen_ref, work_ref, xf_ref, y_ref,
            hot_ref, xs_ref, gate_ref, h_ref, upd_ref, sems):
    def copy(src, dst, sem, *part):
        if part:
            part = tuple(pl.ds(*p) for p in part)
            src, dst = src.at[part], dst.at[part]
        return pltpu.make_async_copy(src, dst, sems.at[sem])

    def params(sem, rows):
        return [copy(src, par_ref.at[i], sem, rows) for i, src in
                enumerate((are_hbm, aim_hbm, bre_hbm, bim_hbm, cre_hbm, cim_hbm))]

    def stream(*copies):
        for cp in copies:
            cp.start(priority=1)

    def wait(*copies):
        for cp in copies:
            cp.wait()

    def trickle(src, dst, sem, i, recent):
        dst[_rows(i, 8), pl.ds(0, 128)] = recent[:8].astype(BF16)
        copy(src.at[_rows(i, 8)], dst.at[_rows(i, 8)], sem).start()

    def with_trickle(jobs, count, phase):
        first = NG + sum(SHORT_PER_PHASE[:phase])
        pieces = short[first:first + SHORT_PER_PHASE[phase]]
        due = {k * count // len(pieces): piece for k, piece in enumerate(pieces)}
        assert len(due) == len(pieces)
        for n, recent in enumerate(jobs):
            if n in due:
                trickle(*due.pop(n), recent)
            yield
        assert not due

    def bulk(src, dst, sem, lo, hi, pieces):
        return copy(src, dst, sem, (lo + 8 * pieces, hi - lo - 8 * pieces))

    def whole(src, dst, sem, lo, hi, pieces):
        return copy(src, dst, sem, (lo, hi - lo))

    early, late = (SSM_UNROLL + 2) * G, CHUNKS[3][0]
    w_gate, w_up, w_down, w_last = weights = [w + (n,) for w, n in zip(
        ((wg_hbm, wg_ref, 0, 0, D), (wu_hbm, wu_ref, 1, 0, D),
         (wd_hbm, wd_ref, 2, 0, late), (wd_hbm, wd_ref, 0, late, D)), SHORT_PER_WEIGHT)]
    short = [(*w[:3], w[3] // 8 + i) for w in weights for i in range(w[5])]
    head = [copy(ldt_hbm, ldt_ref, 0)] + params(0, (0, early))
    rest = params(1, (early, D - early))
    inputs = [copy(x_hbm, x_ref, 2), copy(wr_hbm, wr_ref, 2), copy(dsk_hbm, dsk_ref, 2)]

    def wait_rest():
        wait(*rest)
        stream(bulk(*w_up))

    def wait_inputs():
        wait(*inputs)
        stream(bulk(*w_down))

    stream(*head, *rest, *inputs)
    _kernel_transform(fk_ref, fd_ref)
    _input_transform(fx_ref, fxt_ref)
    wait(*head)
    stream(bulk(*w_gate))
    _column(ldt_ref, dt_ref, lambda v: _round_bf16(jnp.exp(v)))
    zero = _ssm_kernel((wait_rest, wait_inputs), lambda *a: trickle(*w_gate[:3], *a),
                       par_ref, dt_ref, base_ref, kv_ref, kr_ref)

    def tally(p, j, n, value, first):
        kr_ref[p + zero, j, _rows(n, 8), :] = (
            value if first else kr_ref[p, j, _rows(n, 8), :] + value)

    def norm_pass(n, job, pieces, fine):
        count, batch = NORM_SHARE[n]
        first = sum(share[0] for share in NORM_SHARE[:n])
        steps = 4 * count // (1 if fine else batch)
        main = _ssm_spectrum(first, count, batch, fine, kr_ref, fk_ref, fd_ref, kf_ref)
        _weave(with_trickle(main, steps, n), job, pieces / (steps - 1))

    norm_pass(0, _norm_mean(x_ref, xp_ref, tally), 4 * NG // MEAN_GROUPS, True)
    for p, j in itertools.product(range(4), range(4)):
        stat_ref[0, p, j] = _average(kr_ref[p, j, _rows(0, 8), :])
        stat_ref[1, p, j] = _round_bf16(stat_ref[0, p, j])
    pl.when(zero < NG)(lambda: norm_pass(
        1, _norm_centre(xp_ref, cen_ref, stat_ref, tally), 16 * NG // VAR_GROUPS, True))
    for p, j in itertools.product(range(4), range(4)):
        stat_ref[0, p, j] = _norm_factor(kr_ref[p, j, _rows(1, 8), :], stat_ref[0, p, j])
    wait(whole(*w_gate))
    stream(bulk(*w_last))
    norm_pass(2, _norm_scale(wr_ref, cen_ref, stat_ref, work_ref), 20, False)

    def convolve(n):
        first, stop = CONV_CUTS[n:n + 2]
        steps = _convolve(first, stop, zero, kf_ref, fx_ref, fxt_ref, xf_ref, work_ref, y_ref)
        return with_trickle(steps, 4 * (stop - first), 3 + n)

    def ffn_down(i):
        return _ffn_down(*CHUNKS[i], h_ref, wd_ref, gate_ref, upd_ref)

    def gate_and_send(chunk):
        for row, col in _gate(*chunk, upd_ref, hot_ref, xp_ref, work_ref, y_ref, skip_ref,
                              o_ref):
            stream(copy(o_ref, o_hbm, 1, (row, 64), (col, 512)))
            yield

    _weave(convolve(0), itertools.chain(
        _route(stat_ref, work_ref, hot_ref, xs_ref, gate_ref),
        _ffn_up(False, xs_ref, wg_ref, h_ref)))
    wait(whole(*w_up))
    _column(dsk_ref, skip_ref, lambda v: 2.0 * v)
    _weave(convolve(1), _ffn_up(True, xs_ref, wu_ref, h_ref))
    wait(whole(*w_down))
    _weave(convolve(2), ffn_down(0))
    for i, chunk in enumerate(CHUNKS):
        if chunk[0] + chunk[1] == late:
            wait(whole(*w_last))
        _weave(gate_and_send(chunk),
               ffn_down(i + 1) if i + 1 < len(CHUNKS) else iter(()), DOWN_RATE)
    wait(copy(o_ref, o_hbm, 1))


@jax.jit
def pallas_recurrent_scan__ssm_conv_s4__moe_arch_mod__prompt_kernel(
    A_u: jax.Array,
    A_A_re: jax.Array,
    A_A_im: jax.Array,
    A_B_re: jax.Array,
    A_B_im: jax.Array,
    A_C_re: jax.Array,
    A_C_im: jax.Array,
    A_log_dt: jax.Array,
    A_Dskip: jax.Array,
    B_x: jax.Array,
    B_w_r: jax.Array,
    B_w_gate: jax.Array,
    B_w_up: jax.Array,
    B_w_down: jax.Array,
):
    del B_x
    assert A_u.shape == (1, L, D) and A_A_re.shape == (D, N) and B_w_gate.shape == (D, F)
    assert A_A_re.dtype == BF16
    vmem = pltpu.VMEM
    scratch = [
        vmem((D, L), BF16), vmem((6, D, N), BF16),
        vmem((D,), BF16), vmem((D,), BF16), vmem((D,), BF16),
        vmem((D, F), BF16), vmem((D, F), BF16), vmem((D, F), BF16), vmem((D, L), BF16),
        vmem((4, 2, 64, 128), I32), vmem((4, 128, 128), I32),
        vmem((4, 2, 64, 128), I32), vmem((4, 2, 64, 128), I32),
        vmem((D, 128), F32), vmem((D, 128), F32),
        vmem((4, 2, 144, 128), F32), vmem((4, 2, 96, 128), F32),
        vmem((NH + 4, 5, 16, 128), F32), vmem((4 * NH, 8, 8, 128), F32),
        vmem((4, 4, D // 2, 128), I32), vmem((2, 4, 4, 8, 128), F32),
        vmem((4, 4, NG, 8, 256), BF16),
        vmem((NH, 4, XN + 4, 8, 128), F32), vmem((4 * NH, 8, 8, 128), F32),
        vmem((NH, 4, 4, 8, 128), F32),
        vmem((16, 8, 128), F32), vmem((8, D), F32), vmem((8, 128), F32), vmem((8, F), F32),
        vmem((D, TOPK), F32),
        pltpu.SemaphoreType.DMA((3,)),
    ]
    out = pl.pallas_call(
        _kernel,
        out_shape=jax.ShapeDtypeStruct((D, L), BF16),
        in_specs=[pl.BlockSpec(memory_space=pl.ANY)] * 13,
        out_specs=pl.BlockSpec(memory_space=pl.ANY),
        scratch_shapes=scratch,
        compiler_params=pltpu.CompilerParams(vmem_limit_bytes=100 * 1024 * 1024),
    )(A_u.reshape(L, D).T, A_A_re, A_A_im, A_B_re, A_B_im, A_C_re, A_C_im, A_log_dt,
      A_Dskip, B_w_r, B_w_gate, B_w_up, B_w_down.T)
    return out.T.reshape(1, L, D)
```

```python
import itertools
import math

import jax
import jax.numpy as jnp
from jax import lax
import jax.experimental.pallas as pl
import jax.experimental.pallas.tpu as pltpu

F32, BF16, I32 = jnp.float32, jnp.bfloat16, jnp.int32
L, D, N, F, TOPK = 2048, 576, 128, 4608, 8
EPS = 1e-5
G = 16
NG = D // G
NH = D // 8
NN = (((1,), (0,)), ((), ()))
NT = (((1,), (1,)), ((), ()))

SSM_UNROLL = 8
MEAN_GROUPS, VAR_GROUPS = 3, 6
CHUNK, LATE = 128, 384


def _iota(shape, dim):
    return lax.broadcasted_iota(I32, shape, dim)


def _rows(i, n):
    return pl.ds(i * n, n)


def _unrolled(first, stop, body, carry=None):
    return lax.fori_loop(first, stop, body, carry, unroll=True)


def _cat(xs, axis=0):
    return jnp.concatenate(xs, axis=axis)


def _cmul(a, b):
    return a[0] * b[0] - a[1] * b[1], a[0] * b[1] + a[1] * b[0]


def _csq(a):
    return a[0] * a[0] - a[1] * a[1], (a[0] + a[0]) * a[1]


def _cadd(a, b):
    return a[0] + b[0], a[1] + b[1]


def _csub(a, b):
    return a[0] - b[0], a[1] - b[1]


def _cadd_i(a, b):
    return a[0] - b[1], a[1] + b[0]


def _csub_i(a, b):
    return a[0] + b[1], a[1] - b[0]


def _dft4(v):
    s02, d02 = _cadd(v[0], v[2]), _csub(v[0], v[2])
    s13, d13 = _cadd(v[1], v[3]), _csub(v[1], v[3])
    return [_cadd(s02, s13), _cadd_i(d02, d13), _csub(s02, s13), _csub_i(d02, d13)]


def _root(n):
    ang = (((n + 1024) & 2047) - 1024).astype(F32) * (2.0 * math.pi / 2048)
    return jnp.cos(ang), jnp.sin(ang)


def _powers(start, step, count):
    vals = [start]
    for _ in range(count - 1):
        vals.append(_cmul(vals[-1], step))
    return vals


def _pack(x):
    return pltpu.bitcast(x.astype(BF16), I32)


def _bf(x):
    return pltpu.bitcast(x, BF16)


def _round_bf16(x):
    return x.astype(BF16).astype(F32)


def _silu_of_twice(h):
    return h + h * jnp.tanh(h)


def _mm(a, b, dims=NN):
    return lax.dot_general(a, b, dims, precision=lax.Precision.DEFAULT,
                           preferred_element_type=F32)


def _skew(r):
    lane = _iota(r[0].shape, 1)
    b0, b1 = (lane & 1) != 0, (lane & 2) != 0
    t = [lax.select(b0, r[(k + 1) % 4], r[k]) for k in range(4)]
    u = [lax.select(b1, t[(k + 2) % 4], t[k]) for k in range(4)]
    return [u[(-j) % 4] for j in range(4)]


def _x_time(j, m):
    q = (m - j) & 3
    return 128 * q + ((m - q) & 127)


def _weave(main, side, rate=1.0):
    credit = 0.0
    for _ in main:
        credit += rate
        while credit >= 1.0:
            credit -= 1.0
            next(side, None)
    for _ in side:
        pass


def _column(v_ref, out_ref, fn):
    v = fn(v_ref[...].astype(F32).reshape(1, D))
    for lo in range(0, D, 128):
        n = min(128, D - lo)
        out_ref[pl.ds(lo, n), :] = jnp.broadcast_to(v[:, lo:lo + n], (128, n)).T


def _input_transform(fx_ref, fxt_ref):
    freq, row = 4 * _iota((8, 128), 1) + 1, _iota((8, 128), 0)
    step8 = _root(8 * freq)
    step128 = _csq(_csq(_csq(_csq(step8))))
    for j in range(4):
        start = _root((_x_time(j, row + 8) - 8) * freq)
        vals = _powers(start, step8, 16)
        wraps = row < ((row - j) & 3)
        vals[0] = tuple(jnp.where(wraps, a, b) for a, b in zip(_cmul(start, step128), start))
        for part in range(2):
            m = _cat([v[part] for v in vals])
            fx_ref[j, part] = _pack(m)
            fxt_ref[j, pl.ds(64 * part, 64), :] = _pack(m.T)


def _kernel_transform(fk_ref, fd_ref):
    freq, row = 4 * _iota((8, 128), 1) + 1, _iota((8, 128), 0)
    rho = _root(freq)
    step32 = _csq(_csq(_csq(_csq(_csq(rho)))))
    for j, start in enumerate(_powers(_root(4 * row * freq), rho, 4)):
        vals = _powers(start, step32, 16)
        for part in range(2):
            fk_ref[j, part] = _pack(_cat([v[part] for v in vals]))
    rows = _powers(_root((256 * (row & 1) + 8 * (row >> 1)) * freq), step32, 8)
    first = row == 0
    for k in range(4):
        p2 = _csq(rho)
        s3 = _cadd(_cadd(rho, p2), _cmul(p2, rho))
        s4 = _cadd(s3, _csq(p2))
        box = 1.0 + 2.0 * jnp.where((row & 2) == 0, s4[0], s3[0])
        vals = [(r[0] * box, r[1] * box) for r in rows]
        vals[0] = (jnp.where(first, 1.0 + s4[0], vals[0][0]),
                   jnp.where(first, s4[1], vals[0][1]))
        vals.append((jnp.where(first, s4[1], 0.0), jnp.where(first, s4[0], 0.0)))
        for part in range(2):
            fd_ref[k, part, pl.ds(0, 40), :] = _pack(
                _cat([v[part] for v in vals] + [jnp.zeros((8, 128), F32)]))
            fd_ref[k, part, pl.ds(40, 24), :] = jnp.zeros((24, 128), I32)
        rho = (-rho[1], rho[0])


def _ssm_bases(g, h, par_ref, dt_ref, base_ref):
    a_re, a_im, b_re, b_im, c_re, c_im = (
        par_ref[k, _rows(g, G), :].astype(F32) for k in range(6))
    dt = dt_ref[_rows(g, G), :]
    dts = dt * (2.0 / 512)
    row = _iota((8, 128), 0)

    def deal(v):
        return _cat([jnp.take_along_axis(v[lo:lo + 8], (row >> 1) + 4 * (row & 1), axis=0,
                                         mode="promise_in_bounds") for lo in (0, 8)])

    decay, phase = deal(dt * a_re), deal(dt * a_im)
    w = tuple(deal(v) for v in _cmul((c_re, c_im), (dts * b_re, dts * b_im)))
    z, unit = {}, (jnp.cos(phase), jnp.sin(phase))
    for e in (1, 2, 4, 8, 16, 32, 64, 128, 256):
        if e in (1, 4, 8, 16, 256):
            mag = jnp.exp2(decay * (e * math.log2(math.e)))
            z[e] = (mag * unit[0], mag * unit[1])
        if e < 256:
            unit = _csq(unit)
    z1024 = _csq(_csq(z[256]))
    w8, w1024 = _cmul(w, z[8]), _cmul(w, z1024)
    seq = [(jnp.ones_like(dt), jnp.zeros_like(dt)), z[8], z[16], z[16], _cmul(z[16], z[8]),
           z[1], z[1], z[256], z[256], w, _cmul(w, z[4]), w,
           w8, w1024, w8, w1024, _cmul(w1024, z1024), w1024]
    for k, v in enumerate(seq):
        for t in range(2):
            for part in range(2):
                base_ref[h + t, part, pl.ds(8 * k, 8), :] = v[part][8 * t:8 * t + 8]


_OFFSETS = ((0, 4), (1, 5), (2, 6), (3, 7), (258, 262), (256, 260), (512, 516), (768, 772),
            (264, 1280), (520, 1536), (776, 1792), (1024, 2048))


def _ssm_values(h, base_ref, kv_ref):
    for quad in range(2):
        def pair(k):
            return tuple(base_ref[h, part, pl.ds(8 * k + quad, 8, stride=2), :]
                         for part in range(2))

        v = [pair(0)] + _powers(pair(3), pair(2), 15)
        z256 = pair(7)
        w = _powers(pair(9 + quad), pair(5), 4)
        w += [_cmul(w[2], z256)] + _powers(w[0], z256, 4)[1:]
        w += _powers(pair(12 + quad), z256, 4)[1:] + [pair(15 + quad)]
        re, im = (_mm(_cat([t[part] for t in w]), _cat([t[part] for t in v[::-1]]), NT)
                  for part in range(2))
        kv_ref[h, quad] = re - im


def _ssm_arrange(h, slot, kv_ref, kr_ref):
    lane, row = _iota((8, 128), 1), _iota((8, 128), 0)
    src = 4 * (((lane >> 1) & 31) ^ 30) + (row & 3)
    top = row < 4

    def spread(x):
        return jnp.take_along_axis(x, src, axis=1, mode="promise_in_bounds")

    def even(a, b):
        return jnp.where((lane & 1) == 0, a, b)

    def low(a, b):
        return jnp.where(lane < 64, a, b)

    val = {}
    for u, (e0, e1) in enumerate(_OFFSETS):
        a, b = (kv_ref[h, quad, pl.ds(8 * u, 8), :] for quad in range(2))
        val[e0] = spread(jnp.where(top, a, b))
        val[e1] = spread(pltpu.roll(jnp.where(top, b, a), 4, 0))
    mid = even(val[256], val[260])
    q0, q4, q8 = low(val[512], val[768]), low(val[516], val[772]), low(val[520], val[776])
    blocks = [
        (low(even(val[0], val[4]), mid), even(q0, q4)),
        (low(even(val[1], val[5]), mid), even(q0, q4)),
        (low(even(val[2], val[6]), even(val[258], val[262])), even(q0, q8)),
        (low(even(val[3], val[7]), even(val[260], val[264])), even(q4, q8)),
        (low(even(val[1024], val[1280]), val[1536]),
         low(even(val[1536], val[1792]), jnp.where(lane == 64, val[2048], 0.0)))]
    for j, pair in enumerate(blocks):
        kr_ref[slot, j] = _cat(pair)


def _ssm_kernel(waits, every_group, par_ref, dt_ref, base_ref, kv_ref, kr_ref):
    def steps(g0, count, ahead=True):
        def step(r, carry):
            g, slot = g0 + r, 2 * (r & 1)

            def half(t, carry):
                _ssm_arrange(slot + t, 2 * g + t, kv_ref, kr_ref)
                _ssm_values(slot + t, base_ref, kv_ref)

            _unrolled(0, 2, half)
            every_group(g, kv_ref[slot, 0, pl.ds(0, 8), :])
            if ahead:
                _ssm_bases(g + 2, slot, par_ref, dt_ref, base_ref)

        _unrolled(0, count, step)

    def body(n, zero):
        pl.when(n == 1)(waits[0])
        steps(n * SSM_UNROLL, SSM_UNROLL)
        return jnp.minimum(zero, n * L)

    _unrolled(0, 2, lambda g, _: _ssm_bases(g, 2 * g, par_ref, dt_ref, base_ref))
    kv_ref[...] = jnp.zeros_like(kv_ref)
    trips = (NG - 2) // SSM_UNROLL
    zero = lax.fori_loop(0, trips, body, L)
    waits[1]()
    steps(trips * SSM_UNROLL, NG - 2 - trips * SSM_UNROLL)
    steps(NG - 2, 2, ahead=False)
    _unrolled(0, 4, lambda h, _: _ssm_arrange(h, NH + h, kv_ref, kr_ref))
    return zero


def _ssm_spectrum(h0, batches, fine, recent, kr_ref, fk_ref, fd_ref, kf_ref):
    for batch in batches:
        near, far = [], []
        for n in range(4):
            lhs = {j: [] for j in ((0, 1, 2, 3) if n < 2 else (4,))}
            for h in range(batch):
                for j, rows in lhs.items():
                    rows.append(kr_ref[4 + h0 + h, j])
                if fine:
                    yield
            if n < 2:
                near.append([_mm(_cat(lhs[j]), _bf(fk_ref[j, n])) for j in range(4)])
            else:
                far += [[_mm(_cat(lhs[4]), _bf(fd_ref[k, part])) for part in range(2)]
                        for k in (2 * n - 4, 2 * n - 3)]
            if not fine:
                yield
        recent.append(near[0][0])

        def blocks(x):
            x = x.reshape(batch, 2, 1, 8, 128)
            return x[:, :1], x[:, 1:]

        out = []
        for a, b in zip(_dft4(list(zip(*near))), far):
            spec = list(zip(*(blocks(a[part]) + blocks(b[part]) for part in range(2))))
            spec = spec[:1] + [_csub_i(spec[p], spec[p - 1]) for p in range(1, 4)]
            out += [_cat(v, 1) for v in zip(*spec)]
        kf_ref[pl.ds(4 * h0, 4 * batch)] = _cat(out, 2).reshape(4 * batch, 8, 8, 128)
        h0 = h0 + batch


XN = 8


def _fold(x):
    x = x.reshape(3, -1, 8, 128)
    x = x[0] + x[1] + x[2]
    while x.shape[0] > 1:
        x = x[:x.shape[0] // 2] + x[x.shape[0] // 2:]
    return x[0]


def _norm_mean(n, x_ref, xp_ref, tally):
    for i, p in itertools.product((2 * n, 2 * n + 1), range(4)):
        r = [pltpu.bitcast(x_ref[_rows(i, MEAN_GROUPS * G), _rows(4 * p + q, 128)], I32)
             for q in range(4)]
        r = _skew([r[0]] + [pltpu.roll(r[q], q, 1) for q in range(1, 4)])
        for j in range(4):
            xp_ref[p, j, _rows(i, MEAN_GROUPS * 8), :] = r[j]
            tally(p, j, 0, _fold(_bf(r[j]).astype(F32)))
        yield


def _norm_centre(i, xp_ref, cen_ref, stat_ref, tally):
    for p, j in itertools.product(range(4), range(4)):
        x = _bf(xp_ref[p, j, _rows(i, VAR_GROUPS * 8), :]).astype(F32)
        d = x.reshape(VAR_GROUPS, G, 128) - _cat([stat_ref[1, p, j]] * 2)
        cen_ref[p, j, _rows(i, VAR_GROUPS)] = _cat([d[:, :8], d[:, 8:]], 2).astype(BF16)
        tally(p, j, 1, _fold(d * d))
        yield


def _average(v):
    return jnp.broadcast_to(jnp.sum(v, axis=-2, keepdims=True), v.shape) / D


def _norm_factor(squares, mean):
    shift = mean - _round_bf16(mean)
    var = _round_bf16(jnp.maximum(_average(squares) - shift * shift, 0.0))
    eps = _round_bf16(jnp.full_like(var, EPS))
    return 0.5 / _round_bf16(jnp.sqrt(_round_bf16(var + eps)))


def _norm_scale(i, wr_ref, cen_ref, stat_ref, work_ref):
    wr = jnp.broadcast_to(2.0 * wr_ref[...].astype(F32).reshape(1, D), (8, D))
    for p in (2 * i, 2 * i + 1):
        score = [None] * 4
        for lo in range(0, D, 128):
            n = min(128, D - lo)
            for j in range(4):
                d = cen_ref[p, j, pl.ds(lo // G, n // G)].astype(F32)
                half = _cat([d[:, :, :128], d[:, :, 128:]], 1).reshape(n // 8, 8, 128)
                half = half * stat_ref[0, p, j]
                work_ref[pl.ds(lo // 8, n // 8), p, XN + j] = half
                part = _mm(wr[:, lo:lo + n], half.reshape(n, 128))
                score[j] = part if lo == 0 else score[j] + part
            yield
        for j in range(4):
            stat_ref[1, p, j] = score[j]


def _route(stat_ref, hot_ref, gate_ref):
    row, blk = _iota((8, 128), 0), _iota((16, 128), 0)
    halves = []
    for lo in (0, 2):
        dense = stat_ref[1, lo, 0]
        for c in range(1, 8):
            dense = jnp.where(row == c, stat_ref[1, lo + c // 4, c % 4], dense)
        halves.append(dense)
    score = _round_bf16(_cat(halves))
    bits = pltpu.bitcast(jnp.where(score == 0.0, 0.0, score), I32) >> 16
    order = jnp.where(bits < 0, bits ^ 0x7FFF, bits) + 0x8000
    time = 512 * (blk >> 2) + _x_time(blk & 3, _iota((16, 128), 1))
    key = pltpu.bitcast((1 << 29) + (order << 11) + (L - 1 - time), F32)
    rank = jnp.full((16, 128), TOPK, I32)
    best = jnp.zeros((8, 128), F32)
    for i in range(TOPK):
        top = jnp.max(jnp.max(key, axis=0, keepdims=True), axis=1, keepdims=True)
        hit = key == top
        rank = jnp.where(hit, i, rank)
        key = jnp.where(hit, 0.0, key)
        best = jnp.where(row == i, top, best)
    order = ((pltpu.bitcast(best, I32) >> 11) & 0xFFFF) - 0x8000
    best = pltpu.bitcast(jnp.where(order < 0, order ^ 0x7FFF, order) << 16, F32)
    gate_ref[...] = 0.5 * _round_bf16(jax.nn.sigmoid(best))
    for c in range(16):
        hot_ref[c] = jnp.where(jnp.broadcast_to(rank[c:c + 1], (8, 128)) == row, 1.0, 0.0)


def _gather(i, n, work_ref, hot_ref, xs_ref):
    picked = None
    for p in range(4):
        for j in range(4):
            tokens = work_ref[pl.ds(16 * i, n // 8), p, XN + j].reshape(n, 128)
            part = _mm(hot_ref[4 * p + j], tokens, NT)
            picked = part if picked is None else picked + part
        yield
    xs_ref[:, pl.ds(128 * i, n)] = 2.0 * picked


def _ffn_up(i, second, xs_ref, w_ref, h_ref):
    acc, cols = None, _rows(i, 512)
    for lo in range(0, D, 128):
        rows = pl.ds(lo, min(128, D - lo))
        part = _mm(xs_ref[:, rows], w_ref[rows, cols])
        acc = part if lo == 0 else acc + part
        yield
    acc = _round_bf16(acc)
    h_ref[:, cols] = (h_ref[:, cols] * acc if second
                      else _round_bf16(_silu_of_twice(0.5 * acc)))


def _ffn_down(lo, n, h_ref, wd_ref, gate_ref, upd_ref):
    ffn = None
    for k in range(0, F, 512):
        part = _mm(h_ref[:, pl.ds(k, 512)], wd_ref[pl.ds(lo, n), pl.ds(k, 512)], NT)
        ffn = part if ffn is None else ffn + part
        yield
    yield from range(3)
    eye = jnp.where(_iota((n, n), 0) == _iota((n, n), 1), 1.0, 0.0)
    upd_ref[pl.ds(lo, n), :] = _mm(eye, _round_bf16(ffn) * gate_ref[:, :n], NT)


def _conv_finish_forward(g, comp, zero, xf_ref):
    spec = [v.reshape(8, 1, 8, 128) for pair in _dft4(list(zip(*comp))) for v in pair]
    xf_ref[pl.ds(8 * g + zero, 8)] = _cat(spec, 1)


def _conv_step(i, live, before, comp, zero, kf_ref, fx_ref, fxt_ref, xf_ref, work_ref,
               y_ref):
    def products(g):
        for h, k in itertools.product((2 * g, 2 * g + 1), range(4)):
            kf, x = ([tuple(ref[4 * h + p, 2 * k + part] for part in range(2))
                      for p in range(4)] for ref in (kf_ref, xf_ref))
            for c in (3, 0, 2, 1):
                acc = _cmul(kf[0], x[c])
                for p in range(1, c + 1):
                    acc = _cadd(acc, _cmul(kf[p], x[c - p]))
                for part in range(2):
                    work_ref[h + zero, c, 2 * k + part] = acc[part]
                if c < 2:
                    yield

    def operands(g, slots):
        rows = []
        for h, p in itertools.product((2 * g, 2 * g + 1), range(4)):
            rows.append(work_ref[h, pl.ds(p, 1), slots])
            if p % 2:
                next(fill, None)
        rows = _cat(rows)
        return [rows[:, s].reshape(64, 128) for s in range(slots.size)]

    fill = products(i - 2) if live[1] else iter(())
    for odd in range(2):
        if live[2]:
            v = operands(i - 3, pl.ds(0, XN))
            v = list(zip(v[0::2], v[1::2]))
            if odd:
                a, b = _csub(v[0], v[2]), _csub(v[1], v[3])
                back = _csub_i(a, b), _cadd_i(a, b)
            else:
                a, b = _cadd(v[0], v[2]), _cadd(v[1], v[3])
                back = _cadd(a, b), _csub(a, b)
            for j, spec in zip((odd, odd + 2), back):
                y = _mm(_cat(spec, 1), _bf(fxt_ref[j]))
                y_ref[_rows(i - 3, 2), :, j] = y.reshape(2, 4, 8, 128)
        yield
    if before:
        _conv_finish_forward(i - 1, before, zero, xf_ref)
    for part in range(2):
        if live[0]:
            x = operands(i, pl.ds(XN, 4))
            comp.append([_mm(x[j], _bf(fx_ref[j, part])) for j in range(4)])
        yield
    for _ in fill:
        pass


def _gate(i, p, upd_ref, hot_ref, xp_ref, work_ref, y_ref, skip_ref, o_ref):
    r = []
    for j in range(4):
        x = _bf(xp_ref[p, j, _rows(i, 32), :]).astype(F32)
        half = work_ref[_rows(i, 8), p, XN + j].reshape(64, 128)
        s = y_ref[_rows(i, 8), p, j].reshape(64, 128) + half * skip_ref[_rows(i, 64), :]
        routed = _mm(upd_ref[_rows(i, 64), :], hot_ref[4 * p + j])
        r.append(x + s * _silu_of_twice(half + routed))
    r = _skew(r)
    r = [r[0]] + [pltpu.roll(r[q], 128 - q, 1) for q in range(1, 4)]
    o_ref[_rows(i, 64), _rows(p, 512)] = _cat(r, 1).astype(BF16)


def _kernel(x_hbm, are_hbm, aim_hbm, bre_hbm, bim_hbm, cre_hbm, cim_hbm, ldt_hbm, dsk_hbm,
            wr_hbm, wg_hbm, wu_hbm, wd_hbm, o_hbm,
            x_ref, par_ref, ldt_ref, dsk_ref, wr_ref, wg_ref, wu_ref, wd_ref, o_ref,
            fx_ref, fxt_ref, fk_ref, fd_ref, dt_ref, skip_ref, base_ref, kv_ref, kr_ref,
            kf_ref, xp_ref, stat_ref, cen_ref, work_ref, xf_ref, y_ref,
            hot_ref, xs_ref, gate_ref, h_ref, upd_ref, sems):
    def copy(src, dst, sem, *part):
        if part:
            part = tuple(pl.ds(*p) for p in part)
            src, dst = src.at[part], dst.at[part]
        return pltpu.make_async_copy(src, dst, sems.at[sem])

    def params(sem, rows):
        return [copy(src, par_ref.at[i], sem, rows) for i, src in
                enumerate((are_hbm, aim_hbm, bre_hbm, bim_hbm, cre_hbm, cim_hbm))]

    def stream(*copies):
        for cp in copies:
            cp.start(priority=1)

    def wait(*copies):
        for cp in copies:
            cp.wait()

    def trickle(src, dst, sems_of, i, recent):
        sem = jnp.where(8 * i < LATE, *sems_of)
        dst[_rows(i, 8), pl.ds(0, 128)] = recent[:8].astype(BF16)
        copy(src.at[_rows(i, 8)], dst.at[_rows(i, 8)], sem).start()

    def rows_of(weight, lo=0, hi=D):
        return copy(*weight[:2], weight[2][lo >= LATE], (lo, hi - lo))

    w_gate, w_up = (wg_hbm, wg_ref, (0, 0)), (wu_hbm, wu_ref, (1, 1))
    w_down = (wd_hbm, wd_ref, (2, 0))
    early = (SSM_UNROLL + 2) * G
    head = [copy(ldt_hbm, ldt_ref, 0)] + params(0, (0, early))
    rest = params(1, (early, D - early))
    inputs = [copy(x_hbm, x_ref, 2), copy(wr_hbm, wr_ref, 2), copy(dsk_hbm, dsk_ref, 2)]

    def wait_rest():
        wait(*rest)
        stream(rows_of(w_up, 8 * 23))

    def wait_inputs():
        wait(*inputs)
        stream(rows_of(w_down, 0, 8 * 32))

    stream(*head, *rest, *inputs)
    _kernel_transform(fk_ref, fd_ref)
    _input_transform(fx_ref, fxt_ref)
    wait(*head)
    stream(rows_of(w_gate, 8 * (NG + 6)))
    _column(ldt_ref, dt_ref, lambda v: _round_bf16(jnp.exp(v)))
    zero = _ssm_kernel((wait_rest, wait_inputs), lambda *a: trickle(*w_gate, *a),
                       par_ref, dt_ref, base_ref, kv_ref, kr_ref)

    def tally(p, j, n, value):
        kr_ref[p + zero, j, _rows(n, 8), :] = kr_ref[p, j, _rows(n, 8), :] + value

    def norm_pass(h0, trips, batches, fine, job, pieces, weight, first, per_trip=1):
        def body(i, carry):
            recent = []
            main = _ssm_spectrum(h0 + i * sum(batches), batches, fine, recent, kr_ref,
                                 fk_ref, fd_ref, kf_ref)
            _weave(main, job(i), pieces / (4 * (sum(batches) if fine else len(batches))))
            for k in range(per_trip):
                trickle(*weight, first + i * per_trip + k, recent[k])

        _unrolled(0, trips, body)

    norm_pass(0, 6, (2, 2), True, lambda i: _norm_mean(i, x_ref, xp_ref, tally), 8,
              w_gate, NG)
    stat_ref[0] = _average(kr_ref[0:4, 0:4, 0:8, :])
    stat_ref[1] = _round_bf16(stat_ref[0])
    pl.when(zero < NG)(lambda: norm_pass(
        24, 6, (3, 2), True, lambda i: _norm_centre(i, xp_ref, cen_ref, stat_ref, tally), 16,
        w_up, 0))
    stat_ref[0] = _norm_factor(kr_ref[0:4, 0:4, 8:16, :], stat_ref[0])
    wait(rows_of(w_gate))
    stream(rows_of(w_down, 8 * 51))
    norm_pass(54, 2, (3, 3, 3), False,
              lambda i: _norm_scale(i, wr_ref, cen_ref, stat_ref, work_ref), 10, w_up, 6, 3)

    def conv_steps(first, stop, comp):
        for i in range(first, stop):
            before, comp[:] = comp[:], []
            yield from _conv_step(i, [0 <= i - k < NG for k in (0, 2, 3)], before, comp,
                                  zero, kf_ref, fx_ref, fxt_ref, xf_ref, work_ref, y_ref)

    def convolve(first, stop, before, weight, piece, side=lambda n: iter(()), rate=1.0):
        def body(i, before):
            comp = []
            _weave(_conv_step(i, [True] * 3, before, comp, zero, kf_ref, fx_ref, fxt_ref,
                              xf_ref, work_ref, y_ref), side(i - first), rate)
            trickle(*weight, piece + i - first, comp[0][0])
            return comp

        return body(first, before) if stop == first + 1 else _unrolled(
            first, stop, body, before)

    _route(stat_ref, hot_ref, gate_ref)
    comp = []
    _weave(conv_steps(0, 3, comp), iter(()))
    comp = convolve(3, 9, comp, w_up, 12)
    comp = convolve(9, 13, comp, w_up, 18,
                    lambda n: _gather(n, 128, work_ref, hot_ref, xs_ref))
    comp = convolve(13, 14, comp, w_up, 22,
                    lambda n: _gather(4, 64, work_ref, hot_ref, xs_ref))
    comp = convolve(14, 23, comp, w_down, 32,
                    lambda n: _ffn_up(n, False, xs_ref, wg_ref, h_ref), 1.25)
    _conv_finish_forward(22, comp, zero, xf_ref)
    wait(rows_of(w_up))
    _column(dsk_ref, skip_ref, lambda v: 2.0 * v)
    comp = convolve(23, 24, None, w_down, 41)
    comp = convolve(24, 33, comp, w_down, 42,
                    lambda n: _ffn_up(n, True, xs_ref, wu_ref, h_ref), 1.25)
    _conv_finish_forward(32, comp, zero, xf_ref)
    wait(rows_of(w_down, 0, LATE))

    def ffn_down(lo, n):
        return _ffn_down(lo, n, h_ref, wd_ref, gate_ref, upd_ref)

    def gate_and_send(first, count):
        for i, p in itertools.product(range(count), range(4)):
            _gate(first + i, p, upd_ref, hot_ref, xp_ref, work_ref, y_ref, skip_ref, o_ref)
            stream(copy(o_ref, o_hbm, 1, ((first + i) * 64, 64), (512 * p, 512)))
            yield

    def finish(i, ahead):
        _weave(gate_and_send(2 * i, 2), ffn_down((i + 1) * CHUNK, ahead), 2.0)

    _weave(conv_steps(33, NG + 3, []), ffn_down(0, CHUNK))
    _unrolled(0, 2, lambda i, _: finish(i, CHUNK))
    wait(rows_of(w_down, LATE))
    finish(2, CHUNK)
    finish(3, D % CHUNK)
    _weave(gate_and_send(8, 1), iter(()))
    wait(copy(o_ref, o_hbm, 1))


@jax.jit
def pallas_recurrent_scan__ssm_conv_s4__moe_arch_mod__prompt_kernel(
    A_u: jax.Array,
    A_A_re: jax.Array,
    A_A_im: jax.Array,
    A_B_re: jax.Array,
    A_B_im: jax.Array,
    A_C_re: jax.Array,
    A_C_im: jax.Array,
    A_log_dt: jax.Array,
    A_Dskip: jax.Array,
    B_x: jax.Array,
    B_w_r: jax.Array,
    B_w_gate: jax.Array,
    B_w_up: jax.Array,
    B_w_down: jax.Array,
):
    del B_x
    assert A_u.shape == (1, L, D) and A_A_re.shape == (D, N) and B_w_gate.shape == (D, F)
    assert A_A_re.dtype == BF16
    vmem = pltpu.VMEM
    scratch = [
        vmem((D, L), BF16), vmem((6, D, N), BF16),
        vmem((D,), BF16), vmem((D,), BF16), vmem((D,), BF16),
        vmem((D, F), BF16), vmem((D, F), BF16), vmem((D, F), BF16), vmem((D, L), BF16),
        vmem((4, 2, 64, 128), I32), vmem((4, 128, 128), I32),
        vmem((4, 2, 64, 128), I32), vmem((4, 2, 64, 128), I32),
        vmem((D, 128), F32), vmem((D, 128), F32),
        vmem((4, 2, 144, 128), F32), vmem((4, 2, 96, 128), F32),
        vmem((NH + 4, 5, 16, 128), F32), vmem((4 * NH, 8, 8, 128), F32),
        vmem((4, 4, D // 2, 128), I32), vmem((2, 4, 4, 8, 128), F32),
        vmem((4, 4, NG, 8, 256), BF16),
        vmem((NH, 4, XN + 4, 8, 128), F32), vmem((4 * NH, 8, 8, 128), F32),
        vmem((NH, 4, 4, 8, 128), F32),
        vmem((16, 8, 128), F32), vmem((8, D), F32), vmem((8, 128), F32), vmem((8, F), F32),
        vmem((D, TOPK), F32),
        pltpu.SemaphoreType.DMA((3,)),
    ]
    out = pl.pallas_call(
        _kernel,
        out_shape=jax.ShapeDtypeStruct((D, L), BF16),
        in_specs=[pl.BlockSpec(memory_space=pl.ANY)] * 13,
        out_specs=pl.BlockSpec(memory_space=pl.ANY),
        scratch_shapes=scratch,
        compiler_params=pltpu.CompilerParams(vmem_limit_bytes=100 * 1024 * 1024),
    )(A_u.reshape(L, D).T, A_A_re, A_A_im, A_B_re, A_B_im, A_C_re, A_C_im, A_log_dt,
      A_Dskip, B_w_r, B_w_gate, B_w_up, B_w_down.T)
    return out.T.reshape(1, L, D)
```
